```python
import jax
import jax.numpy as jnp

def _softmax(x, axis=-1):
    return jax.nn.softmax(x, axis=axis)
def _gelu(x):
    return jax.nn.gelu(x, approximate=True)
def _silu(x):
    return jax.nn.silu(x)
def _sigmoid(x):
    return jax.nn.sigmoid(x)
def _layernorm(x, axis=-1, eps=1e-5):
    m = jnp.mean(x, axis=axis, keepdims=True)
    v = jnp.var(x, axis=axis, keepdims=True)
    return (x - m) / jnp.sqrt(v + eps)
def _scatter_add(tgt, idx, src, axis=0):
    return tgt.at[idx].add(src)
def _segment_sum(src, seg, n):
    return jax.ops.segment_sum(src, seg, n)
class _Rng:
    def __init__(self, key):
        self._k = key
    def _next(self):
        self._k, sub = jax.random.split(self._k)
        return sub
    def normal(self, shape):
        return jax.random.normal(self._next(), shape, dtype=jnp.bfloat16)
    def randint(self, lo, hi, shape):
        return jax.random.randint(self._next(), shape, lo, hi, dtype=jnp.int32)
    def uniform(self, shape, lo=0.0, hi=1.0):
        return jax.random.uniform(self._next(), shape, jnp.bfloat16, lo, hi)
    def permutation(self, n):
        return jax.random.permutation(self._next(), n)


kernel_name = 'standalone__dcn_v2_cross__recsys'

def setup_inputs():
    _rng = _Rng(jax.random.key(int.from_bytes(__import__("os").urandom(4), "little")))
    _w = (lambda a: (lambda t: t.astype(jnp.bfloat16) if jnp.issubdtype(t.dtype, jnp.floating) else t)(jnp.asarray(a)))
    B, F, D, L = 16384, 26, 128, 6
    Din = min(F * D, 1024)
    return {
        "x0": _w((lambda *s: _rng.normal(s) * 0.05)(B, Din)),
        "ws": _w((lambda *s: _rng.normal(s) * 0.05)(L, Din, Din)),
        "bs": _w((lambda *s: _rng.normal(s) * 0.05)(L, Din)),
    }

def reference(x0, ws, bs):
    x = x0
    for l in range(ws.shape[0]):
        x = x0 * (x @ ws[l] + bs[l]) + x
    return x
```

```python
import functools

import jax
import jax.numpy as jnp
import jax.experimental.pallas as pl
import jax.experimental.pallas.tpu as pltpu


def _kernel(x0_ref, w_ref, b_ref, o_ref, *, num_layers):
    x0 = x0_ref[...].astype(jnp.float32)
    x = x0
    for l in range(num_layers):
        y = jnp.dot(x.astype(jnp.bfloat16), w_ref[l], preferred_element_type=jnp.float32)
        x = x0 * (y + b_ref[l:l + 1, :].astype(jnp.float32)) + x
    o_ref[...] = x.astype(o_ref.dtype)


@jax.jit
def pallas_standalone__dcn_v2_cross__recsys_kernel(
    x0: jax.Array,
    ws: jax.Array,
    bs: jax.Array,
):
    B, D = x0.shape
    L = ws.shape[0]
    tm = 512
    return pl.pallas_call(
        functools.partial(_kernel, num_layers=L),
        grid=(B // tm,),
        in_specs=[
            pl.BlockSpec((tm, D), lambda i: (i, 0)),
            pl.BlockSpec((L, D, D), lambda i: (0, 0, 0)),
            pl.BlockSpec((L, D), lambda i: (0, 0)),
        ],
        out_specs=pl.BlockSpec((tm, D), lambda i: (i, 0)),
        out_shape=jax.ShapeDtypeStruct((B, D), x0.dtype),
        compiler_params=pltpu.CompilerParams(
            dimension_semantics=("arbitrary",),
            vmem_limit_bytes=100 * 1024 * 1024,
        ),
    )(x0, ws, bs)
```

```python
import functools
import math

import jax
import jax.numpy as jnp
import jax.experimental.pallas as pl
import jax.experimental.pallas.tpu as pltpu

f32 = jnp.float32
bf16 = jnp.bfloat16

Q = 128
R = 32
SR = 8
NS = R // SR
TM = 8 * R
CR = 16
S3 = math.sqrt(3.0)
IN = [(p, q) for p in range(4) for q in range(4)]

CORE3 = {1: [(1, 0)], 3: [(1, 1)], 5: [(1, 2)], 2: [(1, 3)],
         4: [(1, 0), (-1, 1)], 7: [(1, 2), (-1, 0)], 6: [(1, 3), (-1, 0)]}
CORE4 = {1: [(1, 0)], 3: [(1, 1)], 5: [(1, 2)], 2: [(1, 3), (1, 0)],
         4: [(1, 0), (-1, 1)], 7: [(1, 2), (-1, 0)], 6: [(1, 3), (-1, 0)]}
SIGMA = {1: 1, 2: 3, 3: 7, 4: 6, 5: 4, 6: 5, 7: 2}
ORDER1 = [3, 5, 1, 4, 7, 6, 2]
QORD = [2, 1, 0, 3]
TORD = [1, 0, 3, 2]
AFTER = {2: [], 1: [(3, 1, 1, 2)], 0: [(1, 0, -1, 1), (2, 0, 1, 1)], 3: [(0, 3, 1, 0)]}

OPT = dict(skip=13, nblk=1, row=3, margin=22, rates=[8, 8, 13, 6, 6, 6, 6], brates=[1] * 7,
           pre=2, ic=24.0, nobc=True)


def lin(terms):
    pos = [v for s, v in terms if s > 0]
    neg = [v for s, v in terms if s < 0]
    acc = pos[0]
    for v in pos[1:]:
        acc = acc + v
    for v in neg:
        acc = acc - v
    return acc


def chain(terms):
    acc = terms[0][1]
    for s, v in terms[1:]:
        acc = acc + v if s > 0 else acc - v
    return acc


def phi3(a):
    l5 = a[0] + a[1]
    return [a[0] + a[3], a[0] - a[1], l5, 0.5 * (l5 + a[3] + a[2])]


def phi4(a):
    return [a[0] + a[3], a[0] - a[1], a[0] + a[1], a[1] + a[2]]


def phi4_inv(e, hf=0.5):
    a11 = hf * (e[1] + e[2])
    a12 = e[2] - a11
    return [a11, a12, e[3] - a12, e[0] - a11]


def psi6(c, hf):
    h = hf * c[3]
    c11 = h + c[0]
    return [c11, h, (h + c[1]) + c[2], (c11 + c[1]) - c[2]]


def rc(o, p, q):
    return (o // 2) * 4 + (p // 2) * 2 + q // 2, (o % 2) * 4 + (p % 2) * 2 + q % 2


def popc(v):
    return bin(v).count("1")


def scale(br, bc):
    return S3 ** (popc(br) - popc(bc))


def plan(skip):
    groups, n = {}, 0
    for i in range(1, 8):
        for j in range(1, 8):
            plain = ((skip == 13 and (i == 1 or j == 1)) or (skip == 7 and i == 1)
                     or (skip == 1 and i == 1 and j == 1))
            groups[(i, j)] = (n, plain)
            n += 4 if plain else 7
    return groups, n


def comb2(u, sg, v, x=None, e=None):
    if x is not None:
        u = u + x
    if e is not None:
        v = v + e if sg > 0 else v - e
    return u + v if sg > 0 else u - v


class RefArr:
    def __init__(self, ref, idx):
        self.ref, self.idx = ref, idx

    def __getitem__(self, k):
        return self.ref[self.idx, k[0] * R:(k[0] + 1) * R, k[1] * Q:(k[1] + 1) * Q]

    def get(self, s, k):
        r = k[0] * R + s * SR
        return self.ref[self.idx, r:r + SR, k[1] * Q:(k[1] + 1) * Q]

    def put(self, s, k, v):
        r = k[0] * R + s * SR
        self.ref[self.idx, r:r + SR, k[1] * Q:(k[1] + 1) * Q] = v

    def putb(self, k, v):
        self.ref[self.idx, k[0] * R:(k[0] + 1) * R, k[1] * Q:(k[1] + 1) * Q] = v


class ValArr:
    def __init__(self, blocks=None):
        self.parts = [dict() for _ in range(NS)]
        self.blocks = dict(blocks or {})

    def __getitem__(self, k):
        if k not in self.blocks:
            self.blocks[k] = jnp.concatenate([p[k] for p in self.parts], axis=0)
        return self.blocks[k]

    def get(self, s, k):
        if k not in self.parts[s]:
            self.parts[s][k] = self.blocks[k][s * SR:(s + 1) * SR]
        return self.parts[s][k]

    def put(self, s, k, v):
        self.parts[s][k] = v

    def putb(self, k, v):
        self.blocks[k] = v


class Sched:
    def __init__(self, never, opt):
        self.never, self.opt = never, opt
        self.q, self.bg, self.lock = [], [], None
        self.g, self.t, self.pace, self.bcredit, self.forced = None, 0, 0.0, 0.0, []

    def gv(self, v):
        return v if self.g is None else jnp.where(self.never, self.g, v)

    def gc(self, c):
        return c if self.g is None else jnp.where(self.never, self.g, jnp.full((SR, Q), c, f32))

    def add(self, gen, deadline, cost, bg=False):
        (self.bg if bg else self.q).append([gen, deadline, cost])
        return gen

    def step(self, q):
        while q:
            try:
                c = next(q[0][0])
            except StopIteration:
                q.pop(0)
                continue
            self.lock = None if isinstance(c, float) else q
            q[0][2] -= c
            return c
        return None

    def tick(self, val, base, brate):
        rate, cum = base, 0.0
        for _, dl, cost in self.q:
            cum += max(cost, 0)
            rate = max(rate, cum / max(dl - self.opt["margin"] - self.t, 1))
        self.bcredit = min(self.bcredit + brate + (0.0 if self.q else base), 40.0)
        self.pace = min(self.pace + rate + (brate if self.bg else 0.0), 40.0)
        if self.pace > 0:
            if self.lock:
                q = self.lock
            elif self.bg and (not self.q or (self.bcredit > 0 and rate <= base)):
                q = self.bg
            else:
                q = self.q
            if q:
                r = self.opt["row"]
                self.g = val[r * SR:(r + 1) * SR]
                c = self.step(q)
                self.g = None
                if c:
                    self.pace -= c
                    if q is self.bg:
                        self.bcredit -= c
        self.t += 1

    def drain(self, gen=None, bg=False):
        n, q = 0, (self.bg if bg else self.q)
        while q and (gen is None or any(e[0] is gen for e in q)):
            if self.step(q) is not None:
                n += 1
        self.forced.append(n)


def load_z(ref, o):
    zz = {}
    for k in IN:
        br, bc = rc(o, *k)
        zz[k] = ref[br * R:(br + 1) * R, bc * Q:(bc + 1) * Q].astype(f32)
    return ValArr(zz)


def head_q(S, o, z, emit):
    for s in range(NS):
        d = {}
        for q in QORD:
            v = []
            for p in range(4):
                sc = scale(*rc(o, p, q))
                v.append(z.get(s, (p, q)) * sc if sc != 1.0 else z.get(s, (p, q)))
            r = phi3([S.gv(v[0])] + v[1:])
            for p in range(4):
                d[(p, q)] = r[p]
                for (b, i, sg, j) in AFTER[q]:
                    emit(s, (p, b), d[(p, i)], sg, d[(p, j)])
            yield 22.0 if q == QORD[-1] else 22


def head(S, z, H, dl):
    d1, d0 = ValArr(), ValArr()

    def e1(s, k, u, sg, v):
        d1.put(s, k, comb2(u, sg, v))

    def e0(s, k, u, sg, v):
        r = comb2(u, sg, v)
        d0.put(s, k, r)
        H[1].put(s, k, r - d1.get(s, k))
        H[2].put(s, k, r + d1.get(s, k))

    def e2(s, k, u, sg, v):
        H[3].put(s, k, comb2(u, sg, v, d1.get(s, k)))

    def e3(s, k, u, sg, v):
        H[0].put(s, k, comb2(u, sg, v, d0.get(s, k)))

    gs = [head_q(S, o, z[o], e) for o, e in ((1, e1), (2, e2), (0, e0), (3, e3))]

    def allq():
        for _ in range(NS):
            for g in gs:
                for _ in range(4):
                    yield next(g)

    return S.add(allq(), dl, 16 * NS * 22)


def costs(o, n, last):
    if last:
        return 1, {1: 44, 0: 34, 3: 46, 2: 42}
    cu = {1: 4, 0: 4, 3: 12, 2: 12}[o]
    pre = {2: 4 * n, 1: 0, 0: 4 * (n - 1), 3: 4}
    return 4 * n, {q: 21 + pre[q] + cu * len(AFTER[q]) for q in QORD}


def epi(S, o, terms, z, bt_ref, l, emit=None, xo=None, out=None):
    ca, cb = costs(o, len(terms), emit is None)
    qord = TORD if emit is None else QORD
    for s in range(NS):
        cmb = lambda k: chain([(sg, m.get(s, k)) for sg, m in terms])
        yield ca
        yield ca
        c, d = {}, {}
        for p in range(4):
            c6, c2 = cmb((p, 1)), cmb((p, 2))
            c[(p, 1)] = cmb((p, 3))
            c[(p, 2)] = (c6 + c2) + c[(p, 1)]
            c[(p, 0)] = cmb((p, 0))
            c[(p, 3)] = (c6 - c2) + c[(p, 0)]
        if emit is None:
            xi = {p: phi4_inv([xo.get(s, (p, q)) for q in range(4)]) for p in range(4)}
        for q in qord:
            hf = S.gc(0.5)
            y = psi6([c[(p, q)] for p in range(4)], hf)
            dd = []
            for p in range(4):
                br, bc = rc(o, p, q)
                dd.append((y[p] + bt_ref[l * 4 + popc(br), :, bc * Q:(bc + 1) * Q]) * z.get(s, (p, q)))
            if emit is None:
                e = [xi[p][q] for p in range(4)]
                a11 = hf * (e[1] + e[2])
                a22 = e[0] - a11
                xn = [a11, e[2] - a11, ((e[3] - a22) + e[3]) - e[2], a22]
                for p in range(4):
                    br, bc = rc(o, p, q)
                    r = dd[p] + xn[p]
                    if scale(br, bc) != 1.0:
                        r = r * (1.0 / scale(br, bc))
                    d[(p, q)] = r
                    if (p, q ^ 1) in d:
                        b0, r0 = bc & ~1, br * R + s * SR
                        pair = jnp.concatenate([d[(p, q & ~1)], d[(p, q | 1)]], axis=1)
                        out[r0:r0 + SR, b0 * Q:(b0 + 2) * Q] = pair.astype(bf16)
            else:
                r = phi3(dd)
                for p in range(4):
                    d[(p, q)] = r[p]
                    for (b, i, sg, j) in AFTER[q]:
                        emit(s, (p, b), d[(p, i)], sg, d[(p, j)])
            yield float(cb[q]) if q == qord[-1] else cb[q]


def add_epi(S, dl, o, terms, *a, **kw):
    last = kw.get("emit") is None
    ca, cb = costs(o, len(terms), last)
    return S.add(epi(S, o, terms, *a, **kw), dl, NS * (2 * ca + sum(cb.values())), bg=last)


def tail(S, z, bt_ref, out, TS, L):
    for o in range(4):
        g = add_epi(S, 0, o, [(1, TS[o])], z[o], bt_ref, L - 1, xo=TS[4 + o], out=out)
    return g


def inv1(S, X, TS):
    for s in range(NS):
        for p in range(4):
            for q0 in (0, 2):
                hf = S.gc(0.5)
                for q in (q0, q0 + 1):
                    r = phi4_inv([X[b].get(s, (p, q)) for b in range(4)], hf)
                    for o in range(4):
                        TS[4 + o].put(s, (p, q), r[o])
                yield S.opt["ic"]


def inner(mul):
    m3 = mul(3)
    m5 = mul(5)
    yield 3, m5 + m3
    c = m3 - m5
    m4 = mul(4)
    c = m4 + c
    m7 = mul(7)
    c = m7 + c
    yield 0, mul(1) + c
    m2 = mul(2)
    yield 2, m2 + m4
    m6 = mul(6)
    yield 1, m6 - m7


def middle(gen):
    c0 = dict(gen(1))
    m4 = {}
    for q, c in gen(4):
        m4[q] = c
        c0[q] = c0[q] + c
    for q, c in gen(2):
        yield 2, q, c + m4[q]
    m7 = {}
    for q, c in gen(7):
        m7[q] = c
        c0[q] = c0[q] + c
    for q, c in gen(6):
        yield 1, q, c - m7[q]
    m5 = {}
    for q, c in gen(5):
        m5[q] = c
        yield 0, q, c0[q] - c
    for q, c in gen(3):
        yield 3, q, c + m5[q]


def body(xs, outs, bt_ref, t_ref, hs_ref, ts_ref, L, groups, never, opt):
    S = Sched(never, opt)
    cum = [0]
    for i in ORDER1:
        cum.append(cum[-1] + sum(8 if groups[(i, j)][1] else 7 for j in range(1, 8)))
    TL, mg = cum[-1], opt["margin"]
    nblk = len(outs)
    zs = [[load_z(x, o) for o in range(4)] for x in xs]
    X = [RefArr(hs_ref, b) for b in range(4)]
    TS = [RefArr(ts_ref, n) for n in range(8)]
    pre = [6 * opt["pre"]]

    def tile(l, n):
        return pltpu.bitcast(t_ref[l, n // 2, :, (n % 2) * Q:(n % 2 + 1) * Q], bf16)

    for sb in range(nblk):
        z = zs[sb + 1]
        need = None
        tl = tail(S, zs[sb], bt_ref, outs[sb], TS, L)
        final = sb == nblk - 1
        for l in range(L):
            T0 = (sb * L + l) * TL
            last = l == L - 1

            def prod1(i):
                base, brate = opt["rates"][ORDER1.index(i)], opt["brates"][ORDER1.index(i)]

                def gen2(j):
                    a = [lin([(s1 * s2, X[b1][(b2, q)]) for s1, b1 in CORE4[i] for s2, b2 in CORE3[j]])
                         for q in range(4)]
                    n, plain = groups[(i, j)]
                    if plain:
                        an = phi4_inv(a)
                        k0 = jnp.concatenate([an[0], an[2]], axis=0).astype(bf16)
                        k1 = jnp.concatenate([an[1], an[3]], axis=0).astype(bf16)

                        def dot2(u, k):
                            r = jnp.dot(u, tile(l, n + k), preferred_element_type=f32)
                            S.tick(r[:R], base, brate)
                            S.tick(r[R:], base, brate)
                            return r

                        c0 = dot2(k0, 0) + dot2(k1, 2)
                        c1 = dot2(k0, 1) + dot2(k1, 3)
                        n11, n12, n21, n22 = c0[:R], c1[:R], c0[R:], c1[R:]
                        df = n22 - n11
                        c6 = 0.5 * ((n21 - n12) + df)
                        yield 0, n11
                        yield 3, n12
                        yield 1, c6
                        yield 2, c6 - df
                    else:
                        def mul(k):
                            u = lin([(s3, a[b]) for s3, b in CORE4[k]])
                            if len(CORE4[k]) == 2:
                                for r_ in range(2):
                                    if pre[0] > 0:
                                        S.g = u[r_ * 16:r_ * 16 + SR]
                                        S.step(S.bg)
                                        S.g = None
                                        pre[0] -= 1
                            r = jnp.dot(u.astype(bf16), tile(l, n + k - 1), preferred_element_type=f32)
                            S.tick(r, base, brate)
                            return r

                        yield from inner(mul)

                return {(p, q): c for p, q, c in middle(gen2)}

            XN = [ValArr() for _ in range(4)]
            d12, d11 = ValArr(), ValArr()

            def emitter(o, X=X, XN=XN, d12=d12, d11=d11):
                def emit(s, k, u, sg, v):
                    if o == 1:
                        d12.put(s, k, comb2(u, sg, v))
                    elif o == 0:
                        e, r = d12.get(s, k), comb2(u, sg, v)
                        d11.put(s, k, r)
                        XN[1].put(s, k, (r + X[1].get(s, k)) - e)
                        XN[2].put(s, k, (r + X[2].get(s, k)) + e)
                    elif o == 3:
                        XN[0].put(s, k, comb2(u, sg, v, X[0].get(s, k), d11.get(s, k)))
                    else:
                        XN[3].put(s, k, comb2(u, sg, v, X[3].get(s, k), d12.get(s, k)))
                return emit

            nn = {}
            if last:
                S.drain(tl, bg=True)
                TS = [RefArr(ts_ref, n) if final else ValArr() for n in range(8)]
                XN = [RefArr(hs_ref, b) if final else ValArr() for b in range(4)]

            def add(o, terms, dl):
                if last:
                    for k in IN:
                        TS[o].putb(k, chain([(sg, m[k]) for sg, m in terms]))
                else:
                    nn[o] = add_epi(S, dl, o, [(sg, ValArr(m)) for sg, m in terms], z[o], bt_ref, l,
                                    emit=emitter(o))

            if need:
                S.drain(need[0])
            m3 = prod1(3)
            m5 = prod1(5)
            if last:
                dl = T0 + TL + (mg if final else 0)
                S.add(inv1(S, X, TS), dl, NS * 8 * opt["ic"])
                head(S, zs[sb + 2], XN, dl)
            h = {k: m5[k] + m3[k] for k in IN}
            w = {k: m3[k] - m5[k] for k in IN}
            add(1, [(1, h)], T0 + cum[5] + mg)
            if need:
                S.drain(need[3])
            m1 = prod1(1)
            w = {k: m1[k] + w[k] for k in IN}
            m4 = prod1(4)
            m7 = prod1(7)
            add(0, [(1, m7), (1, w), (1, m4)], T0 + TL)
            if need:
                S.drain(need[2])
            m6 = prod1(6)
            m2 = prod1(2)
            add(3, [(1, w), (-1, m2), (1, m6)], T0 + TL + cum[2])
            add(2, [(1, m2), (1, m6), (1, h), (1, m4), (-1, m7)], T0 + TL + cum[5])
            need = nn
            X = XN
        S.drain()
    if opt.get("verbose"):
        print("forced", S.forced)


def tcore(e, k):
    if k == 1:
        return e[0] + e[0]
    return lin([(s, e[b]) for s, b in CORE4[SIGMA[k]]])


def build_chunk(w_ref, tb_ref, l, r, groups):
    d = []
    for o in range(4):
        v, t, u = {}, {}, {}
        for k in IN:
            br, bc = rc(o, *k)
            v[k] = w_ref[br, :, bc * Q:(bc + 1) * Q].astype(f32) * (0.25 * scale(br, bc))
        for q in range(4):
            for p, x in enumerate(phi3([v[(p, q)] for p in range(4)])):
                t[(p, q)] = x
        for p in range(4):
            for q, x in enumerate(phi4([t[(p, q)] for q in range(4)])):
                u[(p, q)] = x
        d.append(u)
    E = {k: phi4([d[o][k] for o in range(4)]) for k in IN}
    for i in range(1, 8):
        s1 = {k: tcore(E[k], i) for k in IN}
        for j in range(1, 8):
            e = [lin([(sg, s1[(b, q)]) for sg, b in CORE3[SIGMA[j]]]) for q in range(4)]
            n, plain = groups[(i, j)]
            if plain:
                a, b = e[1] + e[2], e[2] - e[1]
                outs = [a, b, (e[3] - b) + e[3], (e[0] - a) + e[0]]
            else:
                outs = [tcore(e, k) for k in range(1, 8)]
            for k, t in enumerate(outs):
                c0 = ((n + k) % 2) * Q
                tb_ref.at[l, (n + k) // 2][pl.ds(r, CR), c0:c0 + Q] = t.astype(bf16)


NW = 8


def kernel(x_hbm, w_hbm, b_ref, o_hbm, t_ref, bt_ref, hs_ref, ts_ref, w_buf, x_buf, o_buf,
           w_sem, x_sem, o_sem, *, L, nb, groups, opt):
    nblk = opt["nblk"]
    NX, NO = x_buf.shape[0], o_buf.shape[0]
    nch = Q // CR

    def wcopy(c):
        return pltpu.make_async_copy(
            w_hbm.at[c // nch, :, pl.ds(pl.multiple_of((c % nch) * CR, CR), CR), :],
            w_buf.at[c % NW], w_sem.at[c % NW])

    def xcopy(i):
        return pltpu.make_async_copy(x_hbm.at[pl.ds(pl.multiple_of(i * TM, TM), TM), :],
                                     x_buf.at[i % NX], x_sem.at[i % NX])

    def ocopy(i):
        return pltpu.make_async_copy(o_buf.at[i % NO], o_hbm.at[pl.ds(pl.multiple_of(i * TM, TM), TM), :],
                                     o_sem.at[i % NO])

    for c in range(NW - 1):
        wcopy(c).start()
    for i in range(nblk + 1):
        xcopy(i).start()
    for l in range(L):
        for e in range(4):
            for bc in range(8):
                row = b_ref[l:l + 1, bc * Q:(bc + 1) * Q].astype(f32) * (S3 ** (e - popc(bc)))
                bt_ref[l * 4 + e, :, bc * Q:(bc + 1) * Q] = jnp.broadcast_to(row, (SR, Q))
    ts_ref[...] = jnp.zeros(ts_ref.shape, f32)
    tb_ref = t_ref.bitcast(bf16)

    def build(c, carry):
        wcopy(c).wait()

        @pl.when(c + NW - 1 < L * nch)
        def _():
            wcopy(c + NW - 1).start()

        build_chunk(w_buf.at[c % NW], tb_ref, c // nch, pl.multiple_of((c % nch) * CR, CR), groups)
        return carry

    jax.lax.fori_loop(0, L * nch, build, 0)

    xcopy(0).wait()
    S = Sched(None, opt)
    head(S, [load_z(x_buf.at[0], o) for o in range(4)], [RefArr(hs_ref, b) for b in range(4)], 0)
    S.drain()

    def step(it, carry):
        i0 = it * nblk
        for u in range(nblk):
            @pl.when(i0 + u + 1 < nb)
            def _():
                xcopy(i0 + u + 1).wait()

            @pl.when(i0 + u + nblk + 1 < nb)
            def _():
                xcopy(i0 + u + nblk + 1).start()

            @pl.when(i0 + u - 1 - nblk >= 0)
            def _():
                ocopy(i0 + u - 1 - nblk).start()

            @pl.when(i0 + u - 1 - NO >= 0)
            def _():
                ocopy(i0 + u - 1 - NO).wait()

        never = jnp.full((SR, Q), it, jnp.int32) < 0
        xs = [x_buf.at[jnp.clip(i0 + u, 0, nb - 1) % NX] for u in range(-1, nblk + 1)]
        outs = [o_buf.at[(i0 + u + NO) % NO] for u in range(-1, nblk - 1)]
        body(xs, outs, bt_ref, t_ref, hs_ref, ts_ref, L, groups, never, opt)
        return carry

    jax.lax.fori_loop(0, nb // nblk, step, 0)

    for i in range(nb - 1 - nblk, nb - 1):
        if i >= 0:
            ocopy(i).start()
    if nb - 1 - NO >= 0:
        ocopy(nb - 1 - NO).wait()
    S = Sched(None, opt)
    tail(S, [load_z(x_buf.at[(nb - 1) % NX], o) for o in range(4)], bt_ref, o_buf.at[(nb - 1) % NO],
         [RefArr(ts_ref, n) for n in range(8)], L)
    S.drain(bg=True)
    ocopy(nb - 1).start()
    for i in range(max(nb - NO, 0), nb):
        ocopy(i).wait()


def make(o=None):
    opt = dict(OPT)
    opt.update(o or {})
    groups, n = plan(opt["skip"])

    @jax.jit
    def run(x0, ws, bs):
        B, D = x0.shape
        L = ws.shape[0]
        nb, nblk = B // TM, opt["nblk"]
        NX, NO = 2 * nblk + 2, 2 * nblk
        return pl.pallas_call(
            functools.partial(kernel, L=L, nb=nb, groups=groups, opt=opt),
            in_specs=[pl.BlockSpec(memory_space=pl.ANY),
                      pl.BlockSpec(memory_space=pl.ANY),
                      pl.BlockSpec(memory_space=pltpu.VMEM)],
            out_specs=pl.BlockSpec(memory_space=pl.ANY),
            out_shape=jax.ShapeDtypeStruct((B, D), x0.dtype),
            scratch_shapes=[
                pltpu.VMEM((L, (n + 1) // 2, Q // 2, 2 * Q), jnp.uint32),
                pltpu.VMEM((L * 4, SR, D), f32),
                pltpu.VMEM((4, 4 * R, D // 2), f32),
                pltpu.VMEM((8, 4 * R, D // 2), f32),
                pltpu.VMEM((NW, 8, CR, D), bf16),
                pltpu.VMEM((NX, TM, D), bf16),
                pltpu.VMEM((NO, TM, D), bf16),
                pltpu.SemaphoreType.DMA((NW,)),
                pltpu.SemaphoreType.DMA((NX,)),
                pltpu.SemaphoreType.DMA((NO,)),
            ],
            compiler_params=pltpu.CompilerParams(vmem_limit_bytes=120 * 1024 * 1024,
                                                 disable_bounds_checks=opt["nobc"]),
        )(x0, ws.reshape(L, 8, Q, D), bs)

    return run


_run = make()


@jax.jit
def pallas_standalone__dcn_v2_cross__recsys_kernel(x0: jax.Array, ws: jax.Array, bs: jax.Array):
    return _run(x0, ws, bs)
```

```python
import functools
import math

import jax
import jax.numpy as jnp
import jax.experimental.pallas as pl
import jax.experimental.pallas.tpu as pltpu

f32 = jnp.float32
bf16 = jnp.bfloat16

Q = 128
R = 32
SR = 8
NS = R // SR
TM = 8 * R
CR = 16
S3 = math.sqrt(3.0)
IN = [(p, q) for p in range(4) for q in range(4)]

CORE3 = {1: [(1, 0)], 3: [(1, 1)], 5: [(1, 2)], 2: [(1, 3)],
         4: [(1, 0), (-1, 1)], 7: [(1, 2), (-1, 0)], 6: [(1, 3), (-1, 0)]}
CORE4 = {1: [(1, 0)], 3: [(1, 1)], 5: [(1, 2)], 2: [(1, 3), (1, 0)],
         4: [(1, 0), (-1, 1)], 7: [(1, 2), (-1, 0)], 6: [(1, 3), (-1, 0)]}
SIGMA = {1: 1, 2: 3, 3: 7, 4: 6, 5: 4, 6: 5, 7: 2}
ORDER1 = [3, 5, 1, 4, 7, 6, 2]
QORD = [2, 1, 0, 3]
TORD = [1, 0, 3, 2]
AFTER = {2: [], 1: [(3, 1, 1, 2)], 0: [(1, 0, -1, 1), (2, 0, 1, 1)], 3: [(0, 3, 1, 0)]}

OPT = dict(skip=13, nblk=1, row=2, margin=27, rates=[9.2, 7, 11.5, 5.5, 5.5, 5.5, 5.4], brates=[2.0] * 7,
           rates0=[9.2, 9.4, 10, 6, 6, 5.5, 5.4], rates5=[9.2, 7, 12.4, 5.5, 5.5, 5.5, 5.4],
           brates0=[2.0, 2.3, 1.0, 2.0, 3.0, 2.0, 3.0],
           pre=2, ic=18.0, endm=25, tsplit=1, split=0, a3='alt', c3='d', od=[3, 4, 5, 1, 7, 6, 2],
           mj=[1.0] * 7, cap=40.0, o2=[1, 4, 2, 7, 6, 5, 3], o3=[3, 5, 4, 7, 1, 2, 6], raw2=0, raw3=0,
           o1=[3, 5, 1, 4, 7, 6, 2], wh=1, nobc=True)


def lin(terms):
    pos = [v for s, v in terms if s > 0]
    neg = [v for s, v in terms if s < 0]
    acc = pos[0]
    for v in pos[1:]:
        acc = acc + v
    for v in neg:
        acc = acc - v
    return acc


def chain(terms):
    acc = terms[0][1]
    for s, v in terms[1:]:
        acc = acc + v if s > 0 else acc - v
    return acc


def phi3(a):
    l5 = a[0] + a[1]
    return [a[0] + a[3], a[0] - a[1], l5, 0.5 * (l5 + a[3] + a[2])]


def phi4(a):
    return [a[0] + a[3], a[0] - a[1], a[0] + a[1], a[1] + a[2]]


def phi4_inv(e, hf=0.5):
    a11 = hf * (e[1] + e[2])
    a12 = e[2] - a11
    return [a11, a12, e[3] - a12, e[0] - a11]


def psi6(c, hf):
    h = hf * c[3]
    c11 = h + c[0]
    return [c11, h, (h + c[1]) + c[2], (c11 + c[1]) - c[2]]


def rc(o, p, q):
    return (o // 2) * 4 + (p // 2) * 2 + q // 2, (o % 2) * 4 + (p % 2) * 2 + q % 2


def popc(v):
    return bin(v).count("1")


def scale(br, bc):
    return S3 ** (popc(br) - popc(bc))


def plan(skip):
    groups, n = {}, 0
    for i in range(1, 8):
        for j in range(1, 8):
            plain = ((skip == 13 and (i == 1 or j == 1)) or (skip == 7 and i == 1)
                     or (skip == 1 and i == 1 and j == 1))
            groups[(i, j)] = (n, plain)
            n += 4 if plain else 7
    return groups, n


def comb2(u, sg, v, x=None, e=None):
    if x is not None:
        u = u + x
    if e is not None:
        v = v + e if sg > 0 else v - e
    return u + v if sg > 0 else u - v


class RefArr:
    def __init__(self, ref, idx):
        self.ref, self.idx = ref, idx

    def __getitem__(self, k):
        return self.ref[self.idx, k[0] * R:(k[0] + 1) * R, k[1] * Q:(k[1] + 1) * Q]

    def get(self, s, k):
        r = k[0] * R + s * SR
        return self.ref[self.idx, r:r + SR, k[1] * Q:(k[1] + 1) * Q]

    def put(self, s, k, v):
        r = k[0] * R + s * SR
        self.ref[self.idx, r:r + SR, k[1] * Q:(k[1] + 1) * Q] = v

    def putb(self, k, v):
        self.ref[self.idx, k[0] * R:(k[0] + 1) * R, k[1] * Q:(k[1] + 1) * Q] = v


class ValArr:
    def __init__(self, blocks=None):
        self.parts = [dict() for _ in range(NS)]
        self.blocks = dict(blocks or {})

    def __getitem__(self, k):
        if k not in self.blocks:
            self.blocks[k] = jnp.concatenate([p[k] for p in self.parts], axis=0)
        return self.blocks[k]

    def get(self, s, k):
        if k not in self.parts[s]:
            self.parts[s][k] = self.blocks[k][s * SR:(s + 1) * SR]
        return self.parts[s][k]

    def put(self, s, k, v):
        self.parts[s][k] = v

    def putb(self, k, v):
        self.blocks[k] = v


class Sched:
    def __init__(self, never, opt):
        self.never, self.opt = never, opt
        self.q, self.bg, self.lock = [], [], None
        self.g, self.t, self.pace, self.bcredit, self.forced = None, 0, 0.0, 0.0, []

    def gv(self, v):
        return v if self.g is None else jnp.where(self.never, self.g, v)

    def gc(self, c):
        return c if self.g is None else jnp.where(self.never, self.g, jnp.full((SR, Q), c, f32))

    def add(self, gen, deadline, cost, bg=False):
        (self.bg if bg else self.q).append([gen, deadline, cost])
        return gen

    def step(self, q):
        while q:
            try:
                c = next(q[0][0])
            except StopIteration:
                q.pop(0)
                continue
            self.lock = None if isinstance(c, float) else q
            q[0][2] -= c
            return c
        return None

    def tick(self, val, base, brate, mult=1.0):
        rate, cum = base, 0.0
        for _, dl, cost in self.q:
            cum += max(cost, 0)
            rate = max(rate, cum / max(dl - self.opt["margin"] - self.t, 1))
        self.bcredit = min(self.bcredit + brate + (0.0 if self.q else base), 40.0)
        self.pace = min(self.pace + mult * (rate + (brate if self.bg else 0.0)), self.opt['cap'])
        if self.pace > 0:
            if self.lock:
                q = self.lock
            elif self.bg and (not self.q or (self.bcredit > 0 and rate <= base)):
                q = self.bg
            else:
                q = self.q
            if q:
                r = self.opt["row"]
                self.g = val[r * SR:(r + 1) * SR]
                c = self.step(q)
                self.g = None
                if c:
                    self.pace -= c
                    if q is self.bg:
                        self.bcredit -= c
        self.t += 1

    def drain(self, gen=None, bg=False):
        n, q = 0, (self.bg if bg else self.q)
        while q and (gen is None or any(e[0] is gen for e in q)):
            if self.step(q) is not None:
                n += 1
        self.forced.append(n)


def load_z(ref, o):
    zz = {}
    for k in IN:
        br, bc = rc(o, *k)
        zz[k] = ref[br * R:(br + 1) * R, bc * Q:(bc + 1) * Q].astype(f32)
    return ValArr(zz)


def finish(S, dd, q, d, s, emit):
    if S.opt["a3"] == "alt":
        r = phi3(dd)
        for p in range(4):
            d[(p, q)] = r[p]
            for (b, i, sg, j) in AFTER[q]:
                emit(s, (p, b), d[(p, i)], sg, d[(p, j)])
    else:
        emit(s, (0, q), dd[0], 1, dd[3])
        emit(s, (1, q), dd[0], -1, dd[1])
        emit(s, (2, q), dd[0], 1, dd[1])
        emit(s, (3, q), 0.5 * ((dd[0] + dd[1]) + dd[3]), 1, 0.5 * dd[2])


def head_q(S, o, z, emit):
    for s in range(NS):
        d = {}
        for q in QORD:
            v = []
            for p in range(4):
                sc = scale(*rc(o, p, q))
                v.append(z.get(s, (p, q)) * sc if sc != 1.0 else z.get(s, (p, q)))
            finish(S, [S.gv(v[0])] + v[1:], q, d, s, emit)
            yield 22.0 if q == QORD[-1] else 22


def head(S, z, H, dl):
    d1, d0 = ValArr(), ValArr()

    def e1(s, k, u, sg, v):
        d1.put(s, k, comb2(u, sg, v))

    def e0(s, k, u, sg, v):
        r = comb2(u, sg, v)
        d0.put(s, k, r)
        H[1].put(s, k, r - d1.get(s, k))
        H[2].put(s, k, r + d1.get(s, k))

    def e2(s, k, u, sg, v):
        H[3].put(s, k, comb2(u, sg, v, d1.get(s, k)))

    def e3(s, k, u, sg, v):
        H[0].put(s, k, comb2(u, sg, v, d0.get(s, k)))

    gs = [head_q(S, o, z[o], e) for o, e in ((1, e1), (2, e2), (0, e0), (3, e3))]

    def allq():
        for _ in range(NS):
            for g in gs:
                for _ in range(4):
                    yield next(g)

    return S.add(allq(), dl, 16 * NS * 22)


def costs(o, n, last, opt):
    e = 4 * (n - 1)
    if opt["c3"] == "alt":
        ca, pre = (1, {1: e, 0: e, 3: 12 + 2 * e, 2: 8}) if last else (4 * n, {2: 4 * n, 1: 0, 0: e, 3: 4})
    else:
        ca, pre = 1, {q: e for q in range(4)}
    if last:
        post = {1: 23, 0: 13, 3: 13, 2: 13} if opt["a3"] == "alt" else {q: 11 for q in range(4)}
    elif opt["a3"] == "alt":
        post = {q: {1: 4, 0: 4, 3: 12, 2: 12}[o] * len(AFTER[q]) for q in range(4)}
    else:
        post = {q: {1: 1, 0: 1, 3: 10, 2: 10}[o] for q in range(4)}
    return ca, {q: 21 + pre[q] + post[q] for q in range(4)}


def epi(S, o, terms, z, bt_ref, l, emit=None, xo=None, out=None):
    ca, cb = costs(o, len(terms), emit is None, S.opt)
    qord = TORD if emit is None else QORD
    for s in range(NS):
        cmb = lambda k: chain([(sg, m.get(s, k)) for sg, m in terms])
        c, d = {}, {}
        for p in range(4):
            if S.opt["c3"] == "alt":
                c6, c2 = cmb((p, 1)), cmb((p, 2))
                c[(p, 1)] = cmb((p, 3))
                c[(p, 2)] = (c6 + c2) + c[(p, 1)]
                c[(p, 0)] = cmb((p, 0))
                c[(p, 3)] = (c6 - c2) + c[(p, 0)]
            else:
                for q in range(4):
                    c[(p, q)] = cmb((p, q))
            if p % 2 == 1:
                yield ca
        if emit is None:
            xi = {p: (phi4_inv if S.opt['a3'] == 'alt' else list)([xo.get(s, (p, q)) for q in range(4)]) for p in range(4)}
        for q in qord:
            hf = S.gc(0.5)
            y = psi6([c[(p, q)] for p in range(4)], hf)
            c2nd = 0
            if S.opt["split"] and emit is not None:
                c2nd = 14 + {1: 4, 0: 4, 3: 12, 2: 12}[o] * len(AFTER[q])
                yield cb[q] - c2nd
            if S.opt["tsplit"] and emit is None:
                c2nd = cb[q] // 2
                yield cb[q] - c2nd
                hf = S.gc(0.5)
            dd = []
            for p in range(4):
                br, bc = rc(o, p, q)
                yy = S.gv(y[p]) if (p == 0 and S.opt["split"] == 2 and emit is not None) else y[p]
                dd.append((yy + bt_ref[l * 4 + popc(br), :, bc * Q:(bc + 1) * Q]) * z.get(s, (p, q)))
            if emit is None:
                e = [xi[p][q] for p in range(4)]
                a11 = hf * (e[1] + e[2])
                a22 = e[0] - a11
                xn = [a11, e[2] - a11, ((e[3] - a22) + e[3]) - e[2], a22]
                for p in range(4):
                    br, bc = rc(o, p, q)
                    r = dd[p] + xn[p]
                    if scale(br, bc) != 1.0:
                        r = r * (1.0 / scale(br, bc))
                    d[(p, q)] = r
                    if (p, q ^ 1) in d:
                        b0, r0 = bc & ~1, br * R + s * SR
                        pair = jnp.concatenate([d[(p, q & ~1)], d[(p, q | 1)]], axis=1)
                        out[r0:r0 + SR, b0 * Q:(b0 + 2) * Q] = pair.astype(bf16)
            else:
                if S.opt["split"] == 1:
                    dd[0] = S.gv(dd[0])
                finish(S, dd, q, d, s, emit)
            cc = c2nd if c2nd else cb[q]
            yield float(cc) if q == qord[-1] else cc


def add_epi(S, dl, o, terms, *a, **kw):
    last = kw.get("emit") is None
    ca, cb = costs(o, len(terms), last, S.opt)
    return S.add(epi(S, o, terms, *a, **kw), dl, NS * (2 * ca + sum(cb.values())), bg=last)


NAMES = ["h", "w", "m4", "m7", "m6", "m2"]
TERMS = {1: [(1, "h")], 0: [(1, "m7"), (1, "w"), (1, "m4")], 3: [(1, "w"), (-1, "m2"), (1, "m6")],
         2: [(1, "m2"), (1, "m6"), (1, "h"), (1, "m4"), (-1, "m7")]}


def tail(S, z, bt_ref, out, TS, L):
    for o in range(4):
        g = add_epi(S, 0, o, [(sg, TS[4 + NAMES.index(n)]) for sg, n in TERMS[o]], z[o], bt_ref, L - 1,
                    xo=TS[o], out=out)
    return g


def inv1(S, X, TS):
    for s in range(NS):
        for p in range(4):
            for q0 in (0, 2):
                hf = S.gc(0.5)
                for q in (q0, q0 + 1):
                    r = phi4_inv([X[b].get(s, (p, q)) for b in range(4)], hf)
                    for o in range(4):
                        TS[o].put(s, (p, q), r[o])
                yield S.opt["ic"]


def inner(mul):
    m3 = mul(3)
    m5 = mul(5)
    yield 3, m5 + m3
    c = m3 - m5
    m4 = mul(4)
    c = m4 + c
    m7 = mul(7)
    c = m7 + c
    yield 0, mul(1) + c
    m2 = mul(2)
    yield 2, m2 + m4
    m6 = mul(6)
    yield 1, m6 - m7


def sadd(a, b):
    if a is None:
        return b
    if a[0] == b[0]:
        return (a[0], b[1] + a[1])
    return (1, a[1] - b[1]) if a[0] > 0 else (1, b[1] - a[1])


def inner_direct(mul, od):
    need = {"w": {1: 1, 3: 1, 5: -1}, "h": {3: 1, 5: 1}, 0: {"w": 1, 4: 1, 7: 1}, 3: {"w": 1, 6: 1, 2: -1},
            2: {"h": 1, 4: 1, 7: -1, 6: 1, 2: 1}}
    acc = {n: None for n in need}
    left = {n: set(t) for n, t in need.items()}
    for k in od:
        todo = [(k, mul(k))]
        while todo:
            name, v = todo.pop(0)
            for n, t in need.items():
                if name in left[n]:
                    left[n].discard(name)
                    acc[n] = sadd(acc[n], (t[name], v))
                    if not left[n]:
                        assert acc[n][0] > 0
                        if n == "h":
                            yield 1, acc[n][1]
                        if n in ("w", "h"):
                            todo.append((n, acc[n][1]))
                        else:
                            yield n, acc[n][1]


def middle(gen):
    c0 = dict(gen(1))
    m4 = {}
    for q, c in gen(4):
        m4[q] = c
        c0[q] = c0[q] + c
    for q, c in gen(2):
        yield 2, q, c + m4[q]
    m7 = {}
    for q, c in gen(7):
        m7[q] = c
        c0[q] = c0[q] + c
    for q, c in gen(6):
        yield 1, q, c - m7[q]
    m5 = {}
    for q, c in gen(5):
        m5[q] = c
        yield 0, q, c0[q] - c
    for q, c in gen(3):
        yield 3, q, c + m5[q]


OUT2 = {0: {1: 1, 4: 1, 7: 1, 5: -1}, 1: {6: 1, 7: -1}, 2: {2: 1, 4: 1}, 3: {3: 1, 5: 1}}
OUT3 = {0: {1: 1, 4: 1, 7: 1, 5: -1, 3: 1}, 1: {6: 1, 7: -1}, 2: {2: 1, 4: 1}, 3: {3: 1, 5: 1}}


def combine(gen, order, OUT, raw):
    part = {o: [] for o in OUT}
    done = set()
    for j in order:
        done.add(j)
        new = {o: {} for o in OUT}
        for q, c in gen(j):
            for o, t in OUT.items():
                if j not in t:
                    continue
                fin = all(x in done for x in t)
                if fin or (not raw and part[o]):
                    sg, acc = t[j], c
                    for pr in reversed(part[o]):
                        s2, v = pr[q]
                        if sg == s2:
                            acc = acc + v
                        elif sg > 0:
                            acc = acc - v
                        else:
                            sg, acc = 1, v - acc
                    if fin:
                        assert sg > 0
                        yield o, q, acc
                    else:
                        new[o][q] = (sg, acc)
                else:
                    new[o][q] = (t[j], c)
        for o, t in OUT.items():
            if j in t and new[o]:
                part[o] = (part[o] + [new[o]]) if raw else [new[o]]


def body(xs, outs, bt_ref, t_ref, hs_ref, ts_ref, L, groups, never, opt):
    S = Sched(never, opt)
    cum = [0]
    for i in opt['o1']:
        cum.append(cum[-1] + sum(8 if groups[(i, j)][1] else 7 for j in range(1, 8)))
    TL, mg = cum[-1], opt["margin"]
    nblk = len(outs)
    zs = [[load_z(x, o) for o in range(4)] for x in xs]
    X = [RefArr(hs_ref, b) for b in range(4)]
    TS = [RefArr(ts_ref, n) for n in range(10)]
    pre = [(10 if opt["tsplit"] else 6) * opt["pre"]]

    def tile(l, n):
        return pltpu.bitcast(t_ref[l, n // 2, :, (n % 2) * Q:(n % 2 + 1) * Q], bf16)

    for sb in range(nblk):
        z = zs[sb + 1]
        need = None
        tl = tail(S, zs[sb], bt_ref, outs[sb], TS, L)
        final = sb == nblk - 1
        for l in range(L):
            T0 = (sb * L + l) * TL
            last = l == L - 1

            def prod1(i):
                base = opt.get("rates%d" % l, opt["rates"])[ORDER1.index(i)]
                brate = opt.get("brates%d" % l, opt["brates"])[ORDER1.index(i)]

                def gen2(j):
                    a = [lin([(s1 * s2, X[b1][(b2, q)]) for s1, b1 in CORE4[i] for s2, b2 in CORE3[j]])
                         for q in range(4)]
                    n, plain = groups[(i, j)]
                    mult = opt['mj'][opt['o2'].index(j)] * 7.0 / sum(opt['mj'])
                    if plain:
                        an = phi4_inv(a) if opt['a3'] == 'alt' else a
                        k0 = jnp.concatenate([an[0], an[2]], axis=0).astype(bf16)
                        k1 = jnp.concatenate([an[1], an[3]], axis=0).astype(bf16)

                        def dot2(u, k):
                            r = jnp.dot(u, tile(l, n + k), preferred_element_type=f32)
                            S.tick(r[:R], base, brate, mult)
                            S.tick(r[R:], base, brate, mult)
                            return r

                        c0 = dot2(k0, 0) + dot2(k1, 2)
                        c1 = dot2(k0, 1) + dot2(k1, 3)
                        n11, n12, n21, n22 = c0[:R], c1[:R], c0[R:], c1[R:]
                        if opt["c3"] == "alt":
                            df = n22 - n11
                            c6 = 0.5 * ((n21 - n12) + df)
                            yield 0, n11
                            yield 3, n12
                            yield 1, c6
                            yield 2, c6 - df
                        else:
                            yield from enumerate([n11, n12, n21, n22])
                    else:
                        def mul(k):
                            if opt["a3"] == "alt":
                                u = lin([(s3, a[b]) for s3, b in CORE4[k]])
                            else:
                                u = {1: lambda: a[0] + a[3], 3: lambda: a[0] - a[1], 5: lambda: a[0] + a[1],
                                     4: lambda: a[1] + a[3], 7: lambda: a[1] - a[3],
                                     2: lambda: (a[1] + a[2]) + (a[0] + a[3]),
                                     6: lambda: (a[1] + a[2]) - (a[0] + a[3])}[k]()
                            if len(CORE4[k]) == 2:
                                for r_ in range(2):
                                    if pre[0] > 0:
                                        S.g = u[r_ * 16:r_ * 16 + SR]
                                        S.step(S.bg)
                                        S.g = None
                                        pre[0] -= 1
                            r = jnp.dot(u.astype(bf16), tile(l, n + k - 1), preferred_element_type=f32)
                            S.tick(r, base, brate, mult)
                            return r

                        if opt["c3"] == "alt":
                            for q, _, c in combine(lambda k: [(0, mul(k))], opt['o3'], OUT3, opt['raw3']):
                                yield q, c
                        else:
                            yield from inner_direct(mul, opt["od"])

                return {(p, q): c for p, q, c in combine(gen2, opt['o2'], OUT2, opt['raw2'])}

            XN = [ValArr() for _ in range(4)]
            d12, d11 = ValArr(), ValArr()

            def emitter(o, X=X, XN=XN, d12=d12, d11=d11):
                def emit(s, k, u, sg, v):
                    if o == 1:
                        d12.put(s, k, comb2(u, sg, v))
                    elif o == 0:
                        e, r = d12.get(s, k), comb2(u, sg, v)
                        d11.put(s, k, r)
                        XN[1].put(s, k, (r + X[1].get(s, k)) - e)
                        XN[2].put(s, k, (r + X[2].get(s, k)) + e)
                    elif o == 3:
                        XN[0].put(s, k, comb2(u, sg, v, X[0].get(s, k), d11.get(s, k)))
                    else:
                        XN[3].put(s, k, comb2(u, sg, v, X[3].get(s, k), d12.get(s, k)))
                return emit

            nn = {}
            if last:
                S.drain(tl, bg=True)
                TS = [RefArr(ts_ref, n) if final else ValArr() for n in range(10)]
                XN = [RefArr(hs_ref, b) if final else ValArr() for b in range(4)]

            M = {}

            def keep(name, m):
                M[name] = ValArr(m)
                if last:
                    for k in IN:
                        TS[4 + NAMES.index(name)].putb(k, m[k])

            def add(o, dl):
                if not last:
                    nn[o] = add_epi(S, dl, o, [(sg, M[n]) for sg, n in TERMS[o]], z[o], bt_ref, l,
                                    emit=emitter(o))

            if need:
                S.drain(need[0])
            o1 = opt["o1"]
            mm = {i: prod1(i) for i in o1[:2]}
            if last:
                dl = T0 + TL + (opt["endm"] if final else 0)
                S.add(inv1(S, X, TS), dl, NS * 8 * opt["ic"])
                head(S, zs[sb + 2], XN, dl)
            keep("h", {k: mm[o1[1]][k] + mm[o1[0]][k] for k in IN})
            w = {k: mm[3][k] - mm[5][k] for k in IN}
            add(1, T0 + cum[5] + mg)
            if need:
                S.drain(need[3])
            for i in o1[2:5]:
                m = prod1(i)
                if i == 1:
                    keep("w", {k: m[k] + w[k] for k in IN})
                else:
                    keep("m%d" % i, m)
            add(0, T0 + TL)
            if need:
                S.drain(need[2])
            for i in o1[5:]:
                keep("m%d" % i, prod1(i))
            add(3, T0 + TL + cum[2])
            add(2, T0 + TL + cum[5])
            need = nn
            X = XN
        S.drain()
    if opt.get("verbose"):
        print("forced", S.forced)


def tcore(e, k):
    if k == 1:
        return e[0] + e[0]
    return lin([(s, e[b]) for s, b in CORE4[SIGMA[k]]])


def build_chunk(w_ref, tb_ref, l, r, groups):
    d = []
    for o in range(4):
        v, t, u = {}, {}, {}
        for k in IN:
            br, bc = rc(o, *k)
            v[k] = w_ref[br, :, bc * Q:(bc + 1) * Q].astype(f32) * (0.25 * scale(br, bc))
        for q in range(4):
            for p, x in enumerate(phi3([v[(p, q)] for p in range(4)])):
                t[(p, q)] = x
        for p in range(4):
            for q, x in enumerate(phi4([t[(p, q)] for q in range(4)])):
                u[(p, q)] = x
        d.append(u)
    E = {k: phi4([d[o][k] for o in range(4)]) for k in IN}
    for i in range(1, 8):
        s1 = {k: tcore(E[k], i) for k in IN}
        for j in range(1, 8):
            e = [lin([(sg, s1[(b, q)]) for sg, b in CORE3[SIGMA[j]]]) for q in range(4)]
            n, plain = groups[(i, j)]
            if plain:
                a, b = e[1] + e[2], e[2] - e[1]
                outs = [a, b, (e[3] - b) + e[3], (e[0] - a) + e[0]]
            else:
                outs = [tcore(e, k) for k in range(1, 8)]
            for k, t in enumerate(outs):
                c0 = ((n + k) % 2) * Q
                tb_ref.at[l, (n + k) // 2][pl.ds(r, CR), c0:c0 + Q] = t.astype(bf16)


NW = 8


def kernel(x_hbm, w_hbm, b_ref, o_hbm, t_ref, bt_ref, hs_ref, ts_ref, w_buf, x_buf, o_buf,
           w_sem, x_sem, o_sem, *, L, nb, groups, opt):
    nblk = opt["nblk"]
    NX, NO = x_buf.shape[0], o_buf.shape[0]
    nch = Q // CR

    def wcopy(c):
        return pltpu.make_async_copy(
            w_hbm.at[c // nch, :, pl.ds(pl.multiple_of((c % nch) * CR, CR), CR), :],
            w_buf.at[c % NW], w_sem.at[c % NW])

    def xcopy(i):
        return pltpu.make_async_copy(x_hbm.at[pl.ds(pl.multiple_of(i * TM, TM), TM), :],
                                     x_buf.at[i & (NX - 1)], x_sem.at[i & (NX - 1)])

    def ocopy(i):
        return pltpu.make_async_copy(o_buf.at[i & (NO - 1)], o_hbm.at[pl.ds(pl.multiple_of(i * TM, TM), TM), :],
                                     o_sem.at[i & (NO - 1)])

    for c in range(NW - 1):
        wcopy(c).start()
    for i in range(nblk + 1):
        xcopy(i).start()
    for l in range(L):
        for e in range(4):
            for bc in range(8):
                row = b_ref[l:l + 1, bc * Q:(bc + 1) * Q].astype(f32) * (S3 ** (e - popc(bc)))
                bt_ref[l * 4 + e, :, bc * Q:(bc + 1) * Q] = jnp.broadcast_to(row, (SR, Q))
    ts_ref[...] = jnp.zeros(ts_ref.shape, f32)
    tb_ref = t_ref.bitcast(bf16)

    def build(c, carry):
        wcopy(c).wait()

        @pl.when(c + NW - 1 < L * nch)
        def _():
            wcopy(c + NW - 1).start()

        build_chunk(w_buf.at[c % NW], tb_ref, c // nch, pl.multiple_of((c % nch) * CR, CR), groups)
        return carry

    jax.lax.fori_loop(0, L * nch, build, 0)

    xcopy(0).wait()
    S = Sched(None, opt)
    head(S, [load_z(x_buf.at[0], o) for o in range(4)], [RefArr(hs_ref, b) for b in range(4)], 0)
    S.drain()

    def dmas(i0):
        cps = [xcopy(jnp.minimum(i0 + 2, nb - 1)), ocopy(jnp.maximum(i0 - 2, 0)),
               xcopy(jnp.minimum(i0 + 1, nb - 1)), ocopy(jnp.maximum(i0 - 3, 0))]
        pl.when(i0 + 2 < nb)(cps[0].start)
        pl.when(i0 >= 2)(cps[1].start)
        pl.when(i0 + 1 < nb)(cps[2].wait)
        pl.when(i0 >= 3)(cps[3].wait)

    def step(i0, carry):
        never = jnp.full((SR, Q), i0, jnp.int32) < 0
        xs = [x_buf.at[jnp.clip(i0 + u, 0, nb - 1) & (NX - 1)] for u in range(-1, 2)]
        outs = [o_buf.at[(i0 + 1) & 1]]
        body(xs, outs, bt_ref, t_ref, hs_ref, ts_ref, L, groups, never, opt)
        dmas(i0 + 1)
        return carry

    dmas(jnp.int32(0))
    jax.lax.fori_loop(0, nb // nblk, step, 0)
    assert nblk == 1
    S = Sched(None, opt)
    tail(S, [load_z(x_buf.at[(nb - 1) % NX], o) for o in range(4)], bt_ref, o_buf.at[(nb - 1) % NO],
         [RefArr(ts_ref, n) for n in range(10)], L)
    S.drain(bg=True)
    ocopy(nb - 1).start()
    for i in range(max(nb - NO, 0), nb):
        ocopy(i).wait()


def make(o=None):
    opt = dict(OPT)
    opt.update(o or {})
    groups, n = plan(opt["skip"])

    @jax.jit
    def run(x0, ws, bs):
        B, D = x0.shape
        L = ws.shape[0]
        nb, nblk = B // TM, opt["nblk"]
        NX, NO = 2 * nblk + 2, 2 * nblk
        return pl.pallas_call(
            functools.partial(kernel, L=L, nb=nb, groups=groups, opt=opt),
            in_specs=[pl.BlockSpec(memory_space=pl.ANY),
                      pl.BlockSpec(memory_space=pl.ANY),
                      pl.BlockSpec(memory_space=pltpu.VMEM)],
            out_specs=pl.BlockSpec(memory_space=pl.ANY),
            out_shape=jax.ShapeDtypeStruct((B, D), x0.dtype),
            scratch_shapes=[
                pltpu.VMEM((L, (n + 1) // 2, Q // 2, 2 * Q), jnp.uint32),
                pltpu.VMEM((L * 4, SR, D), f32),
                pltpu.VMEM((4, 4 * R, D // 2), f32),
                pltpu.VMEM((10, 4 * R, D // 2), f32),
                pltpu.VMEM((NW, 8, CR, D), bf16),
                pltpu.VMEM((NX, TM, D), bf16),
                pltpu.VMEM((NO, TM, D), bf16),
                pltpu.SemaphoreType.DMA((NW,)),
                pltpu.SemaphoreType.DMA((NX,)),
                pltpu.SemaphoreType.DMA((NO,)),
            ],
            compiler_params=pltpu.CompilerParams(vmem_limit_bytes=120 * 1024 * 1024,
                                                 disable_bounds_checks=opt["nobc"]),
        )(x0, ws.reshape(L, 8, Q, D), bs)

    return run


_run = make()


@jax.jit
def pallas_standalone__dcn_v2_cross__recsys_kernel(x0: jax.Array, ws: jax.Array, bs: jax.Array):
    return _run(x0, ws, bs)
```

```python
import functools
import math

import jax
import jax.numpy as jnp
import jax.experimental.pallas as pl
import jax.experimental.pallas.tpu as pltpu

f32 = jnp.float32
bf16 = jnp.bfloat16

Q = 128
R = 32
SR = 8
NS = R // SR
TM = 8 * R
CR = 16
S3 = math.sqrt(3.0)
IN = [(p, q) for p in range(4) for q in range(4)]

CORE3 = {1: [(1, 0)], 3: [(1, 1)], 5: [(1, 2)], 2: [(1, 3)],
         4: [(1, 0), (-1, 1)], 7: [(1, 2), (-1, 0)], 6: [(1, 3), (-1, 0)]}
CORE4 = {1: [(1, 0)], 3: [(1, 1)], 5: [(1, 2)], 2: [(1, 3), (1, 0)],
         4: [(1, 0), (-1, 1)], 7: [(1, 2), (-1, 0)], 6: [(1, 3), (-1, 0)]}
SIGMA = {1: 1, 2: 3, 3: 7, 4: 6, 5: 4, 6: 5, 7: 2}
ORDER1 = [3, 5, 1, 4, 7, 6, 2]
QORD = [2, 1, 0, 3]
TORD = [1, 0, 3, 2]
AFTER = {2: [], 1: [(3, 1, 1, 2)], 0: [(1, 0, -1, 1), (2, 0, 1, 1)], 3: [(0, 3, 1, 0)]}

OPT = dict(skip=13, nblk=1, row=2, margin=27, rates=[9.2, 7, 11.5, 5.5, 5.5, 5.5, 5.4], brates=[2.0] * 7,
           rates0=[9.2, 9.4, 10, 6, 6, 5.5, 5.4], rates5=[9.2, 7, 12.4, 5.5, 5.5, 5.5, 5.4],
           brates0=[2.0, 2.3, 1.0, 2.0, 3.0, 2.0, 3.0],
           pre=2, ic=18.0, endm=25, tsplit=1, split=0, a3='alt', c3='d', od=[3, 4, 5, 1, 7, 6, 2],
           mj=[1.0] * 7, cap=40.0, o2=[1, 4, 2, 7, 6, 5, 3], o3=[3, 5, 4, 7, 1, 2, 6], raw2=0, raw3=0,
           o1=[3, 5, 1, 4, 7, 6, 2], wh=1, w0=1, nobc=True)


def lin(terms):
    pos = [v for s, v in terms if s > 0]
    neg = [v for s, v in terms if s < 0]
    acc = pos[0]
    for v in pos[1:]:
        acc = acc + v
    for v in neg:
        acc = acc - v
    return acc


def chain(terms):
    acc = terms[0][1]
    for s, v in terms[1:]:
        acc = acc + v if s > 0 else acc - v
    return acc


def phi3(a):
    l5 = a[0] + a[1]
    return [a[0] + a[3], a[0] - a[1], l5, 0.5 * (l5 + a[3] + a[2])]


def phi4(a):
    return [a[0] + a[3], a[0] - a[1], a[0] + a[1], a[1] + a[2]]


def phi4_inv(e, hf=0.5):
    a11 = hf * (e[1] + e[2])
    a12 = e[2] - a11
    return [a11, a12, e[3] - a12, e[0] - a11]


def psi6(c, hf):
    h = hf * c[3]
    c11 = h + c[0]
    return [c11, h, (h + c[1]) + c[2], (c11 + c[1]) - c[2]]


def rc(o, p, q):
    return (o // 2) * 4 + (p // 2) * 2 + q // 2, (o % 2) * 4 + (p % 2) * 2 + q % 2


def popc(v):
    return bin(v).count("1")


def scale(br, bc):
    return S3 ** (popc(br) - popc(bc))


def plan(skip):
    groups, n = {}, 0
    for i in range(1, 8):
        for j in range(1, 8):
            plain = ((skip == 13 and (i == 1 or j == 1)) or (skip == 7 and i == 1)
                     or (skip == 1 and i == 1 and j == 1))
            groups[(i, j)] = (n, plain)
            n += 4 if plain else 7
    return groups, n


def comb2(u, sg, v, x=None, e=None):
    if x is not None:
        u = u + x
    if e is not None:
        v = v + e if sg > 0 else v - e
    return u + v if sg > 0 else u - v


class RefArr:
    def __init__(self, ref, idx):
        self.ref, self.idx = ref, idx

    def __getitem__(self, k):
        return self.ref[self.idx, k[0] * R:(k[0] + 1) * R, k[1] * Q:(k[1] + 1) * Q]

    def get(self, s, k):
        r = k[0] * R + s * SR
        return self.ref[self.idx, r:r + SR, k[1] * Q:(k[1] + 1) * Q]

    def put(self, s, k, v):
        r = k[0] * R + s * SR
        self.ref[self.idx, r:r + SR, k[1] * Q:(k[1] + 1) * Q] = v

    def putb(self, k, v):
        self.ref[self.idx, k[0] * R:(k[0] + 1) * R, k[1] * Q:(k[1] + 1) * Q] = v


class ValArr:
    def __init__(self, blocks=None):
        self.parts = [dict() for _ in range(NS)]
        self.blocks = dict(blocks or {})

    def __getitem__(self, k):
        if k not in self.blocks:
            self.blocks[k] = jnp.concatenate([p[k] for p in self.parts], axis=0)
        return self.blocks[k]

    def get(self, s, k):
        if k not in self.parts[s]:
            self.parts[s][k] = self.blocks[k][s * SR:(s + 1) * SR]
        return self.parts[s][k]

    def put(self, s, k, v):
        self.parts[s][k] = v

    def putb(self, k, v):
        self.blocks[k] = v


class Sched:
    def __init__(self, never, opt):
        self.never, self.opt = never, opt
        self.q, self.bg, self.lock = [], [], None
        self.g, self.t, self.pace, self.bcredit, self.forced = None, 0, 0.0, 0.0, []

    def gv(self, v):
        return v if self.g is None else jnp.where(self.never, self.g, v)

    def gc(self, c):
        return c if self.g is None else jnp.where(self.never, self.g, jnp.full((SR, Q), c, f32))

    def add(self, gen, deadline, cost, bg=False):
        (self.bg if bg else self.q).append([gen, deadline, cost])
        return gen

    def step(self, q):
        while q:
            try:
                c = next(q[0][0])
            except StopIteration:
                q.pop(0)
                continue
            self.lock = None if isinstance(c, float) else q
            q[0][2] -= c
            return c
        return None

    def tick(self, val, base, brate, mult=1.0):
        rate, cum = base, 0.0
        for _, dl, cost in self.q:
            cum += max(cost, 0)
            rate = max(rate, cum / max(dl - self.opt["margin"] - self.t, 1))
        self.bcredit = min(self.bcredit + brate + (0.0 if self.q else base), 40.0)
        self.pace = min(self.pace + mult * (rate + (brate if self.bg else 0.0)), self.opt['cap'])
        if self.pace > 0:
            if self.lock:
                q = self.lock
            elif self.bg and (not self.q or (self.bcredit > 0 and rate <= base)):
                q = self.bg
            else:
                q = self.q
            if q:
                r = self.opt["row"]
                self.g = val[r * SR:(r + 1) * SR]
                c = self.step(q)
                self.g = None
                if c:
                    self.pace -= c
                    if q is self.bg:
                        self.bcredit -= c
        self.t += 1

    def drain(self, gen=None, bg=False):
        n, q = 0, (self.bg if bg else self.q)
        while q and (gen is None or any(e[0] is gen for e in q)):
            if self.step(q) is not None:
                n += 1
        self.forced.append(n)


def load_z(ref, o):
    zz = {}
    for k in IN:
        br, bc = rc(o, *k)
        zz[k] = ref[br * R:(br + 1) * R, bc * Q:(bc + 1) * Q].astype(f32)
    return ValArr(zz)


def finish(S, dd, q, d, s, emit):
    if S.opt["a3"] == "alt":
        r = phi3(dd)
        for p in range(4):
            d[(p, q)] = r[p]
            for (b, i, sg, j) in AFTER[q]:
                emit(s, (p, b), d[(p, i)], sg, d[(p, j)])
    else:
        emit(s, (0, q), dd[0], 1, dd[3])
        emit(s, (1, q), dd[0], -1, dd[1])
        emit(s, (2, q), dd[0], 1, dd[1])
        emit(s, (3, q), 0.5 * ((dd[0] + dd[1]) + dd[3]), 1, 0.5 * dd[2])


def head_q(S, o, z, emit):
    for s in range(NS):
        d = {}
        for q in QORD:
            v = []
            for p in range(4):
                sc = scale(*rc(o, p, q))
                v.append(z.get(s, (p, q)) * sc if sc != 1.0 else z.get(s, (p, q)))
            finish(S, [S.gv(v[0])] + v[1:], q, d, s, emit)
            yield 22.0 if q == QORD[-1] else 22


def head(S, z, H, dl):
    d1, d0 = ValArr(), ValArr()

    def e1(s, k, u, sg, v):
        d1.put(s, k, comb2(u, sg, v))

    def e0(s, k, u, sg, v):
        r = comb2(u, sg, v)
        d0.put(s, k, r)
        H[1].put(s, k, r - d1.get(s, k))
        H[2].put(s, k, r + d1.get(s, k))

    def e2(s, k, u, sg, v):
        H[3].put(s, k, comb2(u, sg, v, d1.get(s, k)))

    def e3(s, k, u, sg, v):
        H[0].put(s, k, comb2(u, sg, v, d0.get(s, k)))

    gs = [head_q(S, o, z[o], e) for o, e in ((1, e1), (2, e2), (0, e0), (3, e3))]

    def allq():
        for _ in range(NS):
            for g in gs:
                for _ in range(4):
                    yield next(g)

    return S.add(allq(), dl, 16 * NS * 22)


def costs(o, n, last, opt):
    e = 4 * (n - 1)
    if opt["c3"] == "alt":
        ca, pre = (1, {1: e, 0: e, 3: 12 + 2 * e, 2: 8}) if last else (4 * n, {2: 4 * n, 1: 0, 0: e, 3: 4})
    else:
        ca, pre = 1, {q: e for q in range(4)}
    if last:
        post = {1: 23, 0: 13, 3: 13, 2: 13} if opt["a3"] == "alt" else {q: 11 for q in range(4)}
    elif opt["a3"] == "alt":
        post = {q: {1: 4, 0: 4, 3: 12, 2: 12}[o] * len(AFTER[q]) for q in range(4)}
    else:
        post = {q: {1: 1, 0: 1, 3: 10, 2: 10}[o] for q in range(4)}
    return ca, {q: 21 + pre[q] + post[q] for q in range(4)}


def epi(S, o, terms, z, bt_ref, l, emit=None, xo=None, out=None):
    ca, cb = costs(o, len(terms), emit is None, S.opt)
    qord = TORD if emit is None else QORD
    for s in range(NS):
        cmb = lambda k: chain([(sg, m.get(s, k)) for sg, m in terms])
        c, d = {}, {}
        for p in range(4):
            if S.opt["c3"] == "alt":
                c6, c2 = cmb((p, 1)), cmb((p, 2))
                c[(p, 1)] = cmb((p, 3))
                c[(p, 2)] = (c6 + c2) + c[(p, 1)]
                c[(p, 0)] = cmb((p, 0))
                c[(p, 3)] = (c6 - c2) + c[(p, 0)]
            else:
                for q in range(4):
                    c[(p, q)] = cmb((p, q))
            if p % 2 == 1:
                yield ca
        if emit is None:
            xi = {p: (phi4_inv if S.opt['a3'] == 'alt' else list)([xo.get(s, (p, q)) for q in range(4)]) for p in range(4)}
        for q in qord:
            hf = S.gc(0.5)
            y = psi6([c[(p, q)] for p in range(4)], hf)
            c2nd = 0
            if S.opt["split"] and emit is not None:
                c2nd = 14 + {1: 4, 0: 4, 3: 12, 2: 12}[o] * len(AFTER[q])
                yield cb[q] - c2nd
            if S.opt["tsplit"] and emit is None:
                c2nd = cb[q] // 2
                yield cb[q] - c2nd
                hf = S.gc(0.5)
            dd = []
            for p in range(4):
                br, bc = rc(o, p, q)
                yy = S.gv(y[p]) if (p == 0 and S.opt["split"] == 2 and emit is not None) else y[p]
                dd.append((yy + bt_ref[l * 4 + popc(br), :, bc * Q:(bc + 1) * Q]) * z.get(s, (p, q)))
            if emit is None:
                e = [xi[p][q] for p in range(4)]
                a11 = hf * (e[1] + e[2])
                a22 = e[0] - a11
                xn = [a11, e[2] - a11, ((e[3] - a22) + e[3]) - e[2], a22]
                for p in range(4):
                    br, bc = rc(o, p, q)
                    r = dd[p] + xn[p]
                    if scale(br, bc) != 1.0:
                        r = r * (1.0 / scale(br, bc))
                    d[(p, q)] = r
                    if (p, q ^ 1) in d:
                        b0, r0 = bc & ~1, br * R + s * SR
                        pair = jnp.concatenate([d[(p, q & ~1)], d[(p, q | 1)]], axis=1)
                        out[r0:r0 + SR, b0 * Q:(b0 + 2) * Q] = pair.astype(bf16)
            else:
                if S.opt["split"] == 1:
                    dd[0] = S.gv(dd[0])
                finish(S, dd, q, d, s, emit)
            cc = c2nd if c2nd else cb[q]
            yield float(cc) if q == qord[-1] else cc


def add_epi(S, dl, o, terms, *a, **kw):
    last = kw.get("emit") is None
    ca, cb = costs(o, len(terms), last, S.opt)
    return S.add(epi(S, o, terms, *a, **kw), dl, NS * (2 * ca + sum(cb.values())), bg=last)


NAMES = ["h", "w", "m4", "m7", "m6", "m2"]
TERMS = {1: [(1, "h")], 0: [(1, "m7"), (1, "w"), (1, "m4")], 3: [(1, "w"), (-1, "m2"), (1, "m6")],
         2: [(1, "m2"), (1, "m6"), (1, "h"), (1, "m4"), (-1, "m7")]}


def tail(S, z, bt_ref, out, TS, L, quads=(0, 1, 2, 3)):
    for o in quads:
        g = add_epi(S, 0, o, [(sg, TS[4 + NAMES.index(n)]) for sg, n in TERMS[o]], z[o], bt_ref, L - 1,
                    xo=TS[o], out=out)
    return g


def inv1(S, X, TS):
    for s in range(NS):
        for p in range(4):
            for q0 in (0, 2):
                hf = S.gc(0.5)
                for q in (q0, q0 + 1):
                    r = phi4_inv([X[b].get(s, (p, q)) for b in range(4)], hf)
                    for o in range(4):
                        TS[o].put(s, (p, q), r[o])
                yield S.opt["ic"]


def inner(mul):
    m3 = mul(3)
    m5 = mul(5)
    yield 3, m5 + m3
    c = m3 - m5
    m4 = mul(4)
    c = m4 + c
    m7 = mul(7)
    c = m7 + c
    yield 0, mul(1) + c
    m2 = mul(2)
    yield 2, m2 + m4
    m6 = mul(6)
    yield 1, m6 - m7


def sadd(a, b):
    if a is None:
        return b
    if a[0] == b[0]:
        return (a[0], b[1] + a[1])
    return (1, a[1] - b[1]) if a[0] > 0 else (1, b[1] - a[1])


def inner_direct(mul, od):
    need = {"w": {1: 1, 3: 1, 5: -1}, "h": {3: 1, 5: 1}, 0: {"w": 1, 4: 1, 7: 1}, 3: {"w": 1, 6: 1, 2: -1},
            2: {"h": 1, 4: 1, 7: -1, 6: 1, 2: 1}}
    acc = {n: None for n in need}
    left = {n: set(t) for n, t in need.items()}
    for k in od:
        todo = [(k, mul(k))]
        while todo:
            name, v = todo.pop(0)
            for n, t in need.items():
                if name in left[n]:
                    left[n].discard(name)
                    acc[n] = sadd(acc[n], (t[name], v))
                    if not left[n]:
                        assert acc[n][0] > 0
                        if n == "h":
                            yield 1, acc[n][1]
                        if n in ("w", "h"):
                            todo.append((n, acc[n][1]))
                        else:
                            yield n, acc[n][1]


def middle(gen):
    c0 = dict(gen(1))
    m4 = {}
    for q, c in gen(4):
        m4[q] = c
        c0[q] = c0[q] + c
    for q, c in gen(2):
        yield 2, q, c + m4[q]
    m7 = {}
    for q, c in gen(7):
        m7[q] = c
        c0[q] = c0[q] + c
    for q, c in gen(6):
        yield 1, q, c - m7[q]
    m5 = {}
    for q, c in gen(5):
        m5[q] = c
        yield 0, q, c0[q] - c
    for q, c in gen(3):
        yield 3, q, c + m5[q]


OUT2 = {0: {1: 1, 4: 1, 7: 1, 5: -1}, 1: {6: 1, 7: -1}, 2: {2: 1, 4: 1}, 3: {3: 1, 5: 1}}
OUT3 = {0: {1: 1, 4: 1, 7: 1, 5: -1, 3: 1}, 1: {6: 1, 7: -1}, 2: {2: 1, 4: 1}, 3: {3: 1, 5: 1}}


def combine(gen, order, OUT, raw):
    part = {o: [] for o in OUT}
    done = set()
    for j in order:
        done.add(j)
        new = {o: {} for o in OUT}
        for q, c in gen(j):
            for o, t in OUT.items():
                if j not in t:
                    continue
                fin = all(x in done for x in t)
                if fin or (not raw and part[o]):
                    sg, acc = t[j], c
                    for pr in reversed(part[o]):
                        s2, v = pr[q]
                        if sg == s2:
                            acc = acc + v
                        elif sg > 0:
                            acc = acc - v
                        else:
                            sg, acc = 1, v - acc
                    if fin:
                        assert sg > 0
                        yield o, q, acc
                    else:
                        new[o][q] = (sg, acc)
                else:
                    new[o][q] = (t[j], c)
        for o, t in OUT.items():
            if j in t and new[o]:
                part[o] = (part[o] + [new[o]]) if raw else [new[o]]


def body(xs, outs, bt_ref, t_ref, hs_ref, ts_ref, L, groups, never, opt):
    S = Sched(never, opt)
    cum = [0]
    for i in opt['o1']:
        cum.append(cum[-1] + sum(8 if groups[(i, j)][1] else 7 for j in range(1, 8)))
    TL, mg = cum[-1], opt["margin"]
    nblk = len(outs)
    zs = [[load_z(x, o) for o in range(4)] for x in xs]
    X = [RefArr(hs_ref, b) for b in range(4)]
    TS = [RefArr(ts_ref, n) for n in range(10)]
    pre = [(10 if opt["tsplit"] else 6) * opt["pre"]]

    def tile(l, n):
        return pltpu.bitcast(t_ref[l, n // 2, :, (n % 2) * Q:(n % 2 + 1) * Q], bf16)

    for sb in range(nblk):
        z = zs[sb + 1]
        need = None
        tl = tail(S, zs[sb], bt_ref, outs[sb], TS, L)
        final = sb == nblk - 1
        for l in range(L):
            T0 = (sb * L + l) * TL
            last = l == L - 1

            def prod1(i):
                base = opt.get("rates%d" % l, opt["rates"])[ORDER1.index(i)]
                brate = opt.get("brates%d" % l, opt["brates"])[ORDER1.index(i)]

                def gen2(j):
                    a = [lin([(s1 * s2, X[b1][(b2, q)]) for s1, b1 in CORE4[i] for s2, b2 in CORE3[j]])
                         for q in range(4)]
                    n, plain = groups[(i, j)]
                    mult = opt['mj'][opt['o2'].index(j)] * 7.0 / sum(opt['mj'])
                    if plain:
                        an = phi4_inv(a) if opt['a3'] == 'alt' else a
                        k0 = jnp.concatenate([an[0], an[2]], axis=0).astype(bf16)
                        k1 = jnp.concatenate([an[1], an[3]], axis=0).astype(bf16)

                        def dot2(u, k):
                            r = jnp.dot(u, tile(l, n + k), preferred_element_type=f32)
                            S.tick(r[:R], base, brate, mult)
                            S.tick(r[R:], base, brate, mult)
                            return r

                        c0 = dot2(k0, 0) + dot2(k1, 2)
                        c1 = dot2(k0, 1) + dot2(k1, 3)
                        n11, n12, n21, n22 = c0[:R], c1[:R], c0[R:], c1[R:]
                        if opt["c3"] == "alt":
                            df = n22 - n11
                            c6 = 0.5 * ((n21 - n12) + df)
                            yield 0, n11
                            yield 3, n12
                            yield 1, c6
                            yield 2, c6 - df
                        else:
                            yield from enumerate([n11, n12, n21, n22])
                    else:
                        def mul(k):
                            if opt["a3"] == "alt":
                                u = lin([(s3, a[b]) for s3, b in CORE4[k]])
                            else:
                                u = {1: lambda: a[0] + a[3], 3: lambda: a[0] - a[1], 5: lambda: a[0] + a[1],
                                     4: lambda: a[1] + a[3], 7: lambda: a[1] - a[3],
                                     2: lambda: (a[1] + a[2]) + (a[0] + a[3]),
                                     6: lambda: (a[1] + a[2]) - (a[0] + a[3])}[k]()
                            if len(CORE4[k]) == 2:
                                for r_ in range(2):
                                    if pre[0] > 0:
                                        S.g = u[r_ * 16:r_ * 16 + SR]
                                        S.step(S.bg)
                                        S.g = None
                                        pre[0] -= 1
                            r = jnp.dot(u.astype(bf16), tile(l, n + k - 1), preferred_element_type=f32)
                            S.tick(r, base, brate, mult)
                            return r

                        if opt["c3"] == "alt":
                            for q, _, c in combine(lambda k: [(0, mul(k))], opt['o3'], OUT3, opt['raw3']):
                                yield q, c
                        else:
                            yield from inner_direct(mul, opt["od"])

                return {(p, q): c for p, q, c in combine(gen2, opt['o2'], OUT2, opt['raw2'])}

            XN = [ValArr() for _ in range(4)]
            d12, d11 = ValArr(), ValArr()

            def emitter(o, X=X, XN=XN, d12=d12, d11=d11):
                def emit(s, k, u, sg, v):
                    if o == 1:
                        d12.put(s, k, comb2(u, sg, v))
                    elif o == 0:
                        e, r = d12.get(s, k), comb2(u, sg, v)
                        d11.put(s, k, r)
                        XN[1].put(s, k, (r + X[1].get(s, k)) - e)
                        XN[2].put(s, k, (r + X[2].get(s, k)) + e)
                    elif o == 3:
                        XN[0].put(s, k, comb2(u, sg, v, X[0].get(s, k), d11.get(s, k)))
                    else:
                        XN[3].put(s, k, comb2(u, sg, v, X[3].get(s, k), d12.get(s, k)))
                return emit

            nn = {}
            if last:
                S.drain(tl, bg=True)
                TS = [RefArr(ts_ref, n) if final else ValArr() for n in range(10)]
                XN = [RefArr(hs_ref, b) if final else ValArr() for b in range(4)]

            M = {}

            def keep(name, m):
                M[name] = ValArr(m)
                if last:
                    for k in IN:
                        TS[4 + NAMES.index(name)].putb(k, m[k])

            def add(o, dl):
                if not last:
                    nn[o] = add_epi(S, dl, o, [(sg, M[n]) for sg, n in TERMS[o]], z[o], bt_ref, l,
                                    emit=emitter(o))

            if need:
                S.drain(need[0])
            o1 = opt["o1"]
            mm = {i: prod1(i) for i in o1[:2]}
            if last:
                dl = T0 + TL + (opt["endm"] if final else 0)
                S.add(inv1(S, X, TS), dl, NS * 8 * opt["ic"])
                head(S, zs[sb + 2], XN, dl)
            keep("h", {k: mm[o1[1]][k] + mm[o1[0]][k] for k in IN})
            w = {k: mm[3][k] - mm[5][k] for k in IN}
            add(1, T0 + cum[5] + mg)
            if need:
                S.drain(need[3])
            for i in o1[2:5]:
                m = prod1(i)
                if i == 1:
                    keep("w", {k: m[k] + w[k] for k in IN})
                else:
                    keep("m%d" % i, m)
            add(0, T0 + TL)
            if need:
                S.drain(need[2])
            for i in o1[5:]:
                keep("m%d" % i, prod1(i))
            add(3, T0 + TL + cum[2])
            add(2, T0 + TL + cum[5])
            need = nn
            X = XN
        S.drain()
    if opt.get("verbose"):
        print("forced", S.forced)


def tcore(e, k):
    if k == 1:
        return e[0] + e[0]
    return lin([(s, e[b]) for s, b in CORE4[SIGMA[k]]])


def table_basis(w_ref, e_ref):
    d = []
    for o in range(4):
        v, t, u = {}, {}, {}
        for k in IN:
            br, bc = rc(o, *k)
            v[k] = w_ref[br, :, bc * Q:(bc + 1) * Q].astype(f32) * (0.25 * scale(br, bc))
        for q in range(4):
            for p, x in enumerate(phi3([v[(p, q)] for p in range(4)])):
                t[(p, q)] = x
        for p in range(4):
            for q, x in enumerate(phi4([t[(p, q)] for q in range(4)])):
                u[(p, q)] = x
        d.append(u)
    for k in IN:
        for b, x in enumerate(phi4([d[o][k] for o in range(4)])):
            e_ref[b * 16 + k[0] * 4 + k[1]] = x


def table_tiles(e_ref, tb_ref, l, r, groups, i):
    s1 = {k: tcore([e_ref[b * 16 + k[0] * 4 + k[1]] for b in range(4)], i) for k in IN}
    for j in range(1, 8):
        e = [lin([(sg, s1[(b, q)]) for sg, b in CORE3[SIGMA[j]]]) for q in range(4)]
        n, plain = groups[(i, j)]
        if plain:
            a, b = e[1] + e[2], e[2] - e[1]
            outs = [a, b, (e[3] - b) + e[3], (e[0] - a) + e[0]]
        else:
            outs = [tcore(e, k) for k in range(1, 8)]
        for k, t in enumerate(outs):
            c0 = ((n + k) % 2) * Q
            tb_ref.at[l, (n + k) // 2][pl.ds(r, CR), c0:c0 + Q] = t.astype(bf16)


NW = 8
NX = 4
NO = 2


def kernel(x_hbm, w_hbm, b_hbm, o_hbm, t_ref, bt_ref, hs_ref, ts_ref, e_ref, w_buf, x_buf, o_buf, b_buf,
           w_sem, x_sem, o_sem, b_sem, *, L, nb, groups, opt):
    nc = L * NW

    def wcopy(c):
        slot = c & (NW - 1)
        return pltpu.make_async_copy(w_hbm.at[c >> 3, :, pl.ds(pl.multiple_of(slot * CR, CR), CR), :],
                                     w_buf.at[slot], w_sem.at[slot])

    def xcopy(i):
        return pltpu.make_async_copy(x_hbm.at[pl.ds(pl.multiple_of(i * TM, TM), TM), :],
                                     x_buf.at[i & (NX - 1)], x_sem.at[i & (NX - 1)])

    def ocopy(i):
        return pltpu.make_async_copy(o_buf.at[i & (NO - 1)], o_hbm.at[pl.ds(pl.multiple_of(i * TM, TM), TM), :],
                                     o_sem.at[i & (NO - 1)])

    bcopy = pltpu.make_async_copy(b_hbm, b_buf, b_sem.at[0])
    bcopy.start()
    xcopy(0).start()
    for c in range(opt["w0"]):
        wcopy(c).start()
    ts_ref[...] = jnp.zeros(ts_ref.shape, f32)
    bcopy.wait()
    for c in range(opt["w0"], NW):
        wcopy(c).start()
    for l in range(L):
        for e in range(4):
            for bc in range(8):
                row = b_buf[l:l + 1, bc * Q:(bc + 1) * Q].astype(f32) * (S3 ** (e - popc(bc)))
                bt_ref[l * 4 + e, :, bc * Q:(bc + 1) * Q] = jnp.broadcast_to(row, (SR, Q))
    xcopy(0).wait()
    S = Sched(None, opt)
    head(S, [load_z(x_buf.at[0], o) for o in range(4)], [RefArr(hs_ref, b) for b in range(4)], 0)
    S.drain()
    tb_ref = t_ref.bitcast(bf16)
    wcopy(0).wait()
    xcopy(1).start()

    def build(c, carry):
        slot = c & (NW - 1)

        def half(h, cc):
            rows = pl.ds(pl.multiple_of(h * SR, SR), SR)
            table_basis(w_buf.at[slot, :, rows, :], e_ref.at[0, :, rows, :])
            return cc

        jax.lax.fori_loop(0, CR // SR, half, 0)
        nxt, refill = wcopy(jnp.minimum(c + 1, nc - 1)), wcopy(jnp.minimum(c + NW, nc - 1))
        for i in range(1, 8):
            table_tiles(e_ref.at[(c + i) >> 10], tb_ref, c >> 3, pl.multiple_of(slot * CR, CR), groups, i)
        pl.when(c + NW < nc)(refill.start)
        pl.when(c + 1 < nc)(nxt.wait)
        return carry

    jax.lax.fori_loop(0, nc, build, 0)

    def dmas(i0):
        cps = [xcopy(jnp.minimum(i0 + 2, nb - 1)), ocopy(jnp.maximum(i0 - 2, 0)),
               xcopy(jnp.minimum(i0 + 1, nb - 1)), ocopy(jnp.maximum(i0 - 3, 0))]
        pl.when(i0 + 2 < nb)(cps[0].start)
        pl.when(i0 >= 2)(cps[1].start)
        pl.when(i0 + 1 < nb)(cps[2].wait)
        pl.when(i0 >= 3)(cps[3].wait)

    def step(i0, carry):
        never = jnp.full((SR, Q), i0, jnp.int32) < 0
        xs = [x_buf.at[jnp.clip(i0 + u, 0, nb - 1) & (NX - 1)] for u in range(-1, 2)]
        outs = [o_buf.at[(i0 + 1) & 1]]
        body(xs, outs, bt_ref, t_ref, hs_ref, ts_ref, L, groups, never, opt)
        dmas(i0 + 1)
        return carry

    dmas(jnp.int32(0))
    jax.lax.fori_loop(0, nb, step, 0)

    last, H = nb - 1, TM // 2
    z = [load_z(x_buf.at[last % NX], o) for o in range(4)]
    halves = [pltpu.make_async_copy(o_buf.at[last % NO, pl.ds(h * H, H), :],
                                    o_hbm.at[pl.ds(last * TM + h * H, H), :], b_sem.at[1 + h]) for h in range(2)]
    for h in range(2):
        S = Sched(None, opt)
        tail(S, z, bt_ref, o_buf.at[last % NO], [RefArr(ts_ref, n) for n in range(10)], L, (2 * h, 2 * h + 1))
        S.drain(bg=True)
        halves[h].start()
    ocopy(last - 1).wait()
    for h in range(2):
        halves[h].wait()


def make(o=None):
    opt = dict(OPT)
    opt.update(o or {})
    groups, n = plan(opt["skip"])

    @jax.jit
    def run(x0, ws, bs):
        B, D = x0.shape
        L = ws.shape[0]
        nb = B // TM
        return pl.pallas_call(
            functools.partial(kernel, L=L, nb=nb, groups=groups, opt=opt),
            in_specs=[pl.BlockSpec(memory_space=pl.ANY),
                      pl.BlockSpec(memory_space=pl.ANY),
                      pl.BlockSpec(memory_space=pl.ANY)],
            out_specs=pl.BlockSpec(memory_space=pl.ANY),
            out_shape=jax.ShapeDtypeStruct((B, D), x0.dtype),
            scratch_shapes=[
                pltpu.VMEM((L, (n + 1) // 2, Q // 2, 2 * Q), jnp.uint32),
                pltpu.VMEM((L * 4, SR, D), f32),
                pltpu.VMEM((4, 4 * R, D // 2), f32),
                pltpu.VMEM((10, 4 * R, D // 2), f32),
                pltpu.VMEM((2, 64, CR, Q), f32),
                pltpu.VMEM((NW, 8, CR, D), bf16),
                pltpu.VMEM((NX, TM, D), bf16),
                pltpu.VMEM((NO, TM, D), bf16),
                pltpu.VMEM((L, D), bf16),
                pltpu.SemaphoreType.DMA((NW,)),
                pltpu.SemaphoreType.DMA((NX,)),
                pltpu.SemaphoreType.DMA((NO,)),
                pltpu.SemaphoreType.DMA((3,)),
            ],
            compiler_params=pltpu.CompilerParams(vmem_limit_bytes=120 * 1024 * 1024,
                                                 disable_bounds_checks=opt["nobc"]),
        )(x0, ws.reshape(L, 8, Q, D), bs)

    return run


_run = make()


@jax.jit
def pallas_standalone__dcn_v2_cross__recsys_kernel(x0: jax.Array, ws: jax.Array, bs: jax.Array):
    return _run(x0, ws, bs)
```

```python
import functools
import math

import jax
import jax.numpy as jnp
import jax.experimental.pallas as pl
import jax.experimental.pallas.tpu as pltpu

f32 = jnp.float32
bf16 = jnp.bfloat16

Q = 128
R = 32
SR = 8
NS = R // SR
TM = 8 * R
CR = 16
NW = Q // CR
NX = 4
NO = 2
S3 = math.sqrt(3.0)
IN = [(p, q) for p in range(4) for q in range(4)]

CORE3 = {1: [(1, 0)], 3: [(1, 1)], 5: [(1, 2)], 2: [(1, 3)],
         4: [(1, 0), (-1, 1)], 7: [(1, 2), (-1, 0)], 6: [(1, 3), (-1, 0)]}
CORE4 = {1: [(1, 0)], 3: [(1, 1)], 5: [(1, 2)], 2: [(1, 3), (1, 0)],
         4: [(1, 0), (-1, 1)], 7: [(1, 2), (-1, 0)], 6: [(1, 3), (-1, 0)]}
SIGMA = {1: 1, 2: 3, 3: 7, 4: 6, 5: 4, 6: 5, 7: 2}
ORDER1 = [3, 5, 1, 4, 7, 6, 2]
QORD = [2, 1, 0, 3]
TORD = [1, 0, 3, 2]
AFTER = {2: [], 1: [(3, 1, 1, 2)], 0: [(1, 0, -1, 1), (2, 0, 1, 1)], 3: [(0, 3, 1, 0)]}
NAMES = ["h", "v", "m4", "m7", "m6", "m2"]
TERMS = {1: [(1, "h")], 0: [(1, "m7"), (1, "v"), (1, "m4")], 3: [(1, "v"), (-1, "m2"), (1, "m6")],
         2: [(1, "m2"), (1, "m6"), (1, "h"), (1, "m4"), (-1, "m7")]}

OPT = dict(
    row=2, margin=27, pre=2, ic=18.0, endm=25,
    rates0=[9.2, 9.4, 10, 6, 6.8, 5.5, 5.4], rates1=[9.2, 7, 11.5, 5.5, 5.5, 5.5, 5.4],
    rates2=[9.2, 7, 11.5, 4.8, 4.2, 5.5, 5.4], rates3=[9.2, 7, 11.5, 5.5, 6.7, 5.5, 5.4],
    rates4=[9.2, 7, 11.5, 5.5, 5.5, 5.5, 5.3], rates5=[9.2, 7, 12.4, 4.3, 5.5, 5.5, 5.4],
    brates=[2.0] * 7, brates0=[2.0, 2.3, 1.0, 2.0, 3.0, 2.0, 3.0], brates1=[2.1, 2.0, 2.0, 2.0, 2.0, 2.0, 2.0],
    od=[3, 4, 5, 1, 7, 6, 2], od3=[3, 4, 1, 5, 7, 2, 6], od4=[3, 4, 1, 5, 7, 2, 6], od5=[3, 4, 5, 1, 7, 2, 6])


def lin(terms):
    pos = [v for s, v in terms if s > 0]
    neg = [v for s, v in terms if s < 0]
    acc = pos[0]
    for v in pos[1:]:
        acc = acc + v
    for v in neg:
        acc = acc - v
    return acc


def chain(terms):
    acc = terms[0][1]
    for s, v in terms[1:]:
        acc = acc + v if s > 0 else acc - v
    return acc


def sadd(a, b):
    if a is None:
        return b
    if a[0] == b[0]:
        return (a[0], b[1] + a[1])
    return (1, a[1] - b[1]) if a[0] > 0 else (1, b[1] - a[1])


def comb2(u, sg, v, x=None, e=None):
    if x is not None:
        u = u + x
    if e is not None:
        v = v + e if sg > 0 else v - e
    return u + v if sg > 0 else u - v


def phi3(a):
    l5 = a[0] + a[1]
    return [a[0] + a[3], a[0] - a[1], l5, 0.5 * (l5 + a[3] + a[2])]


def phi4(a):
    return [a[0] + a[3], a[0] - a[1], a[0] + a[1], a[1] + a[2]]


def phi4_inv(e, hf=0.5):
    a11 = hf * (e[1] + e[2])
    a12 = e[2] - a11
    return [a11, a12, e[3] - a12, e[0] - a11]


def psi(c, hf):
    h = hf * c[3]
    c11 = h + c[0]
    return [c11, h, (h + c[1]) + c[2], (c11 + c[1]) - c[2]]


def rc(o, p, q):
    return (o // 2) * 4 + (p // 2) * 2 + q // 2, (o % 2) * 4 + (p % 2) * 2 + q % 2


def popc(v):
    return bin(v).count("1")


def scale(br, bc):
    return S3 ** (popc(br) - popc(bc))


def plan():
    groups, n = {}, 0
    for i in range(1, 8):
        for j in range(1, 8):
            plain = i == 1 or j == 1
            groups[(i, j)] = (n, plain)
            n += 4 if plain else 7
    return groups, n


class RefArr:
    def __init__(self, ref, idx):
        self.ref, self.idx = ref, idx

    def __getitem__(self, k):
        return self.ref[self.idx, k[0] * R:(k[0] + 1) * R, k[1] * Q:(k[1] + 1) * Q]

    def get(self, s, k):
        r = k[0] * R + s * SR
        return self.ref[self.idx, r:r + SR, k[1] * Q:(k[1] + 1) * Q]

    def put(self, s, k, v):
        r = k[0] * R + s * SR
        self.ref[self.idx, r:r + SR, k[1] * Q:(k[1] + 1) * Q] = v

    def putb(self, k, v):
        self.ref[self.idx, k[0] * R:(k[0] + 1) * R, k[1] * Q:(k[1] + 1) * Q] = v


class ValArr:
    def __init__(self, blocks=None):
        self.parts = [dict() for _ in range(NS)]
        self.blocks = dict(blocks or {})

    def __getitem__(self, k):
        if k not in self.blocks:
            self.blocks[k] = jnp.concatenate([p[k] for p in self.parts], axis=0)
        return self.blocks[k]

    def get(self, s, k):
        if k not in self.parts[s]:
            self.parts[s][k] = self.blocks[k][s * SR:(s + 1) * SR]
        return self.parts[s][k]

    def put(self, s, k, v):
        self.parts[s][k] = v


class Sched:
    def __init__(self, never, opt):
        self.never, self.opt = never, opt
        self.q, self.bg, self.lock = [], [], None
        self.g, self.t, self.pace, self.bcredit = None, 0, 0.0, 0.0

    def gv(self, v):
        return v if self.g is None else jnp.where(self.never, self.g, v)

    def gc(self, c):
        return c if self.g is None else jnp.where(self.never, self.g, jnp.full((SR, Q), c, f32))

    def add(self, gen, deadline, cost, bg=False):
        (self.bg if bg else self.q).append([gen, deadline, cost])
        return gen

    def step(self, q, gate=None):
        self.g = gate
        c = None
        while q and c is None:
            c = next(q[0][0], None)
            if c is None:
                q.pop(0)
        if c is not None:
            self.lock = None if isinstance(c, float) else q
            q[0][2] -= c
        self.g = None
        return c

    def tick(self, val, base, brate):
        rate, cum = base, 0.0
        for _, dl, cost in self.q:
            cum += max(cost, 0)
            rate = max(rate, cum / max(dl - self.opt["margin"] - self.t, 1))
        self.bcredit = min(self.bcredit + brate + (0.0 if self.q else base), 40.0)
        self.pace = min(self.pace + rate + (brate if self.bg else 0.0), 40.0)
        if self.pace > 0:
            if self.lock:
                q = self.lock
            elif self.bg and (not self.q or (self.bcredit > 0 and rate <= base)):
                q = self.bg
            else:
                q = self.q
            if q:
                r = self.opt["row"]
                c = self.step(q, val[r * SR:(r + 1) * SR])
                if c:
                    self.pace -= c
                    if q is self.bg:
                        self.bcredit -= c
        self.t += 1

    def drain(self, gen=None, bg=False):
        q = self.bg if bg else self.q
        while q and (gen is None or any(e[0] is gen for e in q)):
            self.step(q)


def load_z(ref):
    z = []
    for o in range(4):
        zz = {}
        for k in IN:
            br, bc = rc(o, *k)
            zz[k] = ref[br * R:(br + 1) * R, bc * Q:(bc + 1) * Q].astype(f32)
        z.append(ValArr(zz))
    return z


def to_basis(dd, q, d, s, emit):
    r = phi3(dd)
    for p in range(4):
        d[(p, q)] = r[p]
        for (b, i, sg, j) in AFTER[q]:
            emit(s, (p, b), d[(p, i)], sg, d[(p, j)])


def head(S, z, H, dl):
    d1, d0 = ValArr(), ValArr()

    def e1(s, k, u, sg, v):
        d1.put(s, k, comb2(u, sg, v))

    def e0(s, k, u, sg, v):
        r = comb2(u, sg, v)
        d0.put(s, k, r)
        H[1].put(s, k, r - d1.get(s, k))
        H[2].put(s, k, r + d1.get(s, k))

    def e2(s, k, u, sg, v):
        H[3].put(s, k, comb2(u, sg, v, d1.get(s, k)))

    def e3(s, k, u, sg, v):
        H[0].put(s, k, comb2(u, sg, v, d0.get(s, k)))

    def tasks():
        for s in range(NS):
            for o, emit in ((1, e1), (2, e2), (0, e0), (3, e3)):
                d = {}
                for q in QORD:
                    v = []
                    for p in range(4):
                        sc = scale(*rc(o, p, q))
                        v.append(z[o].get(s, (p, q)) * sc if sc != 1.0 else z[o].get(s, (p, q)))
                    to_basis([S.gv(v[0])] + v[1:], q, d, s, emit)
                    yield 22.0 if q == QORD[-1] else 22

    return S.add(tasks(), dl, 16 * NS * 22)


def cross(S, dl, o, terms, z, bt_ref, l, emit=None, xo=None, out=None):
    last = emit is None
    qord = TORD if last else QORD
    post = {1: 23, 0: 13, 3: 13, 2: 13} if last else {q: (4 if o < 2 else 12) * len(AFTER[q]) for q in qord}
    cost = {q: 17 + 4 * len(terms) + post[q] for q in qord}

    def tasks():
        for s in range(NS):
            c = {k: chain([(sg, m.get(s, k)) for sg, m in terms]) for k in IN}
            d = {}
            yield 1
            yield 1
            if last:
                xi = {p: phi4_inv([xo.get(s, (p, q)) for q in range(4)]) for p in range(4)}
            for q in qord:
                cc = cost[q]
                y = psi([c[(p, q)] for p in range(4)], S.gc(0.5))
                if last:
                    cc = cost[q] // 2
                    yield cost[q] - cc
                    hf = S.gc(0.5)
                dd = []
                for p in range(4):
                    br, bc = rc(o, p, q)
                    dd.append((y[p] + bt_ref[l * 4 + popc(br), :, bc * Q:(bc + 1) * Q]) * z.get(s, (p, q)))
                if last:
                    e = [xi[p][q] for p in range(4)]
                    a11 = hf * (e[1] + e[2])
                    a22 = e[0] - a11
                    xn = [a11, e[2] - a11, ((e[3] - a22) + e[3]) - e[2], a22]
                    for p in range(4):
                        br, bc = rc(o, p, q)
                        r = dd[p] + xn[p]
                        if scale(br, bc) != 1.0:
                            r = r * (1.0 / scale(br, bc))
                        d[(p, q)] = r
                        if (p, q ^ 1) in d:
                            b0, r0 = bc & ~1, br * R + s * SR
                            pair = jnp.concatenate([d[(p, q & ~1)], d[(p, q | 1)]], axis=1)
                            out[r0:r0 + SR, b0 * Q:(b0 + 2) * Q] = pair.astype(bf16)
                else:
                    to_basis(dd, q, d, s, emit)
                yield float(cc) if q == qord[-1] else cc

    return S.add(tasks(), dl, NS * (2 + sum(cost.values())), bg=last)


def tail(S, z, bt_ref, out, ts_ref, L, quads=(0, 1, 2, 3)):
    for o in quads:
        g = cross(S, 0, o, [(sg, RefArr(ts_ref, 4 + NAMES.index(n))) for sg, n in TERMS[o]], z[o], bt_ref, L - 1,
                  xo=RefArr(ts_ref, o), out=out)
    return g


def unbasis1(S, X, ts_ref):
    for s in range(NS):
        for p in range(4):
            for q0 in (0, 2):
                hf = S.gc(0.5)
                for q in (q0, q0 + 1):
                    r = phi4_inv([X[b].get(s, (p, q)) for b in range(4)], hf)
                    for o in range(4):
                        RefArr(ts_ref, o).put(s, (p, q), r[o])
                yield S.opt["ic"]


def level3(mul, order):
    need = {"v": {1: 1, 3: 1, 5: -1}, "h": {3: 1, 5: 1}, 0: {"v": 1, 4: 1, 7: 1}, 3: {"v": 1, 6: 1, 2: -1},
            2: {"h": 1, 4: 1, 7: -1, 6: 1, 2: 1}}
    acc = {n: None for n in need}
    left = {n: set(t) for n, t in need.items()}
    for k in order:
        todo = [(k, mul(k))]
        while todo:
            name, v = todo.pop(0)
            for n, t in need.items():
                if name in left[n]:
                    left[n].discard(name)
                    acc[n] = sadd(acc[n], (t[name], v))
                    if not left[n]:
                        assert acc[n][0] > 0
                        if n == "h":
                            yield 1, acc[n][1]
                        if n in ("v", "h"):
                            todo.append((n, acc[n][1]))
                        else:
                            yield n, acc[n][1]


def level2(gen):
    out = {}
    c0 = dict(gen(1))
    for ja, jb, idx in ((4, 2, 2), (7, 6, 1), (5, 3, 3)):
        m = {}
        for q, c in gen(ja):
            m[q] = c
            c0[q] = c0[q] - c if ja == 5 else c + c0[q]
        for q, c in gen(jb):
            out[(idx, q)] = c - m[q] if jb == 6 else c + m[q]
    out.update({(0, q): c for q, c in c0.items()})
    return out


def body(x_prev, x_cur, x_next, out, bt_ref, t_ref, hs_ref, ts_ref, L, groups, never, opt):
    S = Sched(never, opt)
    cum = [0]
    for i in ORDER1:
        cum.append(cum[-1] + sum(8 if groups[(i, j)][1] else 7 for j in range(1, 8)))
    TL, mg = cum[-1], opt["margin"]
    zp, z, zn = load_z(x_prev), load_z(x_cur), load_z(x_next)
    X = [RefArr(hs_ref, b) for b in range(4)]
    pre = [10 * opt["pre"]]
    need = None
    tl = tail(S, zp, bt_ref, out, ts_ref, L)

    for l in range(L):
        T0 = l * TL
        last = l == L - 1

        def dot(u, n):
            w = pltpu.bitcast(t_ref[l, n // 2, :, (n % 2) * Q:(n % 2 + 1) * Q], bf16)
            return jnp.dot(u, w, preferred_element_type=f32)

        def level1(i):
            base = opt["rates%d" % l][ORDER1.index(i)]
            brate = opt.get("brates%d" % l, opt["brates"])[ORDER1.index(i)]

            def group(j):
                a = [lin([(s1 * s2, X[b1][(b2, q)]) for s1, b1 in CORE4[i] for s2, b2 in CORE3[j]])
                     for q in range(4)]
                n, plain = groups[(i, j)]
                if plain:
                    an = phi4_inv(a)
                    k0 = jnp.concatenate([an[0], an[2]], axis=0).astype(bf16)
                    k1 = jnp.concatenate([an[1], an[3]], axis=0).astype(bf16)

                    def mul2(u, k):
                        r = dot(u, n + k)
                        S.tick(r[:R], base, brate)
                        S.tick(r[R:], base, brate)
                        return r

                    c0 = mul2(k0, 0) + mul2(k1, 2)
                    c1 = mul2(k0, 1) + mul2(k1, 3)
                    return enumerate([c0[:R], c1[:R], c0[R:], c1[R:]])

                def mul(k):
                    u = lin([(s3, a[b]) for s3, b in CORE4[k]])
                    if len(CORE4[k]) == 2:
                        for r0 in (0, 2 * SR):
                            if pre[0] > 0:
                                S.step(S.bg, u[r0:r0 + SR])
                                pre[0] -= 1
                    r = dot(u.astype(bf16), n + k - 1)
                    S.tick(r, base, brate)
                    return r

                return level3(mul, opt.get("od%d" % l, opt["od"]))

            return level2(group)

        XN = [ValArr() for _ in range(4)]
        d12, d11 = ValArr(), ValArr()

        def emitter(o, X=X, XN=XN, d12=d12, d11=d11):
            def emit(s, k, u, sg, v):
                if o == 1:
                    d12.put(s, k, comb2(u, sg, v))
                elif o == 0:
                    e, r = d12.get(s, k), comb2(u, sg, v)
                    d11.put(s, k, r)
                    XN[1].put(s, k, (r + X[1].get(s, k)) - e)
                    XN[2].put(s, k, (r + X[2].get(s, k)) + e)
                elif o == 3:
                    XN[0].put(s, k, comb2(u, sg, v, X[0].get(s, k), d11.get(s, k)))
                else:
                    XN[3].put(s, k, comb2(u, sg, v, X[3].get(s, k), d12.get(s, k)))
            return emit

        M, nn = {}, {}

        def keep(name, m):
            M[name] = ValArr(m)
            if last:
                for k in IN:
                    RefArr(ts_ref, 4 + NAMES.index(name)).putb(k, m[k])

        def add(o, dl):
            if not last:
                nn[o] = cross(S, dl, o, [(sg, M[n]) for sg, n in TERMS[o]], z[o], bt_ref, l, emit=emitter(o))

        if last:
            S.drain(tl, bg=True)
        if need:
            S.drain(need[0])
        m3 = level1(3)
        m5 = level1(5)
        if last:
            S.add(unbasis1(S, X, ts_ref), T0 + TL + opt["endm"], NS * 8 * opt["ic"])
            head(S, zn, [RefArr(hs_ref, b) for b in range(4)], T0 + TL + opt["endm"])
        keep("h", {k: m5[k] + m3[k] for k in IN})
        v = {k: m3[k] - m5[k] for k in IN}
        add(1, T0 + cum[5] + mg)
        if need:
            S.drain(need[3])
        m1 = level1(1)
        keep("v", {k: m1[k] + v[k] for k in IN})
        keep("m4", level1(4))
        keep("m7", level1(7))
        add(0, T0 + TL)
        if need:
            S.drain(need[2])
        keep("m6", level1(6))
        keep("m2", level1(2))
        add(3, T0 + TL + cum[2])
        add(2, T0 + TL + cum[5])
        need, X = nn, XN
    S.drain()


def tform(e, k):
    if k == 1:
        return e[0] + e[0]
    return lin([(s, e[b]) for s, b in CORE4[SIGMA[k]]])


def table_basis(w_ref, e_ref):
    d = []
    for o in range(4):
        v, t, u = {}, {}, {}
        for k in IN:
            br, bc = rc(o, *k)
            v[k] = w_ref[br, :, bc * Q:(bc + 1) * Q].astype(f32) * (0.25 * scale(br, bc))
        for q in range(4):
            for p, x in enumerate(phi3([v[(p, q)] for p in range(4)])):
                t[(p, q)] = x
        for p in range(4):
            for q, x in enumerate(phi4([t[(p, q)] for q in range(4)])):
                u[(p, q)] = x
        d.append(u)
    for k in IN:
        for b, x in enumerate(phi4([d[o][k] for o in range(4)])):
            e_ref[b * 16 + k[0] * 4 + k[1]] = x


def table_tiles(e_ref, tb_ref, l, r, groups, i):
    s1 = {k: tform([e_ref[b * 16 + k[0] * 4 + k[1]] for b in range(4)], i) for k in IN}
    for j in range(1, 8):
        e = [lin([(sg, s1[(b, q)]) for sg, b in CORE3[SIGMA[j]]]) for q in range(4)]
        n, plain = groups[(i, j)]
        if plain:
            a, b = e[1] + e[2], e[2] - e[1]
            outs = [a, b, (e[3] - b) + e[3], (e[0] - a) + e[0]]
        else:
            outs = [tform(e, k) for k in range(1, 8)]
        for k, t in enumerate(outs):
            c0 = ((n + k) % 2) * Q
            tb_ref.at[l, (n + k) // 2][pl.ds(r, CR), c0:c0 + Q] = t.astype(bf16)


def kernel(x_hbm, w_hbm, b_hbm, o_hbm, t_ref, bt_ref, hs_ref, ts_ref, e_ref, w_buf, x_buf, o_buf, b_buf,
           w_sem, x_sem, o_sem, m_sem, *, L, nb, groups, opt):
    nc = L * NW

    def wcopy(c):
        slot = c & (NW - 1)
        return pltpu.make_async_copy(w_hbm.at[c >> 3, :, pl.ds(pl.multiple_of(slot * CR, CR), CR), :],
                                     w_buf.at[slot], w_sem.at[slot])

    def xcopy(i):
        return pltpu.make_async_copy(x_hbm.at[pl.ds(pl.multiple_of(i * TM, TM), TM), :],
                                     x_buf.at[i & (NX - 1)], x_sem.at[i & (NX - 1)])

    def ocopy(i):
        return pltpu.make_async_copy(o_buf.at[i & (NO - 1)], o_hbm.at[pl.ds(pl.multiple_of(i * TM, TM), TM), :],
                                     o_sem.at[i & (NO - 1)])

    bcopy = pltpu.make_async_copy(b_hbm, b_buf, m_sem.at[0])
    bcopy.start()
    xcopy(0).start()
    wcopy(0).start()
    ts_ref[...] = jnp.zeros(ts_ref.shape, f32)
    bcopy.wait()
    for c in range(1, NW):
        wcopy(c).start()
    for l in range(L):
        for e in range(4):
            for bc in range(8):
                row = b_buf[l:l + 1, bc * Q:(bc + 1) * Q].astype(f32) * (S3 ** (e - popc(bc)))
                bt_ref[l * 4 + e, :, bc * Q:(bc + 1) * Q] = jnp.broadcast_to(row, (SR, Q))
    xcopy(0).wait()
    S = Sched(None, opt)
    head(S, load_z(x_buf.at[0]), [RefArr(hs_ref, b) for b in range(4)], 0)
    S.drain()
    tb_ref = t_ref.bitcast(bf16)
    wcopy(0).wait()
    xcopy(1).start()

    def build(c, carry):
        slot = c & (NW - 1)

        def half(h, cc):
            rows = pl.ds(pl.multiple_of(h * SR, SR), SR)
            table_basis(w_buf.at[slot, :, rows, :], e_ref.at[0, :, rows, :])
            return cc

        jax.lax.fori_loop(0, CR // SR, half, 0)
        nxt, refill = wcopy(jnp.minimum(c + 1, nc - 1)), wcopy(jnp.minimum(c + NW, nc - 1))
        for i in range(1, 8):
            table_tiles(e_ref.at[(c + i) >> 10], tb_ref, c >> 3, pl.multiple_of(slot * CR, CR), groups, i)
        pl.when(c + NW < nc)(refill.start)
        pl.when(c + 1 < nc)(nxt.wait)
        return carry

    jax.lax.fori_loop(0, nc, build, 0)

    def dmas(i):
        cps = [xcopy(jnp.minimum(i + 2, nb - 1)), ocopy(jnp.maximum(i - 2, 0)),
               xcopy(jnp.minimum(i + 1, nb - 1)), ocopy(jnp.maximum(i - 3, 0))]
        pl.when(i + 2 < nb)(cps[0].start)
        pl.when(i >= 2)(cps[1].start)
        pl.when(i + 1 < nb)(cps[2].wait)
        pl.when(i >= 3)(cps[3].wait)

    def step(i, carry):
        never = jnp.full((SR, Q), i, jnp.int32) < 0
        xs = [x_buf.at[jnp.clip(i + u, 0, nb - 1) & (NX - 1)] for u in (-1, 0, 1)]
        body(*xs, o_buf.at[(i + 1) & (NO - 1)], bt_ref, t_ref, hs_ref, ts_ref, L, groups, never, opt)
        dmas(i + 1)
        return carry

    dmas(jnp.int32(0))
    jax.lax.fori_loop(0, nb, step, 0)

    last, H = nb - 1, TM // 2
    z = load_z(x_buf.at[last % NX])
    halves = [pltpu.make_async_copy(o_buf.at[last % NO, pl.ds(h * H, H), :],
                                    o_hbm.at[pl.ds(last * TM + h * H, H), :], m_sem.at[1 + h]) for h in range(2)]
    for h in range(2):
        S = Sched(None, opt)
        tail(S, z, bt_ref, o_buf.at[last % NO], ts_ref, L, (2 * h, 2 * h + 1))
        S.drain(bg=True)
        halves[h].start()
    ocopy(last - 1).wait()
    for h in range(2):
        halves[h].wait()


def make(o=None):
    opt = dict(OPT)
    opt.update(o or {})
    groups, n = plan()

    @jax.jit
    def run(x0, ws, bs):
        B, D = x0.shape
        L = ws.shape[0]
        assert D == 8 * Q and B % TM == 0 and B >= 2 * TM and L == 6 and n % 2 == 0
        return pl.pallas_call(
            functools.partial(kernel, L=L, nb=B // TM, groups=groups, opt=opt),
            in_specs=[pl.BlockSpec(memory_space=pl.ANY)] * 3,
            out_specs=pl.BlockSpec(memory_space=pl.ANY),
            out_shape=jax.ShapeDtypeStruct((B, D), x0.dtype),
            scratch_shapes=[
                pltpu.VMEM((L, n // 2, Q // 2, 2 * Q), jnp.uint32),
                pltpu.VMEM((L * 4, SR, D), f32),
                pltpu.VMEM((4, 4 * R, D // 2), f32),
                pltpu.VMEM((10, 4 * R, D // 2), f32),
                pltpu.VMEM((2, 64, CR, Q), f32),
                pltpu.VMEM((NW, 8, CR, D), bf16),
                pltpu.VMEM((NX, TM, D), bf16),
                pltpu.VMEM((NO, TM, D), bf16),
                pltpu.VMEM((L, D), bf16),
                pltpu.SemaphoreType.DMA((NW,)),
                pltpu.SemaphoreType.DMA((NX,)),
                pltpu.SemaphoreType.DMA((NO,)),
                pltpu.SemaphoreType.DMA((3,)),
            ],
            compiler_params=pltpu.CompilerParams(vmem_limit_bytes=100 * 1024 * 1024, disable_bounds_checks=True),
        )(x0, ws.reshape(L, 8, Q, D), bs)

    return run


_run = make()


@jax.jit
def pallas_standalone__dcn_v2_cross__recsys_kernel(x0: jax.Array, ws: jax.Array, bs: jax.Array):
    return _run(x0, ws, bs)
```

```python
import functools
import math

import jax
import jax.numpy as jnp
import jax.experimental.pallas as pl
import jax.experimental.pallas.tpu as pltpu

f32 = jnp.float32
bf16 = jnp.bfloat16

Q = 128
R = 32
SR = 8
NS = R // SR
TM = 8 * R
CR = 16
NW = Q // CR
NX = 4
NO = 2
S3 = math.sqrt(3.0)
IN = [(p, q) for p in range(4) for q in range(4)]

CORE3 = {1: [(1, 0)], 3: [(1, 1)], 5: [(1, 2)], 2: [(1, 3)],
         4: [(1, 0), (-1, 1)], 7: [(1, 2), (-1, 0)], 6: [(1, 3), (-1, 0)]}
CORE4 = {1: [(1, 0)], 3: [(1, 1)], 5: [(1, 2)], 2: [(1, 3), (1, 0)],
         4: [(1, 0), (-1, 1)], 7: [(1, 2), (-1, 0)], 6: [(1, 3), (-1, 0)]}
SIGMA = {1: 1, 2: 3, 3: 7, 4: 6, 5: 4, 6: 5, 7: 2}
ORDER1 = [3, 5, 1, 4, 7, 6, 2]
QORD = [2, 1, 0, 3]
TORD = [1, 0, 3, 2]
AFTER = {2: [], 1: [(3, 1, 1, 2)], 0: [(1, 0, -1, 1), (2, 0, 1, 1)], 3: [(0, 3, 1, 0)]}
NAMES = ["h", "v", "m4", "m7", "m6", "m2"]
TERMS = {1: [(1, "h")], 0: [(1, "m7"), (1, "v"), (1, "m4")], 3: [(1, "v"), (-1, "m2"), (1, "m6")],
         2: [(1, "m2"), (1, "m6"), (1, "h"), (1, "m4"), (-1, "m7")]}

OPT = dict(
    pres=8, row=2, margin=27, pre=2, ic=18.0, endm=25,
    rates0=[9.2, 9.4, 10, 6, 6.8, 5.5, 5.4], rates1=[9.2, 7, 11.5, 5.5, 5.5, 5.5, 5.4],
    rates2=[9.2, 7, 11.5, 4.8, 4.2, 5.5, 5.4], rates3=[9.2, 7, 11.5, 5.5, 6.7, 5.5, 5.4],
    rates4=[9.2, 7, 11.5, 5.5, 5.5, 5.5, 5.3], rates5=[9.2, 7, 12.4, 4.3, 5.5, 5.5, 5.4],
    brates=[2.0] * 7, brates0=[2.0, 2.3, 1.0, 2.0, 3.0, 2.0, 3.0], brates1=[2.1, 2.0, 2.0, 2.0, 2.0, 2.0, 2.0],
    od=[3, 4, 5, 1, 7, 6, 2], od3=[3, 4, 1, 5, 7, 2, 6], od4=[3, 4, 1, 5, 7, 2, 6], od5=[3, 4, 5, 1, 7, 2, 6])


def lin(terms):
    pos = [v for s, v in terms if s > 0]
    neg = [v for s, v in terms if s < 0]
    acc = pos[0]
    for v in pos[1:]:
        acc = acc + v
    for v in neg:
        acc = acc - v
    return acc


def chain(terms):
    acc = terms[0][1]
    for s, v in terms[1:]:
        acc = acc + v if s > 0 else acc - v
    return acc


def sadd(a, b):
    if a is None:
        return b
    if a[0] == b[0]:
        return (a[0], b[1] + a[1])
    return (1, a[1] - b[1]) if a[0] > 0 else (1, b[1] - a[1])


def comb2(u, sg, v, x=None, e=None):
    if x is not None:
        u = u + x
    if e is not None:
        v = v + e if sg > 0 else v - e
    return u + v if sg > 0 else u - v


def phi3(a):
    l5 = a[0] + a[1]
    return [a[0] + a[3], a[0] - a[1], l5, 0.5 * (l5 + a[3] + a[2])]


def phi4(a):
    return [a[0] + a[3], a[0] - a[1], a[0] + a[1], a[1] + a[2]]


def phi4_inv(e, hf=0.5):
    a11 = hf * (e[1] + e[2])
    a12 = e[2] - a11
    return [a11, a12, e[3] - a12, e[0] - a11]


def psi(c, hf):
    h = hf * c[3]
    c11 = h + c[0]
    return [c11, h, (h + c[1]) + c[2], (c11 + c[1]) - c[2]]


def rc(o, p, q):
    return (o // 2) * 4 + (p // 2) * 2 + q // 2, (o % 2) * 4 + (p % 2) * 2 + q % 2


def popc(v):
    return bin(v).count("1")


def scale(br, bc):
    return S3 ** (popc(br) - popc(bc))


def plan():
    groups, n = {}, 0
    for i in range(1, 8):
        for j in range(1, 8):
            plain = i == 1 or j == 1
            groups[(i, j)] = (n, plain)
            n += 4 if plain else 7
    return groups, n


class RefArr:
    def __init__(self, ref, idx):
        self.ref, self.idx = ref, idx

    def __getitem__(self, k):
        return self.ref[self.idx, k[0] * R:(k[0] + 1) * R, k[1] * Q:(k[1] + 1) * Q]

    def get(self, s, k):
        r = k[0] * R + s * SR
        return self.ref[self.idx, r:r + SR, k[1] * Q:(k[1] + 1) * Q]

    def put(self, s, k, v):
        r = k[0] * R + s * SR
        self.ref[self.idx, r:r + SR, k[1] * Q:(k[1] + 1) * Q] = v

    def putb(self, k, v):
        self.ref[self.idx, k[0] * R:(k[0] + 1) * R, k[1] * Q:(k[1] + 1) * Q] = v


class ValArr:
    def __init__(self, blocks=None):
        self.parts = [dict() for _ in range(NS)]
        self.blocks = dict(blocks or {})

    def __getitem__(self, k):
        if k not in self.blocks:
            self.blocks[k] = jnp.concatenate([p[k] for p in self.parts], axis=0)
        return self.blocks[k]

    def get(self, s, k):
        if k not in self.parts[s]:
            self.parts[s][k] = self.blocks[k][s * SR:(s + 1) * SR]
        return self.parts[s][k]

    def put(self, s, k, v):
        self.parts[s][k] = v


class Sched:
    def __init__(self, never, opt):
        self.never, self.opt = never, opt
        self.q, self.bg, self.lock = [], [], None
        self.g, self.t, self.pace, self.bcredit = None, 0, 0.0, 0.0

    def gv(self, v):
        return v if self.g is None else jnp.where(self.never, self.g, v)

    def gc(self, c):
        return c if self.g is None else jnp.where(self.never, self.g, jnp.full((SR, Q), c, f32))

    def add(self, gen, deadline, cost, bg=False):
        (self.bg if bg else self.q).append([gen, deadline, cost])
        return gen

    def step(self, q, gate=None):
        self.g = gate
        c = None
        while q and c is None:
            c = next(q[0][0], None)
            if c is None:
                q.pop(0)
        if c is not None:
            self.lock = None if isinstance(c, float) else q
            q[0][2] -= c
        self.g = None
        return c

    def tick(self, val, base, brate):
        rate, cum = base, 0.0
        for _, dl, cost in self.q:
            cum += max(cost, 0)
            rate = max(rate, cum / max(dl - self.opt["margin"] - self.t, 1))
        self.bcredit = min(self.bcredit + brate + (0.0 if self.q else base), 40.0)
        self.pace = min(self.pace + rate + (brate if self.bg else 0.0), 40.0)
        if self.pace > 0:
            if self.lock:
                q = self.lock
            elif self.bg and (not self.q or (self.bcredit > 0 and rate <= base)):
                q = self.bg
            else:
                q = self.q
            if q:
                r = self.opt["row"]
                c = self.step(q, val[r * SR:(r + 1) * SR])
                if c:
                    self.pace -= c
                    if q is self.bg:
                        self.bcredit -= c
        self.t += 1

    def drain(self, gen=None, bg=False):
        q = self.bg if bg else self.q
        while q and (gen is None or any(e[0] is gen for e in q)):
            self.step(q)


def load_z(ref):
    z = []
    for o in range(4):
        zz = {}
        for k in IN:
            br, bc = rc(o, *k)
            zz[k] = ref[br * R:(br + 1) * R, bc * Q:(bc + 1) * Q].astype(f32)
        z.append(ValArr(zz))
    return z


def to_basis(dd, q, d, s, emit):
    r = phi3(dd)
    for p in range(4):
        d[(p, q)] = r[p]
        for (b, i, sg, j) in AFTER[q]:
            emit(s, (p, b), d[(p, i)], sg, d[(p, j)])


def head(S, z, H, dl):
    d1, d0 = ValArr(), ValArr()

    def e1(s, k, u, sg, v):
        d1.put(s, k, comb2(u, sg, v))

    def e0(s, k, u, sg, v):
        r = comb2(u, sg, v)
        d0.put(s, k, r)
        H[1].put(s, k, r - d1.get(s, k))
        H[2].put(s, k, r + d1.get(s, k))

    def e2(s, k, u, sg, v):
        H[3].put(s, k, comb2(u, sg, v, d1.get(s, k)))

    def e3(s, k, u, sg, v):
        H[0].put(s, k, comb2(u, sg, v, d0.get(s, k)))

    def tasks():
        for s in range(NS):
            for o, emit in ((1, e1), (2, e2), (0, e0), (3, e3)):
                d = {}
                for q in QORD:
                    v = []
                    for p in range(4):
                        sc = scale(*rc(o, p, q))
                        v.append(z[o].get(s, (p, q)) * sc if sc != 1.0 else z[o].get(s, (p, q)))
                    to_basis([S.gv(v[0])] + v[1:], q, d, s, emit)
                    yield 22.0 if q == QORD[-1] else 22

    return S.add(tasks(), dl, 16 * NS * 22)


def cross(S, dl, o, terms, z, bt_ref, l, emit=None, xo=None, out=None):
    last = emit is None
    qord = TORD if last else QORD
    post = {1: 23, 0: 13, 3: 13, 2: 13} if last else {q: (4 if o < 2 else 12) * len(AFTER[q]) for q in qord}
    cost = {q: 17 + 4 * len(terms) + post[q] for q in qord}

    def tasks():
        for s in range(NS):
            c = {k: chain([(sg, m.get(s, k)) for sg, m in terms]) for k in IN}
            d = {}
            yield 1
            yield 1
            if last:
                xi = {p: phi4_inv([xo.get(s, (p, q)) for q in range(4)]) for p in range(4)}
            for q in qord:
                cc = cost[q]
                y = psi([c[(p, q)] for p in range(4)], S.gc(0.5))
                if last:
                    cc = cost[q] // 2
                    yield cost[q] - cc
                    hf = S.gc(0.5)
                dd = []
                for p in range(4):
                    br, bc = rc(o, p, q)
                    dd.append((y[p] + bt_ref[l * 4 + popc(br), :, bc * Q:(bc + 1) * Q]) * z.get(s, (p, q)))
                if last:
                    e = [xi[p][q] for p in range(4)]
                    a11 = hf * (e[1] + e[2])
                    a22 = e[0] - a11
                    xn = [a11, e[2] - a11, ((e[3] - a22) + e[3]) - e[2], a22]
                    for p in range(4):
                        br, bc = rc(o, p, q)
                        r = dd[p] + xn[p]
                        if scale(br, bc) != 1.0:
                            r = r * (1.0 / scale(br, bc))
                        d[(p, q)] = r
                        if (p, q ^ 1) in d:
                            b0, r0 = bc & ~1, br * R + s * SR
                            pair = jnp.concatenate([d[(p, q & ~1)], d[(p, q | 1)]], axis=1)
                            out[r0:r0 + SR, b0 * Q:(b0 + 2) * Q] = pair.astype(bf16)
                else:
                    to_basis(dd, q, d, s, emit)
                yield float(cc) if q == qord[-1] else cc

    return S.add(tasks(), dl, NS * (2 + sum(cost.values())), bg=last)


def tail(S, z, bt_ref, out, ts_ref, L, quads=(0, 1, 2, 3)):
    for o in quads:
        g = cross(S, 0, o, [(sg, RefArr(ts_ref, 4 + NAMES.index(n))) for sg, n in TERMS[o]], z[o], bt_ref, L - 1,
                  xo=RefArr(ts_ref, o), out=out)
    return g


def unbasis1(S, X, ts_ref):
    for s in range(NS):
        for p in range(4):
            for q0 in (0, 2):
                hf = S.gc(0.5)
                for q in (q0, q0 + 1):
                    r = phi4_inv([X[b].get(s, (p, q)) for b in range(4)], hf)
                    for o in range(4):
                        RefArr(ts_ref, o).put(s, (p, q), r[o])
                yield S.opt["ic"]


def level3(mul, order):
    need = {"v": {1: 1, 3: 1, 5: -1}, "h": {3: 1, 5: 1}, 0: {"v": 1, 4: 1, 7: 1}, 3: {"v": 1, 6: 1, 2: -1},
            2: {"h": 1, 4: 1, 7: -1, 6: 1, 2: 1}}
    acc = {n: None for n in need}
    left = {n: set(t) for n, t in need.items()}
    for k in order:
        todo = [(k, mul(k))]
        while todo:
            name, v = todo.pop(0)
            for n, t in need.items():
                if name in left[n]:
                    left[n].discard(name)
                    acc[n] = sadd(acc[n], (t[name], v))
                    if not left[n]:
                        assert acc[n][0] > 0
                        if n == "h":
                            yield 1, acc[n][1]
                        if n in ("v", "h"):
                            todo.append((n, acc[n][1]))
                        else:
                            yield n, acc[n][1]


def level2(gen):
    out = {}
    c0 = dict(gen(1))
    for ja, jb, idx in ((4, 2, 2), (7, 6, 1), (5, 3, 3)):
        m = {}
        for q, c in gen(ja):
            m[q] = c
            c0[q] = c0[q] - c if ja == 5 else c + c0[q]
        for q, c in gen(jb):
            out[(idx, q)] = c - m[q] if jb == 6 else c + m[q]
    out.update({(0, q): c for q, c in c0.items()})
    return out


def body(x_prev, x_cur, x_next, out, bt_ref, t_ref, hs_ref, ts_ref, L, groups, never, opt):
    S = Sched(never, opt)
    cum = [0]
    for i in ORDER1:
        cum.append(cum[-1] + sum(8 if groups[(i, j)][1] else 7 for j in range(1, 8)))
    TL, mg = cum[-1], opt["margin"]
    zp, z, zn = load_z(x_prev), load_z(x_cur), load_z(x_next)
    X = [RefArr(hs_ref, b) for b in range(4)]
    pre = [10 * opt["pre"]]
    need = None
    tl = tail(S, zp, bt_ref, out, ts_ref, L)

    for l in range(L):
        T0 = l * TL
        last = l == L - 1

        def dot(u, n):
            w = pltpu.bitcast(t_ref[l, n // 2, :, (n % 2) * Q:(n % 2 + 1) * Q], bf16)
            return jnp.dot(u, w, preferred_element_type=f32)

        def level1(i):
            base = opt["rates%d" % l][ORDER1.index(i)]
            brate = opt.get("brates%d" % l, opt["brates"])[ORDER1.index(i)]

            def group(j):
                a = [lin([(s1 * s2, X[b1][(b2, q)]) for s1, b1 in CORE4[i] for s2, b2 in CORE3[j]])
                     for q in range(4)]
                n, plain = groups[(i, j)]
                if plain:
                    an = phi4_inv(a)
                    k0 = jnp.concatenate([an[0], an[2]], axis=0).astype(bf16)
                    k1 = jnp.concatenate([an[1], an[3]], axis=0).astype(bf16)

                    def mul2(u, k):
                        r = dot(u, n + k)
                        S.tick(r[:R], base, brate)
                        S.tick(r[R:], base, brate)
                        return r

                    c0 = mul2(k0, 0) + mul2(k1, 2)
                    c1 = mul2(k0, 1) + mul2(k1, 3)
                    return enumerate([c0[:R], c1[:R], c0[R:], c1[R:]])

                def mul(k):
                    u = lin([(s3, a[b]) for s3, b in CORE4[k]])
                    if len(CORE4[k]) == 2:
                        for r0 in (0, 2 * SR):
                            if pre[0] > 0:
                                S.step(S.bg, u[r0:r0 + SR])
                                pre[0] -= 1
                    r = dot(u.astype(bf16), n + k - 1)
                    S.tick(r, base, brate)
                    return r

                return level3(mul, opt.get("od%d" % l, opt["od"]))

            return level2(group)

        XN = [ValArr() for _ in range(4)]
        d12, d11 = ValArr(), ValArr()

        def emitter(o, X=X, XN=XN, d12=d12, d11=d11):
            def emit(s, k, u, sg, v):
                if o == 1:
                    d12.put(s, k, comb2(u, sg, v))
                elif o == 0:
                    e, r = d12.get(s, k), comb2(u, sg, v)
                    d11.put(s, k, r)
                    XN[1].put(s, k, (r + X[1].get(s, k)) - e)
                    XN[2].put(s, k, (r + X[2].get(s, k)) + e)
                elif o == 3:
                    XN[0].put(s, k, comb2(u, sg, v, X[0].get(s, k), d11.get(s, k)))
                else:
                    XN[3].put(s, k, comb2(u, sg, v, X[3].get(s, k), d12.get(s, k)))
            return emit

        M, nn = {}, {}

        def keep(name, m):
            M[name] = ValArr(m)
            if last:
                for k in IN:
                    RefArr(ts_ref, 4 + NAMES.index(name)).putb(k, m[k])

        def add(o, dl):
            if not last:
                nn[o] = cross(S, dl, o, [(sg, M[n]) for sg, n in TERMS[o]], z[o], bt_ref, l, emit=emitter(o))

        if last:
            S.drain(tl, bg=True)
        if need:
            S.drain(need[0])
        m3 = level1(3)
        m5 = level1(5)
        if last:
            S.add(unbasis1(S, X, ts_ref), T0 + TL + opt["endm"], NS * 8 * opt["ic"])
            head(S, zn, [RefArr(hs_ref, b) for b in range(4)], T0 + TL + opt["endm"])
        keep("h", {k: m5[k] + m3[k] for k in IN})
        v = {k: m3[k] - m5[k] for k in IN}
        add(1, T0 + cum[5] + mg)
        if need:
            S.drain(need[3])
        m1 = level1(1)
        keep("v", {k: m1[k] + v[k] for k in IN})
        keep("m4", level1(4))
        keep("m7", level1(7))
        add(0, T0 + TL)
        if need:
            S.drain(need[2])
        keep("m6", level1(6))
        keep("m2", level1(2))
        add(3, T0 + TL + cum[2])
        add(2, T0 + TL + cum[5])
        need, X = nn, XN
    S.drain()


def tform(e, k):
    if k == 1:
        return e[0] + e[0]
    return lin([(s, e[b]) for s, b in CORE4[SIGMA[k]]])


def table_tasks(S, w_ref, tb_ref, l, groups):
    for c in range(Q // CR):
        E = []
        for r0 in range(c * CR, (c + 1) * CR, SR):
            H, d1, d0 = [{} for _ in range(4)], {}, {}
            for o in (1, 2, 0, 3):
                def emit(s, k, u, sg, v):
                    if o == 1:
                        d1[k] = comb2(u, sg, v)
                    elif o == 2:
                        H[3][k] = comb2(u, sg, v, d1[k])
                    elif o == 0:
                        d0[k] = comb2(u, sg, v)
                        H[1][k], H[2][k] = d0[k] - d1[k], d0[k] + d1[k]
                    else:
                        H[0][k] = comb2(u, sg, v, d0[k])

                d = {}
                for q in QORD:
                    v = []
                    for p in range(4):
                        br, bc = rc(o, p, q)
                        sc = 0.25 * scale(br, bc)
                        v.append(w_ref[br, r0:r0 + SR, bc * Q:(bc + 1) * Q].astype(f32) * (S.gc(sc) if p == 0 else sc))
                    to_basis(v, q, d, 0, emit)
                    yield 23
            E.append(H)
        for i in range(1, 8):
            s1, first = {}, CORE4[SIGMA[i]][0][1]
            for b2 in range(4):
                for q in range(4):
                    s1[(b2, q)] = jnp.concatenate(
                        [tform([S.gv(H[b][(b2, q)]) if b == first else H[b][(b2, q)] for b in range(4)], i) for H in E],
                        axis=0)
                js = [j for j in range(1, 8) if max(b for _, b in CORE3[SIGMA[j]]) == b2]
                for j in js:
                    e = [lin([(sg, s1[(b, q)]) for sg, b in CORE3[SIGMA[j]]]) for q in range(4)]
                    n, plain = groups[(i, j)]
                    if plain:
                        a, b = e[1] + e[2], e[2] - e[1]
                        outs = [a, b, (e[3] - b) + e[3], (e[0] - a) + e[0]]
                    else:
                        outs = [tform(e, k) for k in range(1, 8)]
                    for k, t in enumerate(outs):
                        c0 = ((n + k) % 2) * Q
                        tb_ref.at[l, (n + k) // 2][c * CR:(c + 1) * CR, c0:c0 + Q] = t.astype(bf16)
                yield 16 + 21 * len(js)


def first_layer(l, w_ref, x0_ref, xi_ref, xo_ref, bt_ref, tb_ref, groups, opt):
    S = Sched(jnp.full((SR, Q), l, jnp.int32) < 0, opt)
    S.add(table_tasks(S, w_ref, tb_ref, l, groups), 0, 0)
    rate = (Q // CR) * (32 * 23 + 7 * (4 * 16 + 7 * 21)) / (16 * TM // SR - opt["pres"])
    pace = 0.0
    x = xi_ref[...]
    xb = x.astype(bf16)
    for n in range(8):
        cs = slice(n * Q, (n + 1) * Q)
        acc = None
        for kh in range(2):
            rs = [jnp.dot(xb[:, k * Q:(k + 1) * Q], w_ref[k, :, cs], preferred_element_type=f32)
                  for k in range(4 * kh, 4 * kh + 4)]
            oth = (rs[1] + rs[2]) + rs[3]
            acc = oth if acc is None else acc + oth
            for g in range(TM // SR):
                pace += rate
                if pace > 0:
                    pace -= S.step(S.q, rs[0][g * SR:(g + 1) * SR]) or 0
            acc = acc + rs[0]
        xo_ref[:, cs] = x0_ref[:, cs].astype(f32) * (acc + bt_ref[l * 4 + popc(n), 0:1, cs]) + x[:, cs]
    S.drain()


def kernel(x_hbm, w_hbm, b_hbm, o_hbm, t_ref, bt_ref, hs_ref, ts_ref, xs_ref, w_buf, x_buf, o_buf, o0_buf, b_buf,
           w_sem, x_sem, o_sem, m_sem, *, L, nb, groups, opt):
    def wcopy(l):
        return pltpu.make_async_copy(w_hbm.at[l], w_buf.at[l & 1], w_sem.at[l & 1])

    def xcopy(i):
        return pltpu.make_async_copy(x_hbm.at[pl.ds(pl.multiple_of(i * TM, TM), TM), :],
                                     x_buf.at[i & (NX - 1)], x_sem.at[i & (NX - 1)])

    def ocopy(i):
        return pltpu.make_async_copy(o_buf.at[i & (NO - 1)], o_hbm.at[pl.ds(pl.multiple_of(i * TM, TM), TM), :],
                                     o_sem.at[i & (NO - 1)])

    bcopy = pltpu.make_async_copy(b_hbm, b_buf, m_sem.at[0])
    bcopy.start()
    xcopy(0).start()
    wcopy(0).start()
    ts_ref[...] = jnp.zeros(ts_ref.shape, f32)
    bcopy.wait()
    for l in range(L):
        for e in range(4):
            for bc in range(8):
                row = b_buf[l:l + 1, bc * Q:(bc + 1) * Q].astype(f32) * (S3 ** (e - popc(bc)))
                bt_ref[l * 4 + e, :, bc * Q:(bc + 1) * Q] = jnp.broadcast_to(row, (SR, Q))
    xcopy(0).wait()
    xs_ref[0] = x_buf[0].astype(f32)
    tb_ref = t_ref.bitcast(bf16)
    wcopy(0).wait()

    def first(l, carry):
        nxt = wcopy(jnp.minimum(l + 1, L - 1))
        pl.when(l + 1 < L)(nxt.start)

        @pl.when(l + 1 == L)
        def _():
            xcopy(1).start()
            xcopy(2).start()

        first_layer(l, w_buf.at[l & 1], x_buf.at[0], xs_ref.at[l & 1], xs_ref.at[1 - (l & 1)], bt_ref, tb_ref,
                    groups, opt)
        pl.when(l + 1 < L)(nxt.wait)
        return carry

    jax.lax.fori_loop(0, L, first, 0)
    o0_buf[...] = xs_ref[L % 2].astype(bf16)
    o0copy = pltpu.make_async_copy(o0_buf, o_hbm.at[pl.ds(0, TM), :], m_sem.at[3])
    o0copy.start()
    xcopy(1).wait()
    S = Sched(None, opt)
    head(S, load_z(x_buf.at[1]), [RefArr(hs_ref, b) for b in range(4)], 0)
    S.drain()

    def dmas(i):
        cps = [xcopy(jnp.minimum(i + 2, nb - 1)), ocopy(jnp.maximum(i - 2, 1)),
               xcopy(jnp.minimum(i + 1, nb - 1)), ocopy(jnp.maximum(i - 3, 1))]
        pl.when(i + 2 < nb)(cps[0].start)
        pl.when(i >= 3)(cps[1].start)
        pl.when(i + 1 < nb)(cps[2].wait)
        pl.when(i >= 4)(cps[3].wait)

    def step(i, carry):
        never = jnp.full((SR, Q), i, jnp.int32) < 0
        xs = [x_buf.at[jnp.clip(i + u, 0, nb - 1) & (NX - 1)] for u in (-1, 0, 1)]
        body(*xs, o_buf.at[(i + 1) & (NO - 1)], bt_ref, t_ref, hs_ref, ts_ref, L, groups, never, opt)
        dmas(i + 1)
        return carry

    dmas(jnp.int32(1))
    jax.lax.fori_loop(1, nb, step, 0)

    last, H = nb - 1, TM // 2
    z = load_z(x_buf.at[last % NX])
    halves = [pltpu.make_async_copy(o_buf.at[last % NO, pl.ds(h * H, H), :],
                                    o_hbm.at[pl.ds(last * TM + h * H, H), :], m_sem.at[1 + h]) for h in range(2)]
    for h in range(2):
        S = Sched(None, opt)
        tail(S, z, bt_ref, o_buf.at[last % NO], ts_ref, L, (2 * h, 2 * h + 1))
        S.drain(bg=True)
        halves[h].start()
    o0copy.wait()
    ocopy(last - 1).wait()
    for h in range(2):
        halves[h].wait()


def make(o=None):
    opt = dict(OPT)
    opt.update(o or {})
    groups, n = plan()

    @jax.jit
    def run(x0, ws, bs):
        B, D = x0.shape
        L = ws.shape[0]
        assert D == 8 * Q and B % TM == 0 and B >= 3 * TM and L == 6 and n % 2 == 0
        return pl.pallas_call(
            functools.partial(kernel, L=L, nb=B // TM, groups=groups, opt=opt),
            in_specs=[pl.BlockSpec(memory_space=pl.ANY)] * 3,
            out_specs=pl.BlockSpec(memory_space=pl.ANY),
            out_shape=jax.ShapeDtypeStruct((B, D), x0.dtype),
            scratch_shapes=[
                pltpu.VMEM((L, n // 2, Q // 2, 2 * Q), jnp.uint32),
                pltpu.VMEM((L * 4, SR, D), f32),
                pltpu.VMEM((4, 4 * R, D // 2), f32),
                pltpu.VMEM((10, 4 * R, D // 2), f32),
                pltpu.VMEM((2, TM, D), f32),
                pltpu.VMEM((2, 8, Q, D), bf16),
                pltpu.VMEM((NX, TM, D), bf16),
                pltpu.VMEM((NO, TM, D), bf16),
                pltpu.VMEM((TM, D), bf16),
                pltpu.VMEM((L, D), bf16),
                pltpu.SemaphoreType.DMA((2,)),
                pltpu.SemaphoreType.DMA((NX,)),
                pltpu.SemaphoreType.DMA((NO,)),
                pltpu.SemaphoreType.DMA((4,)),
            ],
            compiler_params=pltpu.CompilerParams(vmem_limit_bytes=100 * 1024 * 1024, disable_bounds_checks=True),
        )(x0, ws.reshape(L, 8, Q, D), bs)

    return run


_run = make()


@jax.jit
def pallas_standalone__dcn_v2_cross__recsys_kernel(x0: jax.Array, ws: jax.Array, bs: jax.Array):
    return _run(x0, ws, bs)
```

```python
import functools
import math

import jax
import jax.numpy as jnp
import jax.experimental.pallas as pl
import jax.experimental.pallas.tpu as pltpu

f32 = jnp.float32
bf16 = jnp.bfloat16

Q = 128
R = 32
SR = 8
NS = R // SR
TM = 8 * R
CR = 16
NX = 4
NO = 2
S3 = math.sqrt(3.0)
IN = [(p, q) for p in range(4) for q in range(4)]

CORE3 = {1: [(1, 0)], 3: [(1, 1)], 5: [(1, 2)], 2: [(1, 3)],
         4: [(1, 0), (-1, 1)], 7: [(1, 2), (-1, 0)], 6: [(1, 3), (-1, 0)]}
CORE4 = {1: [(1, 0)], 3: [(1, 1)], 5: [(1, 2)], 2: [(1, 3), (1, 0)],
         4: [(1, 0), (-1, 1)], 7: [(1, 2), (-1, 0)], 6: [(1, 3), (-1, 0)]}
SIGMA = {1: 1, 2: 3, 3: 7, 4: 6, 5: 4, 6: 5, 7: 2}
ORDER1 = [3, 5, 1, 4, 7, 6, 2]
QORD = [2, 1, 0, 3]
TORD = [1, 0, 3, 2]
AFTER = {2: [], 1: [(3, 1, 1, 2)], 0: [(1, 0, -1, 1), (2, 0, 1, 1)], 3: [(0, 3, 1, 0)]}
NAMES = ["h", "v", "m4", "m7", "m6", "m2"]
TERMS = {1: [(1, "h")], 0: [(1, "m7"), (1, "v"), (1, "m4")], 3: [(1, "v"), (-1, "m2"), (1, "m6")],
         2: [(1, "m2"), (1, "m6"), (1, "h"), (1, "m4"), (-1, "m7")]}

OPT = dict(
    row=2, margin=27, pre=2, ic=18.0, endm=25,
    rates0=[9.2, 9.4, 10, 6, 6.8, 5.5, 5.4], rates1=[9.2, 7, 11.5, 5.5, 5.5, 5.5, 5.4],
    rates2=[9.2, 7, 11.5, 4.8, 4.2, 5.5, 5.4], rates3=[9.2, 7, 11.5, 5.5, 6.7, 5.5, 5.4],
    rates4=[9.2, 7, 11.5, 5.5, 5.5, 5.5, 5.3], rates5=[9.2, 7, 12.4, 4.3, 5.5, 5.5, 5.4],
    brates=[2.0] * 7, brates0=[2.0, 2.3, 1.0, 2.0, 3.0, 2.0, 3.0], brates1=[2.1, 2.0, 2.0, 2.0, 2.0, 2.0, 2.0],
    od=[3, 4, 5, 1, 7, 6, 2], od3=[3, 4, 1, 5, 7, 2, 6], od4=[3, 4, 1, 5, 7, 2, 6], od5=[3, 4, 5, 1, 7, 2, 6])


def lin(terms):
    pos = [v for s, v in terms if s > 0]
    neg = [v for s, v in terms if s < 0]
    acc = pos[0]
    for v in pos[1:]:
        acc = acc + v
    for v in neg:
        acc = acc - v
    return acc


def chain(terms):
    acc = terms[0][1]
    for s, v in terms[1:]:
        acc = acc + v if s > 0 else acc - v
    return acc


def sadd(a, b):
    if a is None:
        return b
    if a[0] == b[0]:
        return (a[0], b[1] + a[1])
    return (1, a[1] - b[1]) if a[0] > 0 else (1, b[1] - a[1])


def comb2(u, sg, v, x=None, e=None):
    if x is not None:
        u = u + x
    if e is not None:
        v = v + e if sg > 0 else v - e
    return u + v if sg > 0 else u - v


def phi3(a):
    l5 = a[0] + a[1]
    return [a[0] + a[3], a[0] - a[1], l5, 0.5 * (l5 + a[3] + a[2])]


def phi4(a):
    return [a[0] + a[3], a[0] - a[1], a[0] + a[1], a[1] + a[2]]


def phi4_inv(e, hf=0.5):
    a11 = hf * (e[1] + e[2])
    a12 = e[2] - a11
    return [a11, a12, e[3] - a12, e[0] - a11]


def psi(c, hf):
    h = hf * c[3]
    c11 = h + c[0]
    return [c11, h, (h + c[1]) + c[2], (c11 + c[1]) - c[2]]


def rc(o, p, q):
    return (o // 2) * 4 + (p // 2) * 2 + q // 2, (o % 2) * 4 + (p % 2) * 2 + q % 2


def popc(v):
    return bin(v).count("1")


def scale(br, bc):
    return S3 ** (popc(br) - popc(bc))


def plan():
    groups, n = {}, 0
    for i in range(1, 8):
        for j in range(1, 8):
            plain = i == 1 or j == 1
            groups[(i, j)] = (n, plain)
            n += 4 if plain else 7
    return groups, n


class RefArr:
    def __init__(self, ref, idx):
        self.ref, self.idx = ref, idx

    def __getitem__(self, k):
        return self.ref[self.idx, k[0] * R:(k[0] + 1) * R, k[1] * Q:(k[1] + 1) * Q]

    def get(self, s, k):
        r = k[0] * R + s * SR
        return self.ref[self.idx, r:r + SR, k[1] * Q:(k[1] + 1) * Q]

    def put(self, s, k, v):
        r = k[0] * R + s * SR
        self.ref[self.idx, r:r + SR, k[1] * Q:(k[1] + 1) * Q] = v

    def putb(self, k, v):
        self.ref[self.idx, k[0] * R:(k[0] + 1) * R, k[1] * Q:(k[1] + 1) * Q] = v


class ValArr:
    def __init__(self, blocks=None):
        self.parts = [dict() for _ in range(NS)]
        self.blocks = dict(blocks or {})

    def __getitem__(self, k):
        if k not in self.blocks:
            self.blocks[k] = jnp.concatenate([p[k] for p in self.parts], axis=0)
        return self.blocks[k]

    def get(self, s, k):
        if k not in self.parts[s]:
            self.parts[s][k] = self.blocks[k][s * SR:(s + 1) * SR]
        return self.parts[s][k]

    def put(self, s, k, v):
        self.parts[s][k] = v


class Sched:
    def __init__(self, never, opt):
        self.never, self.opt = never, opt
        self.q, self.bg, self.lock = [], [], None
        self.g, self.t, self.pace, self.bcredit = None, 0, 0.0, 0.0

    def gv(self, v):
        return v if self.g is None else jnp.where(self.never, self.g, v)

    def gc(self, c):
        return c if self.g is None else jnp.where(self.never, self.g, jnp.full((SR, Q), c, f32))

    def add(self, gen, deadline, cost, bg=False):
        (self.bg if bg else self.q).append([gen, deadline, cost])
        return gen

    def step(self, q, gate=None):
        self.g = gate
        c = None
        while q and c is None:
            c = next(q[0][0], None)
            if c is None:
                q.pop(0)
        if c is not None:
            self.lock = None if isinstance(c, float) else q
            q[0][2] -= c
        self.g = None
        return c

    def tick(self, val, base, brate):
        rate, cum = base, 0.0
        for _, dl, cost in self.q:
            cum += max(cost, 0)
            rate = max(rate, cum / max(dl - self.opt["margin"] - self.t, 1))
        self.bcredit = min(self.bcredit + brate + (0.0 if self.q else base), 40.0)
        self.pace = min(self.pace + rate + (brate if self.bg else 0.0), 40.0)
        if self.pace > 0:
            if self.lock:
                q = self.lock
            elif self.bg and (not self.q or (self.bcredit > 0 and rate <= base)):
                q = self.bg
            else:
                q = self.q
            if q:
                r = self.opt["row"]
                c = self.step(q, val[r * SR:(r + 1) * SR])
                if c:
                    self.pace -= c
                    if q is self.bg:
                        self.bcredit -= c
        self.t += 1

    def drain(self, gen=None, bg=False):
        q = self.bg if bg else self.q
        while q and (gen is None or any(e[0] is gen for e in q)):
            self.step(q)


def load_z(ref):
    z = []
    for o in range(4):
        zz = {}
        for k in IN:
            br, bc = rc(o, *k)
            zz[k] = ref[br * R:(br + 1) * R, bc * Q:(bc + 1) * Q].astype(f32)
        z.append(ValArr(zz))
    return z


def to_basis(dd, q, d, s, emit):
    r = phi3(dd)
    for p in range(4):
        d[(p, q)] = r[p]
        for (b, i, sg, j) in AFTER[q]:
            emit(s, (p, b), d[(p, i)], sg, d[(p, j)])


def head(S, z, H, dl):
    d1, d0 = ValArr(), ValArr()

    def e1(s, k, u, sg, v):
        d1.put(s, k, comb2(u, sg, v))

    def e0(s, k, u, sg, v):
        r = comb2(u, sg, v)
        d0.put(s, k, r)
        H[1].put(s, k, r - d1.get(s, k))
        H[2].put(s, k, r + d1.get(s, k))

    def e2(s, k, u, sg, v):
        H[3].put(s, k, comb2(u, sg, v, d1.get(s, k)))

    def e3(s, k, u, sg, v):
        H[0].put(s, k, comb2(u, sg, v, d0.get(s, k)))

    def tasks():
        for s in range(NS):
            for o, emit in ((1, e1), (2, e2), (0, e0), (3, e3)):
                d = {}
                for q in QORD:
                    v = []
                    for p in range(4):
                        sc = scale(*rc(o, p, q))
                        v.append(z[o].get(s, (p, q)) * sc if sc != 1.0 else z[o].get(s, (p, q)))
                    to_basis([S.gv(v[0])] + v[1:], q, d, s, emit)
                    yield 22.0 if q == QORD[-1] else 22

    return S.add(tasks(), dl, 16 * NS * 22)


def cross(S, dl, o, terms, z, bt_ref, l, emit=None, xo=None, out=None):
    last = emit is None
    qord = TORD if last else QORD
    post = {1: 23, 0: 13, 3: 13, 2: 13} if last else {q: (4 if o < 2 else 12) * len(AFTER[q]) for q in qord}
    cost = {q: 17 + 4 * len(terms) + post[q] for q in qord}

    def tasks():
        for s in range(NS):
            c = {k: chain([(sg, m.get(s, k)) for sg, m in terms]) for k in IN}
            d = {}
            yield 1
            yield 1
            if last:
                xi = {p: phi4_inv([xo.get(s, (p, q)) for q in range(4)]) for p in range(4)}
            for q in qord:
                cc = cost[q]
                y = psi([c[(p, q)] for p in range(4)], S.gc(0.5))
                if last:
                    cc = cost[q] // 2
                    yield cost[q] - cc
                    hf = S.gc(0.5)
                dd = []
                for p in range(4):
                    br, bc = rc(o, p, q)
                    dd.append((y[p] + bt_ref[l * 4 + popc(br), :, bc * Q:(bc + 1) * Q]) * z.get(s, (p, q)))
                if last:
                    e = [xi[p][q] for p in range(4)]
                    a11 = hf * (e[1] + e[2])
                    a22 = e[0] - a11
                    xn = [a11, e[2] - a11, ((e[3] - a22) + e[3]) - e[2], a22]
                    for p in range(4):
                        br, bc = rc(o, p, q)
                        r = dd[p] + xn[p]
                        if scale(br, bc) != 1.0:
                            r = r * (1.0 / scale(br, bc))
                        d[(p, q)] = r
                        if (p, q ^ 1) in d:
                            b0, r0 = bc & ~1, br * R + s * SR
                            pair = jnp.concatenate([d[(p, q & ~1)], d[(p, q | 1)]], axis=1)
                            out[r0:r0 + SR, b0 * Q:(b0 + 2) * Q] = pair.astype(bf16)
                else:
                    to_basis(dd, q, d, s, emit)
                yield float(cc) if q == qord[-1] else cc

    return S.add(tasks(), dl, NS * (2 + sum(cost.values())), bg=last)


def tail(S, z, bt_ref, out, ts_ref, L, quads=(0, 1, 2, 3)):
    for o in quads:
        g = cross(S, 0, o, [(sg, RefArr(ts_ref, 4 + NAMES.index(n))) for sg, n in TERMS[o]], z[o], bt_ref, L - 1,
                  xo=RefArr(ts_ref, o), out=out)
    return g


def unbasis1(S, X, ts_ref):
    for s in range(NS):
        for p in range(4):
            for q0 in (0, 2):
                hf = S.gc(0.5)
                for q in (q0, q0 + 1):
                    r = phi4_inv([X[b].get(s, (p, q)) for b in range(4)], hf)
                    for o in range(4):
                        RefArr(ts_ref, o).put(s, (p, q), r[o])
                yield S.opt["ic"]


def level3(mul, order):
    need = {"v": {1: 1, 3: 1, 5: -1}, "h": {3: 1, 5: 1}, 0: {"v": 1, 4: 1, 7: 1}, 3: {"v": 1, 6: 1, 2: -1},
            2: {"h": 1, 4: 1, 7: -1, 6: 1, 2: 1}}
    acc = {n: None for n in need}
    left = {n: set(t) for n, t in need.items()}
    for k in order:
        todo = [(k, mul(k))]
        while todo:
            name, v = todo.pop(0)
            for n, t in need.items():
                if name in left[n]:
                    left[n].discard(name)
                    acc[n] = sadd(acc[n], (t[name], v))
                    if not left[n]:
                        assert acc[n][0] > 0
                        if n == "h":
                            yield 1, acc[n][1]
                        if n in ("v", "h"):
                            todo.append((n, acc[n][1]))
                        else:
                            yield n, acc[n][1]


def level2(gen):
    out = {}
    c0 = dict(gen(1))
    for ja, jb, idx in ((4, 2, 2), (7, 6, 1), (5, 3, 3)):
        m = {}
        for q, c in gen(ja):
            m[q] = c
            c0[q] = c0[q] - c if ja == 5 else c + c0[q]
        for q, c in gen(jb):
            out[(idx, q)] = c - m[q] if jb == 6 else c + m[q]
    out.update({(0, q): c for q, c in c0.items()})
    return out


def body(x_prev, x_cur, x_next, out, bt_ref, t_ref, hs_ref, ts_ref, L, groups, never, opt):
    S = Sched(never, opt)
    cum = [0]
    for i in ORDER1:
        cum.append(cum[-1] + sum(8 if groups[(i, j)][1] else 7 for j in range(1, 8)))
    TL, mg = cum[-1], opt["margin"]
    zp, z, zn = load_z(x_prev), load_z(x_cur), load_z(x_next)
    X = [RefArr(hs_ref, b) for b in range(4)]
    pre = [10 * opt["pre"]]
    need = None
    tl = tail(S, zp, bt_ref, out, ts_ref, L)

    for l in range(L):
        T0 = l * TL
        last = l == L - 1

        def dot(u, n):
            w = pltpu.bitcast(t_ref[l, n // 2, :, (n % 2) * Q:(n % 2 + 1) * Q], bf16)
            return jnp.dot(u, w, preferred_element_type=f32)

        def level1(i):
            base = opt["rates%d" % l][ORDER1.index(i)]
            brate = opt.get("brates%d" % l, opt["brates"])[ORDER1.index(i)]

            def group(j):
                a = [lin([(s1 * s2, X[b1][(b2, q)]) for s1, b1 in CORE4[i] for s2, b2 in CORE3[j]])
                     for q in range(4)]
                n, plain = groups[(i, j)]
                if plain:
                    an = phi4_inv(a)
                    k0 = jnp.concatenate([an[0], an[2]], axis=0).astype(bf16)
                    k1 = jnp.concatenate([an[1], an[3]], axis=0).astype(bf16)

                    def mul2(u, k):
                        r = dot(u, n + k)
                        S.tick(r[:R], base, brate)
                        S.tick(r[R:], base, brate)
                        return r

                    c0 = mul2(k0, 0) + mul2(k1, 2)
                    c1 = mul2(k0, 1) + mul2(k1, 3)
                    return enumerate([c0[:R], c1[:R], c0[R:], c1[R:]])

                def mul(k):
                    u = lin([(s3, a[b]) for s3, b in CORE4[k]])
                    if len(CORE4[k]) == 2:
                        for r0 in (0, 2 * SR):
                            if pre[0] > 0:
                                S.step(S.bg, u[r0:r0 + SR])
                                pre[0] -= 1
                    r = dot(u.astype(bf16), n + k - 1)
                    S.tick(r, base, brate)
                    return r

                return level3(mul, opt.get("od%d" % l, opt["od"]))

            return level2(group)

        XN = [ValArr() for _ in range(4)]
        d12, d11 = ValArr(), ValArr()

        def emitter(o, X=X, XN=XN, d12=d12, d11=d11):
            def emit(s, k, u, sg, v):
                if o == 1:
                    d12.put(s, k, comb2(u, sg, v))
                elif o == 0:
                    e, r = d12.get(s, k), comb2(u, sg, v)
                    d11.put(s, k, r)
                    XN[1].put(s, k, (r + X[1].get(s, k)) - e)
                    XN[2].put(s, k, (r + X[2].get(s, k)) + e)
                elif o == 3:
                    XN[0].put(s, k, comb2(u, sg, v, X[0].get(s, k), d11.get(s, k)))
                else:
                    XN[3].put(s, k, comb2(u, sg, v, X[3].get(s, k), d12.get(s, k)))
            return emit

        M, nn = {}, {}

        def keep(name, m):
            M[name] = ValArr(m)
            if last:
                for k in IN:
                    RefArr(ts_ref, 4 + NAMES.index(name)).putb(k, m[k])

        def add(o, dl):
            if not last:
                nn[o] = cross(S, dl, o, [(sg, M[n]) for sg, n in TERMS[o]], z[o], bt_ref, l, emit=emitter(o))

        if last:
            S.drain(tl, bg=True)
        if need:
            S.drain(need[0])
        m3 = level1(3)
        m5 = level1(5)
        if last:
            S.add(unbasis1(S, X, ts_ref), T0 + TL + opt["endm"], NS * 8 * opt["ic"])
            head(S, zn, [RefArr(hs_ref, b) for b in range(4)], T0 + TL + opt["endm"])
        keep("h", {k: m5[k] + m3[k] for k in IN})
        v = {k: m3[k] - m5[k] for k in IN}
        add(1, T0 + cum[5] + mg)
        if need:
            S.drain(need[3])
        m1 = level1(1)
        keep("v", {k: m1[k] + v[k] for k in IN})
        keep("m4", level1(4))
        keep("m7", level1(7))
        add(0, T0 + TL)
        if need:
            S.drain(need[2])
        keep("m6", level1(6))
        keep("m2", level1(2))
        add(3, T0 + TL + cum[2])
        add(2, T0 + TL + cum[5])
        need, X = nn, XN
    S.drain()


def tform(e, k):
    if k == 1:
        return e[0] + e[0]
    return lin([(s, e[b]) for s, b in CORE4[SIGMA[k]]])


def table_tasks(S, w_ref, tb_ref, l, groups):
    for c in range(Q // CR):
        E = []
        for r0 in range(c * CR, (c + 1) * CR, SR):
            H, d1, d0 = [{} for _ in range(4)], {}, {}
            for o in (1, 2, 0, 3):
                def emit(s, k, u, sg, v):
                    if o == 1:
                        d1[k] = comb2(u, sg, v)
                    elif o == 2:
                        H[3][k] = comb2(u, sg, v, d1[k])
                    elif o == 0:
                        d0[k] = comb2(u, sg, v)
                        H[1][k], H[2][k] = d0[k] - d1[k], d0[k] + d1[k]
                    else:
                        H[0][k] = comb2(u, sg, v, d0[k])

                d = {}
                for q in QORD:
                    v = []
                    for p in range(4):
                        br, bc = rc(o, p, q)
                        sc = 0.25 * scale(br, bc)
                        v.append(w_ref[br, r0:r0 + SR, bc * Q:(bc + 1) * Q].astype(f32) * (S.gc(sc) if p == 0 else sc))
                    to_basis(v, q, d, 0, emit)
                    yield 23
            E.append(H)
        for i in range(1, 8):
            s1, first = {}, CORE4[SIGMA[i]][0][1]
            for b2 in range(4):
                two = S.gc(2.0) if i == 1 else None
                for q in range(4):
                    if i == 1:
                        hs = [two * H[0][(b2, q)] for H in E]
                    else:
                        hs = [tform([S.gv(H[b][(b2, q)]) if b == first else H[b][(b2, q)] for b in range(4)], i)
                              for H in E]
                    s1[(b2, q)] = jnp.concatenate(hs, axis=0)
                js = [j for j in range(1, 8) if max(b for _, b in CORE3[SIGMA[j]]) == b2]
                for j in js:
                    e = [lin([(sg, s1[(b, q)]) for sg, b in CORE3[SIGMA[j]]]) for q in range(4)]
                    n, plain = groups[(i, j)]
                    if plain:
                        a, b = e[1] + e[2], e[2] - e[1]
                        outs = [a, b, (e[3] - b) + e[3], (e[0] - a) + e[0]]
                    else:
                        outs = [tform(e, k) for k in range(1, 8)]
                    for k, t in enumerate(outs):
                        c0 = ((n + k) % 2) * Q
                        tb_ref.at[l, (n + k) // 2][c * CR:(c + 1) * CR, c0:c0 + Q] = t.astype(bf16)
                yield 16 + 21 * len(js)


def first_layer(l, w_ref, z_ref, xi_ref, xo_ref, bt_ref, tb_ref, groups, opt):
    S = Sched(jnp.full((SR, Q), l, jnp.int32) < 0, opt)
    S.add(table_tasks(S, w_ref, tb_ref, l, groups), 0, 0)
    rate = (Q // CR) * (32 * 23 + 7 * (4 * 16 + 7 * 21)) / (16 * TM // SR)
    pace = 0.0
    x = xi_ref[...]
    xb = x.astype(bf16)
    for n in range(8):
        cs = slice(n * Q, (n + 1) * Q)
        acc = None
        for kh in range(2):
            rs = [jnp.dot(xb[:, k * Q:(k + 1) * Q], w_ref[k, :, cs], preferred_element_type=f32)
                  for k in range(4 * kh, 4 * kh + 4)]
            oth = (rs[1] + rs[2]) + rs[3]
            acc = oth if acc is None else acc + oth
            for g in range(TM // SR):
                pace += rate
                for r in (rs[0], rs[3]):
                    if pace > 0:
                        pace -= S.step(S.q, r[g * SR:(g + 1) * SR]) or 0
            acc = acc + rs[0]
        xo_ref[:, cs] = z_ref[:, cs] * (acc + bt_ref[l * 4 + popc(n), 0:1, cs]) + x[:, cs]
    S.drain()


def kernel(x_hbm, w_hbm, b_hbm, o_hbm, t_ref, bt_ref, hs_ref, ts_ref, xs_ref, w_buf, x_buf, o_buf, o0_buf, b_buf,
           w_sem, x_sem, o_sem, m_sem, *, L, nb, groups, opt):
    def wcopy(l):
        return pltpu.make_async_copy(w_hbm.at[l], w_buf.at[l & 1], w_sem.at[l & 1])

    def xcopy(i):
        return pltpu.make_async_copy(x_hbm.at[pl.ds(pl.multiple_of(i * TM, TM), TM), :],
                                     x_buf.at[i & (NX - 1)], x_sem.at[i & (NX - 1)])

    def ocopy(i):
        return pltpu.make_async_copy(o_buf.at[i & (NO - 1)], o_hbm.at[pl.ds(pl.multiple_of(i * TM, TM), TM), :],
                                     o_sem.at[i & (NO - 1)])

    bcopy = pltpu.make_async_copy(b_hbm, b_buf, m_sem.at[0])
    bcopy.start()
    xcopy(0).start()
    wcopy(0).start()
    ts_ref[...] = jnp.zeros(ts_ref.shape, f32)
    bcopy.wait()
    for l in range(L):
        for e in range(4):
            for bc in range(8):
                row = b_buf[l:l + 1, bc * Q:(bc + 1) * Q].astype(f32) * (S3 ** (e - popc(bc)))
                bt_ref[l * 4 + e, :, bc * Q:(bc + 1) * Q] = jnp.broadcast_to(row, (SR, Q))
    xcopy(0).wait()
    xs_ref[0] = x_buf[0].astype(f32)
    xs_ref[2] = x_buf[0].astype(f32)
    tb_ref = t_ref.bitcast(bf16)
    wcopy(0).wait()

    def first(l, carry):
        nxt = wcopy(jnp.minimum(l + 1, L - 1))
        pl.when(l + 1 < L)(nxt.start)

        @pl.when(l + 1 == L)
        def _():
            xcopy(1).start()
            xcopy(2).start()

        first_layer(l, w_buf.at[l & 1], xs_ref.at[2], xs_ref.at[l & 1], xs_ref.at[1 - (l & 1)], bt_ref, tb_ref,
                    groups, opt)
        pl.when(l + 1 < L)(nxt.wait)
        return carry

    jax.lax.fori_loop(0, L, first, 0)
    o0_buf[...] = xs_ref[L % 2].astype(bf16)
    o0copy = pltpu.make_async_copy(o0_buf, o_hbm.at[pl.ds(0, TM), :], m_sem.at[3])
    o0copy.start()
    xcopy(1).wait()
    S = Sched(None, opt)
    head(S, load_z(x_buf.at[1]), [RefArr(hs_ref, b) for b in range(4)], 0)
    S.drain()

    def dmas(i):
        cps = [xcopy(jnp.minimum(i + 2, nb - 1)), ocopy(jnp.maximum(i - 2, 1)),
               xcopy(jnp.minimum(i + 1, nb - 1)), ocopy(jnp.maximum(i - 3, 1))]
        pl.when(i + 2 < nb)(cps[0].start)
        pl.when(i >= 3)(cps[1].start)
        pl.when(i + 1 < nb)(cps[2].wait)
        pl.when(i >= 4)(cps[3].wait)

    def step(i, carry):
        never = jnp.full((SR, Q), i, jnp.int32) < 0
        xs = [x_buf.at[jnp.clip(i + u, 0, nb - 1) & (NX - 1)] for u in (-1, 0, 1)]
        body(*xs, o_buf.at[(i + 1) & (NO - 1)], bt_ref, t_ref, hs_ref, ts_ref, L, groups, never, opt)
        dmas(i + 1)
        return carry

    dmas(jnp.int32(1))
    jax.lax.fori_loop(1, nb, step, 0)

    last, H = nb - 1, TM // 2
    z = load_z(x_buf.at[last % NX])
    halves = [pltpu.make_async_copy(o_buf.at[last % NO, pl.ds(h * H, H), :],
                                    o_hbm.at[pl.ds(last * TM + h * H, H), :], m_sem.at[1 + h]) for h in range(2)]
    for h in range(2):
        S = Sched(None, opt)
        tail(S, z, bt_ref, o_buf.at[last % NO], ts_ref, L, (2 * h, 2 * h + 1))
        S.drain(bg=True)
        halves[h].start()
    o0copy.wait()
    ocopy(last - 1).wait()
    for h in range(2):
        halves[h].wait()


def make(o=None):
    opt = dict(OPT)
    opt.update(o or {})
    groups, n = plan()

    @jax.jit
    def run(x0, ws, bs):
        B, D = x0.shape
        L = ws.shape[0]
        assert D == 8 * Q and B % TM == 0 and B >= 3 * TM and L == 6 and n % 2 == 0
        return pl.pallas_call(
            functools.partial(kernel, L=L, nb=B // TM, groups=groups, opt=opt),
            in_specs=[pl.BlockSpec(memory_space=pl.ANY)] * 3,
            out_specs=pl.BlockSpec(memory_space=pl.ANY),
            out_shape=jax.ShapeDtypeStruct((B, D), x0.dtype),
            scratch_shapes=[
                pltpu.VMEM((L, n // 2, Q // 2, 2 * Q), jnp.uint32),
                pltpu.VMEM((L * 4, SR, D), f32),
                pltpu.VMEM((4, 4 * R, D // 2), f32),
                pltpu.VMEM((10, 4 * R, D // 2), f32),
                pltpu.VMEM((3, TM, D), f32),
                pltpu.VMEM((2, 8, Q, D), bf16),
                pltpu.VMEM((NX, TM, D), bf16),
                pltpu.VMEM((NO, TM, D), bf16),
                pltpu.VMEM((TM, D), bf16),
                pltpu.VMEM((L, D), bf16),
                pltpu.SemaphoreType.DMA((2,)),
                pltpu.SemaphoreType.DMA((NX,)),
                pltpu.SemaphoreType.DMA((NO,)),
                pltpu.SemaphoreType.DMA((4,)),
            ],
            compiler_params=pltpu.CompilerParams(vmem_limit_bytes=100 * 1024 * 1024, disable_bounds_checks=True),
        )(x0, ws.reshape(L, 8, Q, D), bs)

    return run


_run = make()


@jax.jit
def pallas_standalone__dcn_v2_cross__recsys_kernel(x0: jax.Array, ws: jax.Array, bs: jax.Array):
    return _run(x0, ws, bs)
```

```python
import functools
import math

import jax
import jax.numpy as jnp
import jax.experimental.pallas as pl
import jax.experimental.pallas.tpu as pltpu

f32 = jnp.float32
bf16 = jnp.bfloat16

Q = 128
R = 32
SR = 8
NS = R // SR
TM = 8 * R
CR = 16
XG = 8
NX = 4 * XG
NO = 2
S3 = math.sqrt(3.0)
IN = [(p, q) for p in range(4) for q in range(4)]

CORE3 = {1: [(1, 0)], 3: [(1, 1)], 5: [(1, 2)], 2: [(1, 3)],
         4: [(1, 0), (-1, 1)], 7: [(1, 2), (-1, 0)], 6: [(1, 3), (-1, 0)]}
CORE4 = {1: [(1, 0)], 3: [(1, 1)], 5: [(1, 2)], 2: [(1, 3), (1, 0)],
         4: [(1, 0), (-1, 1)], 7: [(1, 2), (-1, 0)], 6: [(1, 3), (-1, 0)]}
SIGMA = {1: 1, 2: 3, 3: 7, 4: 6, 5: 4, 6: 5, 7: 2}
ORDER1 = [3, 5, 1, 4, 7, 6, 2]
QORD = [2, 1, 0, 3]
TORD = [1, 0, 3, 2]
AFTER = {2: [], 1: [(3, 1, 1, 2)], 0: [(1, 0, -1, 1), (2, 0, 1, 1)], 3: [(0, 3, 1, 0)]}
NAMES = ["h", "v", "m4", "m7", "m6", "m2"]
TERMS = {1: [(1, "h")], 0: [(1, "m7"), (1, "v"), (1, "m4")], 3: [(1, "v"), (-1, "m2"), (1, "m6")],
         2: [(1, "m2"), (1, "m6"), (1, "h"), (1, "m4"), (-1, "m7")]}

OPT = dict(
    row=2, margin=27, pre=2, ic=18.0, endm=25,
    rates0=[9.2, 9.4, 10, 6, 6.8, 5.5, 5.4], rates1=[9.2, 7, 11.5, 5.5, 5.5, 5.5, 5.4],
    rates2=[9.2, 7, 11.5, 4.8, 4.2, 5.5, 5.4], rates3=[9.2, 7, 11.5, 5.5, 6.7, 5.5, 5.4],
    rates4=[9.2, 7, 11.5, 5.5, 5.5, 5.5, 5.3], rates5=[9.2, 7, 12.4, 4.3, 5.5, 5.5, 5.4],
    brates=[2.0] * 7, brates0=[2.0, 2.3, 1.0, 2.0, 3.0, 2.0, 3.0], brates1=[2.1, 2.0, 2.0, 2.0, 2.0, 2.0, 2.0],
    od=[3, 4, 5, 1, 7, 6, 2], od3=[3, 4, 1, 5, 7, 2, 6], od4=[3, 4, 1, 5, 7, 2, 6], od5=[3, 4, 5, 1, 7, 2, 6])


def lin(terms):
    pos = [v for s, v in terms if s > 0]
    neg = [v for s, v in terms if s < 0]
    acc = pos[0]
    for v in pos[1:]:
        acc = acc + v
    for v in neg:
        acc = acc - v
    return acc


def chain(terms):
    acc = terms[0][1]
    for s, v in terms[1:]:
        acc = acc + v if s > 0 else acc - v
    return acc


def sadd(a, b):
    if a is None:
        return b
    if a[0] == b[0]:
        return (a[0], b[1] + a[1])
    return (1, a[1] - b[1]) if a[0] > 0 else (1, b[1] - a[1])


def comb2(u, sg, v, x=None, e=None):
    if x is not None:
        u = u + x
    if e is not None:
        v = v + e if sg > 0 else v - e
    return u + v if sg > 0 else u - v


def phi3(a):
    l5 = a[0] + a[1]
    return [a[0] + a[3], a[0] - a[1], l5, 0.5 * (l5 + a[3] + a[2])]


def phi4(a):
    return [a[0] + a[3], a[0] - a[1], a[0] + a[1], a[1] + a[2]]


def phi4_inv(e, hf=0.5):
    a11 = hf * (e[1] + e[2])
    a12 = e[2] - a11
    return [a11, a12, e[3] - a12, e[0] - a11]


def psi(c, hf):
    h = hf * c[3]
    c11 = h + c[0]
    return [c11, h, (h + c[1]) + c[2], (c11 + c[1]) - c[2]]


def rc(o, p, q):
    return (o // 2) * 4 + (p // 2) * 2 + q // 2, (o % 2) * 4 + (p % 2) * 2 + q % 2


def popc(v):
    return bin(v).count("1")


def scale(br, bc):
    return S3 ** (popc(br) - popc(bc))


def plan():
    groups, n = {}, 0
    for i in range(1, 8):
        for j in range(1, 8):
            plain = i == 1 or j == 1
            groups[(i, j)] = (n, plain)
            n += 4 if plain else 7
    return groups, n


class RefArr:
    def __init__(self, ref, idx):
        self.ref, self.idx = ref, idx

    def __getitem__(self, k):
        return self.ref[self.idx, k[0] * R:(k[0] + 1) * R, k[1] * Q:(k[1] + 1) * Q]

    def get(self, s, k):
        r = k[0] * R + s * SR
        return self.ref[self.idx, r:r + SR, k[1] * Q:(k[1] + 1) * Q]

    def put(self, s, k, v):
        r = k[0] * R + s * SR
        self.ref[self.idx, r:r + SR, k[1] * Q:(k[1] + 1) * Q] = v

    def putb(self, k, v):
        self.ref[self.idx, k[0] * R:(k[0] + 1) * R, k[1] * Q:(k[1] + 1) * Q] = v


class ValArr:
    def __init__(self, blocks=None):
        self.parts = [dict() for _ in range(NS)]
        self.blocks = dict(blocks or {})

    def __getitem__(self, k):
        if k not in self.blocks:
            self.blocks[k] = jnp.concatenate([p[k] for p in self.parts], axis=0)
        return self.blocks[k]

    def get(self, s, k):
        if k not in self.parts[s]:
            self.parts[s][k] = self.blocks[k][s * SR:(s + 1) * SR]
        return self.parts[s][k]

    def put(self, s, k, v):
        self.parts[s][k] = v


class Sched:
    def __init__(self, never, opt):
        self.never, self.opt = never, opt
        self.q, self.bg, self.lock = [], [], None
        self.g, self.t, self.pace, self.bcredit = None, 0, 0.0, 0.0

    def gv(self, v):
        return v if self.g is None else jnp.where(self.never, self.g, v)

    def gc(self, c):
        return c if self.g is None else jnp.where(self.never, self.g, jnp.full((SR, Q), c, f32))

    def add(self, gen, deadline, cost, bg=False):
        (self.bg if bg else self.q).append([gen, deadline, cost])
        return gen

    def step(self, q, gate=None):
        self.g = gate
        c = None
        while q and c is None:
            c = next(q[0][0], None)
            if c is None:
                q.pop(0)
        if c is not None:
            self.lock = None if isinstance(c, float) else q
            q[0][2] -= c
        self.g = None
        return c

    def tick(self, val, base, brate):
        rate, cum = base, 0.0
        for _, dl, cost in self.q:
            cum += max(cost, 0)
            rate = max(rate, cum / max(dl - self.opt["margin"] - self.t, 1))
        self.bcredit = min(self.bcredit + brate + (0.0 if self.q else base), 40.0)
        self.pace = min(self.pace + rate + (brate if self.bg else 0.0), 40.0)
        if self.pace > 0:
            if self.lock:
                q = self.lock
            elif self.bg and (not self.q or (self.bcredit > 0 and rate <= base)):
                q = self.bg
            else:
                q = self.q
            if q:
                r = self.opt["row"]
                c = self.step(q, val[r * SR:(r + 1) * SR])
                if c:
                    self.pace -= c
                    if q is self.bg:
                        self.bcredit -= c
        self.t += 1

    def drain(self, gen=None, bg=False):
        q = self.bg if bg else self.q
        while q and (gen is None or any(e[0] is gen for e in q)):
            self.step(q)


def load_z(ref):
    z = []
    for o in range(4):
        zz = {}
        for k in IN:
            br, bc = rc(o, *k)
            zz[k] = ref[br * R:(br + 1) * R, bc * Q:(bc + 1) * Q].astype(f32)
        z.append(ValArr(zz))
    return z


def to_basis(dd, q, d, s, emit):
    r = phi3(dd)
    for p in range(4):
        d[(p, q)] = r[p]
        for (b, i, sg, j) in AFTER[q]:
            emit(s, (p, b), d[(p, i)], sg, d[(p, j)])


def head(S, z, H, dl):
    d1, d0 = ValArr(), ValArr()

    def e1(s, k, u, sg, v):
        d1.put(s, k, comb2(u, sg, v))

    def e0(s, k, u, sg, v):
        r = comb2(u, sg, v)
        d0.put(s, k, r)
        H[1].put(s, k, r - d1.get(s, k))
        H[2].put(s, k, r + d1.get(s, k))

    def e2(s, k, u, sg, v):
        H[3].put(s, k, comb2(u, sg, v, d1.get(s, k)))

    def e3(s, k, u, sg, v):
        H[0].put(s, k, comb2(u, sg, v, d0.get(s, k)))

    def tasks():
        for s in range(NS):
            for o, emit in ((1, e1), (2, e2), (0, e0), (3, e3)):
                d = {}
                for q in QORD:
                    v = []
                    for p in range(4):
                        sc = scale(*rc(o, p, q))
                        v.append(z[o].get(s, (p, q)) * sc if sc != 1.0 else z[o].get(s, (p, q)))
                    to_basis([S.gv(v[0])] + v[1:], q, d, s, emit)
                    yield 22.0 if q == QORD[-1] else 22

    return S.add(tasks(), dl, 16 * NS * 22)


def cross(S, dl, o, terms, z, bt_ref, l, emit=None, xo=None, out=None):
    last = emit is None
    qord = TORD if last else QORD
    post = {1: 23, 0: 13, 3: 13, 2: 13} if last else {q: (4 if o < 2 else 12) * len(AFTER[q]) for q in qord}
    cost = {q: 17 + 4 * len(terms) + post[q] for q in qord}

    def tasks():
        for s in range(NS):
            c = {k: chain([(sg, m.get(s, k)) for sg, m in terms]) for k in IN}
            d = {}
            yield 1
            yield 1
            if last:
                xi = {p: phi4_inv([xo.get(s, (p, q)) for q in range(4)]) for p in range(4)}
            for q in qord:
                cc = cost[q]
                y = psi([c[(p, q)] for p in range(4)], S.gc(0.5))
                if last:
                    cc = cost[q] // 2
                    yield cost[q] - cc
                    hf = S.gc(0.5)
                dd = []
                for p in range(4):
                    br, bc = rc(o, p, q)
                    dd.append((y[p] + bt_ref[l * 4 + popc(br), :, bc * Q:(bc + 1) * Q]) * z.get(s, (p, q)))
                if last:
                    e = [xi[p][q] for p in range(4)]
                    a11 = hf * (e[1] + e[2])
                    a22 = e[0] - a11
                    xn = [a11, e[2] - a11, ((e[3] - a22) + e[3]) - e[2], a22]
                    for p in range(4):
                        br, bc = rc(o, p, q)
                        r = dd[p] + xn[p]
                        if scale(br, bc) != 1.0:
                            r = r * (1.0 / scale(br, bc))
                        d[(p, q)] = r
                        if (p, q ^ 1) in d:
                            b0, r0 = bc & ~1, br * R + s * SR
                            pair = jnp.concatenate([d[(p, q & ~1)], d[(p, q | 1)]], axis=1)
                            out[r0:r0 + SR, b0 * Q:(b0 + 2) * Q] = pair.astype(bf16)
                else:
                    to_basis(dd, q, d, s, emit)
                yield float(cc) if q == qord[-1] else cc

    return S.add(tasks(), dl, NS * (2 + sum(cost.values())), bg=last)


def tail(S, z, bt_ref, out, ts_ref, L, quads=(0, 1, 2, 3)):
    for o in quads:
        g = cross(S, 0, o, [(sg, RefArr(ts_ref, 4 + NAMES.index(n))) for sg, n in TERMS[o]], z[o], bt_ref, L - 1,
                  xo=RefArr(ts_ref, o), out=out)
    return g


def unbasis1(S, X, ts_ref):
    for s in range(NS):
        for p in range(4):
            for q0 in (0, 2):
                hf = S.gc(0.5)
                for q in (q0, q0 + 1):
                    r = phi4_inv([X[b].get(s, (p, q)) for b in range(4)], hf)
                    for o in range(4):
                        RefArr(ts_ref, o).put(s, (p, q), r[o])
                yield S.opt["ic"]


def level3(mul, order):
    need = {"v": {1: 1, 3: 1, 5: -1}, "h": {3: 1, 5: 1}, 0: {"v": 1, 4: 1, 7: 1}, 3: {"v": 1, 6: 1, 2: -1},
            2: {"h": 1, 4: 1, 7: -1, 6: 1, 2: 1}}
    acc = {n: None for n in need}
    left = {n: set(t) for n, t in need.items()}
    for k in order:
        todo = [(k, mul(k))]
        while todo:
            name, v = todo.pop(0)
            for n, t in need.items():
                if name in left[n]:
                    left[n].discard(name)
                    acc[n] = sadd(acc[n], (t[name], v))
                    if not left[n]:
                        assert acc[n][0] > 0
                        if n == "h":
                            yield 1, acc[n][1]
                        if n in ("v", "h"):
                            todo.append((n, acc[n][1]))
                        else:
                            yield n, acc[n][1]


def level2(gen):
    out = {}
    c0 = dict(gen(1))
    for ja, jb, idx in ((4, 2, 2), (7, 6, 1), (5, 3, 3)):
        m = {}
        for q, c in gen(ja):
            m[q] = c
            c0[q] = c0[q] - c if ja == 5 else c + c0[q]
        for q, c in gen(jb):
            out[(idx, q)] = c - m[q] if jb == 6 else c + m[q]
    out.update({(0, q): c for q, c in c0.items()})
    return out


def body(x_prev, x_cur, x_next, out, bt_ref, t_ref, hs_ref, ts_ref, L, groups, never, opt):
    S = Sched(never, opt)
    cum = [0]
    for i in ORDER1:
        cum.append(cum[-1] + sum(8 if groups[(i, j)][1] else 7 for j in range(1, 8)))
    TL, mg = cum[-1], opt["margin"]
    zp, z, zn = load_z(x_prev), load_z(x_cur), load_z(x_next)
    X = [RefArr(hs_ref, b) for b in range(4)]
    pre = [10 * opt["pre"]]
    need = None
    tl = tail(S, zp, bt_ref, out, ts_ref, L)

    for l in range(L):
        T0 = l * TL
        last = l == L - 1

        def dot(u, n):
            w = pltpu.bitcast(t_ref[l, n // 2, :, (n % 2) * Q:(n % 2 + 1) * Q], bf16)
            return jnp.dot(u, w, preferred_element_type=f32)

        def level1(i):
            base = opt["rates%d" % l][ORDER1.index(i)]
            brate = opt.get("brates%d" % l, opt["brates"])[ORDER1.index(i)]

            def group(j):
                a = [lin([(s1 * s2, X[b1][(b2, q)]) for s1, b1 in CORE4[i] for s2, b2 in CORE3[j]])
                     for q in range(4)]
                n, plain = groups[(i, j)]
                if plain:
                    an = phi4_inv(a)
                    k0 = jnp.concatenate([an[0], an[2]], axis=0).astype(bf16)
                    k1 = jnp.concatenate([an[1], an[3]], axis=0).astype(bf16)

                    def mul2(u, k):
                        r = dot(u, n + k)
                        S.tick(r[:R], base, brate)
                        S.tick(r[R:], base, brate)
                        return r

                    c0 = mul2(k0, 0) + mul2(k1, 2)
                    c1 = mul2(k0, 1) + mul2(k1, 3)
                    return enumerate([c0[:R], c1[:R], c0[R:], c1[R:]])

                def mul(k):
                    u = lin([(s3, a[b]) for s3, b in CORE4[k]])
                    if len(CORE4[k]) == 2:
                        for r0 in (0, 2 * SR):
                            if pre[0] > 0:
                                S.step(S.bg, u[r0:r0 + SR])
                                pre[0] -= 1
                    r = dot(u.astype(bf16), n + k - 1)
                    S.tick(r, base, brate)
                    return r

                return level3(mul, opt.get("od%d" % l, opt["od"]))

            return level2(group)

        XN = [ValArr() for _ in range(4)]
        d12, d11 = ValArr(), ValArr()

        def emitter(o, X=X, XN=XN, d12=d12, d11=d11):
            def emit(s, k, u, sg, v):
                if o == 1:
                    d12.put(s, k, comb2(u, sg, v))
                elif o == 0:
                    e, r = d12.get(s, k), comb2(u, sg, v)
                    d11.put(s, k, r)
                    XN[1].put(s, k, (r + X[1].get(s, k)) - e)
                    XN[2].put(s, k, (r + X[2].get(s, k)) + e)
                elif o == 3:
                    XN[0].put(s, k, comb2(u, sg, v, X[0].get(s, k), d11.get(s, k)))
                else:
                    XN[3].put(s, k, comb2(u, sg, v, X[3].get(s, k), d12.get(s, k)))
            return emit

        M, nn = {}, {}

        def keep(name, m):
            M[name] = ValArr(m)
            if last:
                for k in IN:
                    RefArr(ts_ref, 4 + NAMES.index(name)).putb(k, m[k])

        def add(o, dl):
            if not last:
                nn[o] = cross(S, dl, o, [(sg, M[n]) for sg, n in TERMS[o]], z[o], bt_ref, l, emit=emitter(o))

        if last:
            S.drain(tl, bg=True)
        if need:
            S.drain(need[0])
        m3 = level1(3)
        m5 = level1(5)
        if last:
            S.add(unbasis1(S, X, ts_ref), T0 + TL + opt["endm"], NS * 8 * opt["ic"])
            head(S, zn, [RefArr(hs_ref, b) for b in range(4)], T0 + TL + opt["endm"])
        keep("h", {k: m5[k] + m3[k] for k in IN})
        v = {k: m3[k] - m5[k] for k in IN}
        add(1, T0 + cum[5] + mg)
        if need:
            S.drain(need[3])
        m1 = level1(1)
        keep("v", {k: m1[k] + v[k] for k in IN})
        keep("m4", level1(4))
        keep("m7", level1(7))
        add(0, T0 + TL)
        if need:
            S.drain(need[2])
        keep("m6", level1(6))
        keep("m2", level1(2))
        add(3, T0 + TL + cum[2])
        add(2, T0 + TL + cum[5])
        need, X = nn, XN
    S.drain()


def tform(e, k):
    if k == 1:
        return e[0] + e[0]
    return lin([(s, e[b]) for s, b in CORE4[SIGMA[k]]])


def table_tasks(S, w_ref, tb_ref, l, groups):
    for c in range(Q // CR):
        E = []
        for r0 in range(c * CR, (c + 1) * CR, SR):
            H, d1, d0 = [{} for _ in range(4)], {}, {}
            for o in (1, 2, 0, 3):
                def emit(s, k, u, sg, v):
                    if o == 1:
                        d1[k] = comb2(u, sg, v)
                    elif o == 2:
                        H[3][k] = comb2(u, sg, v, d1[k])
                    elif o == 0:
                        d0[k] = comb2(u, sg, v)
                        H[1][k], H[2][k] = d0[k] - d1[k], d0[k] + d1[k]
                    else:
                        H[0][k] = comb2(u, sg, v, d0[k])

                d = {}
                for q in QORD:
                    v = []
                    for p in range(4):
                        br, bc = rc(o, p, q)
                        sc = 0.25 * scale(br, bc)
                        v.append(w_ref[br, r0:r0 + SR, bc * Q:(bc + 1) * Q].astype(f32) * (S.gc(sc) if p == 0 else sc))
                    to_basis(v, q, d, 0, emit)
                    yield 23
            E.append(H)
        for i in range(1, 8):
            s1, first = {}, CORE4[SIGMA[i]][0][1]
            for b2 in range(4):
                two = S.gc(2.0) if i == 1 else None
                for q in range(4):
                    if i == 1:
                        hs = [two * H[0][(b2, q)] for H in E]
                    else:
                        hs = [tform([S.gv(H[b][(b2, q)]) if b == first else H[b][(b2, q)] for b in range(4)], i)
                              for H in E]
                    s1[(b2, q)] = jnp.concatenate(hs, axis=0)
                js = [j for j in range(1, 8) if max(b for _, b in CORE3[SIGMA[j]]) == b2]
                for j in js:
                    e = [lin([(sg, s1[(b, q)]) for sg, b in CORE3[SIGMA[j]]]) for q in range(4)]
                    n, plain = groups[(i, j)]
                    if plain:
                        a, b = e[1] + e[2], e[2] - e[1]
                        outs = [a, b, (e[3] - b) + e[3], (e[0] - a) + e[0]]
                    else:
                        outs = [tform(e, k) for k in range(1, 8)]
                    for k, t in enumerate(outs):
                        c0 = ((n + k) % 2) * Q
                        tb_ref.at[l, (n + k) // 2][c * CR:(c + 1) * CR, c0:c0 + Q] = t.astype(bf16)
                yield 16 + 21 * len(js)


def first_layer(l, w_ref, z_ref, xi_ref, xo_ref, bt_ref, tb_ref, groups, opt):
    S = Sched(jnp.full((SR, Q), l, jnp.int32) < 0, opt)
    S.add(table_tasks(S, w_ref, tb_ref, l, groups), 0, 0)
    rate = (Q // CR) * (32 * 23 + 7 * (4 * 16 + 7 * 21)) / (16 * TM // SR)
    pace = 0.0
    x = xi_ref[...]
    xb = x.astype(bf16)
    for n in range(8):
        cs = slice(n * Q, (n + 1) * Q)
        acc = None
        for kh in range(2):
            rs = [jnp.dot(xb[:, k * Q:(k + 1) * Q], w_ref[k, :, cs], preferred_element_type=f32)
                  for k in range(4 * kh, 4 * kh + 4)]
            oth = (rs[1] + rs[2]) + rs[3]
            acc = oth if acc is None else acc + oth
            for g in range(TM // SR):
                pace += rate
                for r in (rs[0], rs[3]):
                    if pace > 0:
                        pace -= S.step(S.q, r[g * SR:(g + 1) * SR]) or 0
            acc = acc + rs[0]
        xo_ref[:, cs] = z_ref[:, cs] * (acc + bt_ref[l * 4 + popc(n), 0:1, cs]) + x[:, cs]
    S.drain()


def kernel(x_hbm, w_hbm, b_hbm, o_hbm, t_ref, bt_ref, hs_ref, ts_ref, xs_ref, w_buf, x_buf, o_buf, o0_buf, b_buf,
           w_sem, x_sem, o_sem, m_sem, *, L, nb, groups, opt):
    def wcopy(l):
        return pltpu.make_async_copy(w_hbm.at[l], w_buf.at[l & 1], w_sem.at[l & 1])

    def xcopy(i, n=1):
        return pltpu.make_async_copy(x_hbm.at[pl.ds(i, n)], x_buf.at[pl.ds(i, n)], x_sem.at[4 + i])

    def gcopy(g):
        return pltpu.make_async_copy(x_hbm.at[pl.ds(g * XG, XG)], x_buf.at[pl.ds((g & 3) * XG, XG)], x_sem.at[g & 3])

    def ocopy(i):
        return pltpu.make_async_copy(o_buf.at[i & (NO - 1)], o_hbm.at[pl.ds(pl.multiple_of(i * TM, TM), TM), :],
                                     o_sem.at[i & (NO - 1)])

    bcopy = pltpu.make_async_copy(b_hbm, b_buf, m_sem.at[0])
    bcopy.start()
    xcopy(0).start()
    wcopy(0).start()
    ts_ref[...] = jnp.zeros(ts_ref.shape, f32)
    bcopy.wait()
    for l in range(L):
        for e in range(4):
            for bc in range(8):
                row = b_buf[l:l + 1, bc * Q:(bc + 1) * Q].astype(f32) * (S3 ** (e - popc(bc)))
                bt_ref[l * 4 + e, :, bc * Q:(bc + 1) * Q] = jnp.broadcast_to(row, (SR, Q))
    xcopy(0).wait()
    xs_ref[0] = x_buf[0].astype(f32)
    xs_ref[2] = x_buf[0].astype(f32)
    tb_ref = t_ref.bitcast(bf16)
    wcopy(0).wait()

    def first(l, carry):
        nxt = wcopy(jnp.minimum(l + 1, L - 1))
        pl.when(l + 1 < L)(nxt.start)

        @pl.when(l + 1 == L)
        def _():
            xcopy(1).start()
            xcopy(2).start()

        first_layer(l, w_buf.at[l & 1], xs_ref.at[2], xs_ref.at[l & 1], xs_ref.at[1 - (l & 1)], bt_ref, tb_ref,
                    groups, opt)
        pl.when(l + 1 < L)(nxt.wait)
        return carry

    jax.lax.fori_loop(0, L, first, 0)
    o0_buf[...] = xs_ref[L % 2].astype(bf16)
    o0copy = pltpu.make_async_copy(o0_buf, o_hbm.at[pl.ds(0, TM), :], m_sem.at[3])
    o0copy.start()
    xcopy(1).wait()
    S = Sched(None, opt)
    head(S, load_z(x_buf.at[1]), [RefArr(hs_ref, b) for b in range(4)], 0)
    S.drain()

    def dmas(i):
        g, ng = (i + 1) >> 3, nb // XG
        turn = ((i + 1) & (XG - 1)) == 0
        cps = [gcopy(jnp.minimum(g + 1, ng - 1)), ocopy(jnp.maximum(i - 2, 1)),
               gcopy(jnp.minimum(g, ng - 1)), ocopy(jnp.maximum(i - 3, 1))]
        pl.when(turn & (g + 1 < ng))(cps[0].start)
        pl.when(i >= 3)(cps[1].start)
        pl.when(turn & (g < ng))(cps[2].wait)
        pl.when(i == 2)(xcopy(3, XG - 3).wait)
        pl.when(i >= 4)(cps[3].wait)

    def step(i, carry):
        never = jnp.full((SR, Q), i, jnp.int32) < 0
        xs = [x_buf.at[jnp.clip(i + u, 0, nb - 1) & (NX - 1)] for u in (-1, 0, 1)]
        body(*xs, o_buf.at[(i + 1) & (NO - 1)], bt_ref, t_ref, hs_ref, ts_ref, L, groups, never, opt)
        dmas(i + 1)
        return carry

    xcopy(2).wait()
    xcopy(3, XG - 3).start()
    gcopy(1).start()
    jax.lax.fori_loop(1, nb, step, 0)

    last, H = nb - 1, TM // 2
    z = load_z(x_buf.at[last % NX])
    halves = [pltpu.make_async_copy(o_buf.at[last % NO, pl.ds(h * H, H), :],
                                    o_hbm.at[pl.ds(last * TM + h * H, H), :], m_sem.at[1 + h]) for h in range(2)]
    for h in range(2):
        S = Sched(None, opt)
        tail(S, z, bt_ref, o_buf.at[last % NO], ts_ref, L, (2 * h, 2 * h + 1))
        S.drain(bg=True)
        halves[h].start()
    o0copy.wait()
    ocopy(last - 1).wait()
    for h in range(2):
        halves[h].wait()


def make(o=None):
    opt = dict(OPT)
    opt.update(o or {})
    groups, n = plan()

    @jax.jit
    def run(x0, ws, bs):
        B, D = x0.shape
        L = ws.shape[0]
        assert D == 8 * Q and B % (XG * TM) == 0 and B >= 2 * XG * TM and L == 6 and n % 2 == 0
        return pl.pallas_call(
            functools.partial(kernel, L=L, nb=B // TM, groups=groups, opt=opt),
            in_specs=[pl.BlockSpec(memory_space=pl.ANY)] * 3,
            out_specs=pl.BlockSpec(memory_space=pl.ANY),
            out_shape=jax.ShapeDtypeStruct((B, D), x0.dtype),
            scratch_shapes=[
                pltpu.VMEM((L, n // 2, Q // 2, 2 * Q), jnp.uint32),
                pltpu.VMEM((L * 4, SR, D), f32),
                pltpu.VMEM((4, 4 * R, D // 2), f32),
                pltpu.VMEM((10, 4 * R, D // 2), f32),
                pltpu.VMEM((3, TM, D), f32),
                pltpu.VMEM((2, 8, Q, D), bf16),
                pltpu.VMEM((NX, TM, D), bf16),
                pltpu.VMEM((NO, TM, D), bf16),
                pltpu.VMEM((TM, D), bf16),
                pltpu.VMEM((L, D), bf16),
                pltpu.SemaphoreType.DMA((2,)),
                pltpu.SemaphoreType.DMA((8,)),
                pltpu.SemaphoreType.DMA((NO,)),
                pltpu.SemaphoreType.DMA((4,)),
            ],
            compiler_params=pltpu.CompilerParams(vmem_limit_bytes=110 * 1024 * 1024, disable_bounds_checks=True),
        )(x0.reshape(B // TM, TM, D), ws.reshape(L, 8, Q, D), bs)

    return run


_run = make()


@jax.jit
def pallas_standalone__dcn_v2_cross__recsys_kernel(x0: jax.Array, ws: jax.Array, bs: jax.Array):
    return _run(x0, ws, bs)
```

```python
import functools
import math

import jax
import jax.numpy as jnp
import jax.experimental.pallas as pl
import jax.experimental.pallas.tpu as pltpu

f32 = jnp.float32
bf16 = jnp.bfloat16

Q = 128
R = 32
SR = 8
NS = R // SR
TM = 8 * R
CR = 16
XG = 8
NX = 4 * XG
NO = 2
S3 = math.sqrt(3.0)

CORE3 = {1: [(1, 0)], 3: [(1, 1)], 5: [(1, 2)], 2: [(1, 3)],
         4: [(1, 0), (-1, 1)], 7: [(1, 2), (-1, 0)], 6: [(1, 3), (-1, 0)]}
CORE4 = {1: [(1, 0)], 3: [(1, 1)], 5: [(1, 2)], 2: [(1, 3), (1, 0)],
         4: [(1, 0), (-1, 1)], 7: [(1, 2), (-1, 0)], 6: [(1, 3), (-1, 0)]}
SIGMA = {1: 1, 2: 3, 3: 7, 4: 6, 5: 4, 6: 5, 7: 2}
ORDER1 = [3, 5, 1, 4, 7, 6, 2]
QORD = [2, 1, 0, 3]
TORD = [1, 0, 3, 2]
PHI4 = [(3, 1, 0), (0, -1, 1), (0, 1, 1), (1, 1, 2)]
NAMES = ["h", "v", "m4", "m7", "m6", "m2"]
TERMS = {1: [(1, "h")], 0: [(1, "m7"), (1, "v"), (1, "m4")], 3: [(1, "v"), (-1, "m2"), (1, "m6")],
         2: [(1, "m2"), (1, "m6"), (1, "h"), (1, "m4"), (-1, "m7")]}

OPT = dict(
    row=2, margin=27, pre=2, ic=18.0, endm=25,
    rates0=[9.2, 9.4, 10, 5.4, 6.8, 5.5, 5.4], rates1=[9.2, 7, 11.5, 4.6, 6.2, 5.5, 5.4],
    rates2=[9.2, 7, 11.5, 5.9, 4.2, 5.5, 5.4], rates3=[9.2, 7, 11.5, 6.0, 6.7, 5.5, 5.4],
    rates4=[9.2, 7, 11.5, 5.5, 5.5, 5.5, 5.3], rates5=[9.2, 7, 12.4, 4.3, 6.9, 5.5, 5.4],
    brates=[2.0] * 7, brates0=[2.0, 2.9, 1.0, 2.0, 3.0, 2.0, 3.0], brates1=[2.1, 2.0, 2.0, 2.0, 2.0, 2.0, 2.0],
    od0=[3, 4, 5, 1, 7, 2, 6], od1=[3, 4, 5, 1, 7, 6, 2], od2=[3, 4, 5, 1, 7, 6, 2],
    od3=[3, 4, 1, 5, 7, 2, 6], od4=[3, 6, 1, 5, 7, 2, 4], od5=[3, 4, 5, 1, 7, 2, 6])


def lin(terms):
    pos = [v for s, v in terms if s > 0]
    neg = [v for s, v in terms if s < 0]
    acc = pos[0]
    for v in pos[1:]:
        acc = acc + v
    for v in neg:
        acc = acc - v
    return acc


def chain(terms):
    acc = terms[0][1]
    for s, v in terms[1:]:
        acc = acc + v if s > 0 else acc - v
    return acc


def sadd(a, b):
    if a is None:
        return b
    if a[0] == b[0]:
        return (a[0], b[1] + a[1])
    return (1, a[1] - b[1]) if a[0] > 0 else (1, b[1] - a[1])


def comb2(u, sg, v, x=None, e=None):
    if x is not None:
        u = u + x
    if e is not None:
        v = v + e if sg > 0 else v - e
    return u + v if sg > 0 else u - v


def phi3(a):
    l5 = a[0] + a[1]
    return [a[0] + a[3], a[0] - a[1], l5, 0.5 * (l5 + a[3] + a[2])]


def phi4_inv(e, hf=0.5):
    a11 = hf * (e[1] + e[2])
    a12 = e[2] - a11
    return [a11, a12, e[3] - a12, e[0] - a11]


def psi(c, hf):
    h = hf * c[3]
    c11 = h + c[0]
    return [c11, h, (h + c[1]) + c[2], (c11 + c[1]) - c[2]]


def rc(o, p, q):
    return (o // 2) * 4 + (p // 2) * 2 + q // 2, (o % 2) * 4 + (p % 2) * 2 + q % 2


def popc(v):
    return bin(v).count("1")


def scale(br, bc):
    return S3 ** (popc(br) - popc(bc))


def plan():
    groups, n = {}, 0
    for i in range(1, 8):
        for j in range(1, 8):
            plain = i == 1 or j == 1
            groups[(i, j)] = (n, plain)
            n += 4 if plain else 7
    return groups, n


def cat(xs, axis):
    return jnp.concatenate(list(xs), axis=axis)


def rows(x, p):
    return x[p * R:(p + 1) * R]


def cols(x, q):
    return x[:, q * Q:(q + 1) * Q]


class Sched:
    def __init__(self, it, opt):
        self.it, self.opt = it, opt
        self.q, self.bg, self.lock = [], [], None
        self.g, self.t, self.pace, self.bcredit = None, 0, 0.0, 0.0

    def gated(self, gates, v):
        shape = (len(gates) * SR, len(gates[0]) * Q)
        if all(g is None for r in gates for g in r):
            return v
        if not isinstance(v, jax.Array):
            v = jnp.full(shape, v, f32)
        g = cat([cat([v[i * SR:(i + 1) * SR, j * Q:(j + 1) * Q] if x is None else x for j, x in enumerate(r)], 1)
                 for i, r in enumerate(gates)], 0)
        return jnp.where(jnp.full(shape, self.it, jnp.int32) < 0, g, v)

    def add(self, gen, deadline, cost, bg=False):
        (self.bg if bg else self.q).append([gen, deadline, cost])
        return gen

    def step(self, q, gate=None):
        self.g = gate
        c = None
        while q and c is None:
            c = next(q[0][0], None)
            if c is None:
                q.pop(0)
        if c is not None:
            self.lock = None if isinstance(c, float) else q
            q[0][2] -= c
        self.g = None
        return c

    def tick(self, val, base, brate):
        rate, cum = base, 0.0
        for _, dl, cost in self.q:
            cum += max(cost, 0)
            rate = max(rate, cum / max(dl - self.opt["margin"] - self.t, 1))
        self.bcredit = min(self.bcredit + brate + (0.0 if self.q else base), 40.0)
        self.pace = min(self.pace + rate + (brate if self.bg else 0.0), 40.0)
        if self.pace > 0:
            if self.lock:
                q = self.lock
            elif self.bg and (not self.q or (self.bcredit > 0 and rate <= base)):
                q = self.bg
            else:
                q = self.q
            if q:
                r = self.opt["row"]
                c = self.step(q, val[r * SR:(r + 1) * SR])
                if c:
                    self.pace -= c
                    if q is self.bg:
                        self.bcredit -= c
        self.t += 1

    def drain(self, gen=None, bg=False):
        q = self.bg if bg else self.q
        while q and (gen is None or any(e[0] is gen for e in q)):
            self.step(q)


def load_panel(get, o, p):
    return cat([get(br, bc * Q, (bc + 1) * Q).astype(f32) for br, bc in (rc(o, p, q) for q in range(4))], 1)


def load_z(ref):
    get = lambda br, c0, c1: ref[br * R:(br + 1) * R, c0:c1]
    return [[load_panel(get, o, p) for p in range(4)] for o in range(4)]


def rescale(x, f):
    return cat([cols(x, q) if f(q) == 1.0 else cols(x, q) * f(q) for q in range(4)], 1)


def to_basis(dd, x=None, e=None):
    d = cat(phi3(dd), 0)
    return cat([comb2(cols(d, i), sg, cols(d, j), None if x is None else cols(x, b), None if e is None else cols(e, b))
                for b, (i, sg, j) in enumerate(PHI4)], 1)


def basis1(v):
    d1, d0 = to_basis(v[1]), to_basis(v[0])
    return [to_basis(v[3], d0), d0 - d1, d0 + d1, to_basis(v[2], d1)]


def head(S, z, hs_ref, dl):
    def job():
        g = {o: [[None] * 4 for _ in range(NS)] for o in range(4)}
        for s in range(NS):
            for o in (1, 2, 0, 3):
                for q in QORD:
                    g[o][s][q] = S.g
                    if (s, o, q) == (NS - 1, 3, QORD[-1]):
                        v = [[rescale(z[o][p], lambda q: scale(*rc(o, p, q))) for p in range(4)] for o in range(4)]
                        for b, x in enumerate(basis1([[S.gated(g[o], v[o][0])] + v[o][1:] for o in range(4)])):
                            hs_ref[b] = x
                    yield 22.0 if q == QORD[-1] else 22

    return S.add(job(), dl, 16 * NS * 22)


def cross(S, dl, o, terms, z, bt_ref, l, emit=None, xo=None, out=None):
    last = emit is None
    qord = TORD if last else QORD
    post = {1: 23, 0: 13, 3: 13, 2: 13} if last else {q: (4 if o < 2 else 12) * n for q, n in zip(QORD, (0, 1, 2, 1))}
    cost = {q: 17 + 4 * len(terms) + post[q] for q in qord}

    def finish(g1, g2):
        c = chain([(sg, m()) for sg, m in terms])
        y = psi([rows(c, p) for p in range(4)], S.gated(g1, 0.5))
        bias = lambda br, c0, c1: bt_ref[l * 4 + popc(br), :, c0:c1]
        dd = [(y[p] + cat([load_panel(bias, o, p)] * NS, 0)) * z[p] for p in range(4)]
        if not last:
            return emit(dd)
        x = xo()
        x = cat(phi4_inv([cols(x, q) for q in range(4)]), 1)
        e = [rows(x, p) for p in range(4)]
        a11 = S.gated(g2, 0.5) * (e[1] + e[2])
        a22 = e[0] - a11
        xn = [a11, e[2] - a11, ((e[3] - a22) + e[3]) - e[2], a22]
        for p in range(4):
            r = rescale(dd[p] + xn[p], lambda q: 1.0 / scale(*rc(o, p, q)))
            br, bc = rc(o, p, 0)
            for t in range(2):
                out[(br + t) * R:(br + t + 1) * R, bc * Q:(bc + 2) * Q] = r[:, 2 * t * Q:2 * (t + 1) * Q].astype(bf16)

    def job():
        g1, g2 = ([[None] * 4 for _ in range(NS)] for _ in range(2))
        for s in range(NS):
            yield 1
            yield 1
            for q in qord:
                cc = cost[q]
                g1[s][q] = S.g
                if last:
                    cc = cost[q] // 2
                    yield cost[q] - cc
                    g2[s][q] = S.g
                if (s, q) == (NS - 1, qord[-1]):
                    finish(g1, g2)
                yield float(cc) if q == qord[-1] else cc

    return S.add(job(), dl, NS * (2 + sum(cost.values())), bg=last)


def tail(S, z, bt_ref, out, ts_ref, L, quads=(0, 1, 2, 3)):
    for o in quads:
        g = cross(S, 0, o, [(sg, functools.partial(lambda n: ts_ref[n], 4 + NAMES.index(n))) for sg, n in TERMS[o]],
                  z[o], bt_ref, L - 1, xo=functools.partial(lambda n: ts_ref[n], o), out=out)
    return g


def unbasis1(S, X, ts_ref):
    g = [[None] * 2 for _ in range(4 * NS)]
    for s in range(NS):
        for p in range(4):
            for t in range(2):
                g[p * NS + s][t] = S.g
                if (s, p, t) == (NS - 1, 3, 1):
                    hf = S.gated(g, 0.5)
                    if isinstance(hf, jax.Array):
                        hf = cat([cols(hf, q // 2) for q in range(4)], 1)
                    for o, x in enumerate(phi4_inv([X[b]() for b in range(4)], hf)):
                        ts_ref[o] = x
                yield S.opt["ic"]


def level3(mul, order):
    need = {"v": {1: 1, 3: 1, 5: -1}, 1: {3: 1, 5: 1}, 0: {"v": 1, 4: 1, 7: 1}, 3: {"v": 1, 6: 1, 2: -1},
            2: {"h": 1, 4: 1, 7: -1, 6: 1, 2: 1}}
    acc = {n: None for n in need}
    left = {n: set(t) for n, t in need.items()}
    for k in order:
        todo = [(k, mul(k))]
        while todo:
            name, v = todo.pop(0)
            for n, t in need.items():
                if name in left[n]:
                    left[n].discard(name)
                    acc[n] = sadd(acc[n], (t[name], v))
                    if not left[n] and n in ("v", 1):
                        todo.append(("v" if n == "v" else "h", acc[n][1]))
    assert all(a[0] > 0 for a in acc.values())
    return cat([acc[q][1] for q in range(4)], 1)


def level2(mul):
    c0 = mul(1)
    m4 = mul(4)
    c0 = m4 + c0
    c2 = mul(2) + m4
    m7 = mul(7)
    c0 = m7 + c0
    c1 = mul(6) - m7
    m5 = mul(5)
    c0 = c0 - m5
    return cat([c0, c1, c2, mul(3) + m5], 0)


def body(it, x_prev, x_cur, x_next, out, bt_ref, t_ref, hs_ref, ts_ref, L, groups, opt):
    S = Sched(it, opt)
    cum = [0]
    for i in ORDER1:
        cum.append(cum[-1] + sum(8 if groups[(i, j)][1] else 7 for j in range(1, 8)))
    TL, mg = cum[-1], opt["margin"]
    z = load_z(x_cur)
    X = {b: hs_ref[b] for b in range(4)}
    pre = [10 * opt["pre"]]
    need = None
    tl = tail(S, load_z(x_prev), bt_ref, out, ts_ref, L)

    for l in range(L):
        T0 = l * TL
        last = l == L - 1

        def dot(u, n):
            return jnp.dot(u, t_ref[l, n // 2, :, (n % 2) * Q:(n % 2 + 1) * Q], preferred_element_type=f32)

        def level1(i):
            base = opt["rates%d" % l][ORDER1.index(i)]
            brate = opt.get("brates%d" % l, opt["brates"])[ORDER1.index(i)]

            def group(j):
                a = lin([(s1 * s2, rows(X[b1], b2)) for s1, b1 in CORE4[i] for s2, b2 in CORE3[j]])
                a = [cols(a, q) for q in range(4)]
                n, plain = groups[(i, j)]
                if plain:
                    an = phi4_inv(a)
                    k0 = cat([an[0], an[2]], 0).astype(bf16)
                    k1 = cat([an[1], an[3]], 0).astype(bf16)

                    def mul2(u, k):
                        r = dot(u, n + k)
                        S.tick(r[:R], base, brate)
                        S.tick(r[R:], base, brate)
                        return r

                    c0 = mul2(k0, 0) + mul2(k1, 2)
                    c1 = mul2(k0, 1) + mul2(k1, 3)
                    return cat([c0[:R], c1[:R], c0[R:], c1[R:]], 1)

                def mul(k):
                    u = lin([(s3, a[b]) for s3, b in CORE4[k]])
                    if len(CORE4[k]) == 2:
                        for r0 in (0, 2 * SR):
                            if pre[0] > 0:
                                S.step(S.bg, u[r0:r0 + SR])
                                pre[0] -= 1
                    r = dot(u.astype(bf16), n + k - 1)
                    S.tick(r, base, brate)
                    return r

                return level3(mul, opt["od%d" % l])

            return level2(group)

        XN, D, M, nn = {}, {}, {}, {}

        def emitter(o, X=X, XN=XN, D=D):
            def emit(dd):
                if o < 2:
                    D[o] = to_basis(dd)
                if o == 0:
                    XN[1] = (D[0] + X[1]) - D[1]
                    XN[2] = (D[0] + X[2]) + D[1]
                elif o == 3:
                    XN[0] = to_basis(dd, X[0], D[0])
                elif o == 2:
                    XN[3] = to_basis(dd, X[3], D[1])
            return emit

        def keep(name, m):
            M[name] = m
            if last:
                ts_ref[4 + NAMES.index(name)] = m

        def add(o, dl):
            if not last:
                nn[o] = cross(S, dl, o, [(sg, functools.partial(M.get, n)) for sg, n in TERMS[o]], z[o], bt_ref, l,
                              emit=emitter(o))

        if last:
            S.drain(tl, bg=True)
        if need:
            S.drain(need[0])
        m3 = level1(3)
        m5 = level1(5)
        if last:
            S.add(unbasis1(S, [functools.partial(X.get, b) for b in range(4)], ts_ref), T0 + TL + opt["endm"],
                  NS * 8 * opt["ic"])
            head(S, load_z(x_next), hs_ref, T0 + TL + opt["endm"])
        keep("h", m5 + m3)
        v = m3 - m5
        add(1, T0 + cum[5] + mg)
        if need:
            S.drain(need[3])
        keep("v", level1(1) + v)
        keep("m4", level1(4))
        keep("m7", level1(7))
        add(0, T0 + TL)
        if need:
            S.drain(need[2])
        keep("m6", level1(6))
        keep("m2", level1(2))
        add(3, T0 + TL + cum[2])
        add(2, T0 + TL + cum[5])
        need, X = nn, XN
    S.drain()


def tform(e, k):
    if k == 1:
        return e[0] + e[0]
    return lin([(s, e[b]) for s, b in CORE4[SIGMA[k]]])


def table_job(S, w_ref, tb_ref, l, groups):
    ga = {o: [[None] * 4 for _ in range(Q // SR)] for o in range(4)}
    gb = {(i, b): [None] * (Q // CR) for i in range(1, 8) for b in range(4)}
    js = {b: [j for j in range(1, 8) if max(t for _, t in CORE3[SIGMA[j]]) == b] for b in range(4)}
    for c in range(Q // CR):
        for s in range(c * CR // SR, (c + 1) * CR // SR):
            for o in (1, 2, 0, 3):
                for q in QORD:
                    ga[o][s][q] = S.g
                    yield 23
        for i in range(1, 8):
            for b in range(4):
                gb[(i, b)][c] = S.g
                yield 16 + 21 * len(js[b])
    v = []
    for o in range(4):
        w = [load_panel(lambda br, c0, c1: w_ref[br, :, c0:c1], o, p) for p in range(4)]
        sc = cat([jnp.full((Q, Q), 0.25 * scale(*rc(o, 0, q)), f32) for q in range(4)], 1)
        v.append([w[0] * S.gated(ga[o], sc)]
                 + [rescale(w[p], lambda q: 0.25 * scale(*rc(o, p, q))) for p in range(1, 4)])
    E = basis1(v)
    for i in range(1, 8):
        if i == 1:
            two = S.gated([[gb[(i, b)][c]] for b in range(4) for c in range(Q // CR)], 2.0)
            two = cat([two[t // 2 * SR:(t // 2 + 1) * SR] for t in range(4 * Q // SR)], 0)
            s1 = cat([two] * 4, 1) * E[0]
        else:
            first = CORE4[SIGMA[i]][0][1]
            g = [[gb[(i, b)][s * SR // CR]] * 4 for b in range(4) for s in range(Q // SR)]
            s1 = tform([S.gated(g, E[b]) if b == first else E[b] for b in range(4)], i)
        for j in range(1, 8):
            e = lin([(sg, s1[b * Q:(b + 1) * Q]) for sg, b in CORE3[SIGMA[j]]])
            e = [cols(e, q) for q in range(4)]
            n, plain = groups[(i, j)]
            if plain:
                a, b = e[1] + e[2], e[2] - e[1]
                outs = [a, b, (e[3] - b) + e[3], (e[0] - a) + e[0]]
            else:
                outs = [tform(e, k) for k in range(1, 8)]
            for k, t in enumerate(outs):
                c0 = ((n + k) % 2) * Q
                tb_ref.at[l, (n + k) // 2][:, c0:c0 + Q] = t.astype(bf16)


def first_layer(l, w_ref, z_ref, xi_ref, xo_ref, bt_ref, tb_ref, groups, opt):
    S = Sched(l, opt)
    S.add(table_job(S, w_ref, tb_ref, l, groups), 0, 0)
    rate = (Q // CR) * (32 * 23 + 7 * (4 * 16 + 7 * 21)) / (16 * TM // SR)
    pace = 0.0
    x = xi_ref[...]
    xb = x.astype(bf16)
    for n in range(8):
        cs = slice(n * Q, (n + 1) * Q)
        acc = None
        for kh in range(2):
            rs = [jnp.dot(cols(xb, k), w_ref[k, :, cs], preferred_element_type=f32) for k in range(4 * kh, 4 * kh + 4)]
            oth = (rs[1] + rs[2]) + rs[3]
            acc = oth if acc is None else acc + oth
            for g in range(TM // SR):
                pace += rate
                for r in (rs[0], rs[3]):
                    if pace > 0:
                        pace -= S.step(S.q, r[g * SR:(g + 1) * SR]) or 0
            acc = acc + rs[0]
        xo_ref[:, cs] = z_ref[:, cs] * (acc + bt_ref[l * 4 + popc(n), 0:1, cs]) + x[:, cs]
    S.drain()


def kernel(x_hbm, w_hbm, b_hbm, o_hbm, t_ref, bt_ref, hs_ref, ts_ref, xs_ref, w_buf, x_buf, o_buf, o0_buf, b_buf,
           w_sem, x_sem, o_sem, m_sem, *, L, nb, groups, opt):
    def wcopy(l):
        return pltpu.make_async_copy(w_hbm.at[l], w_buf.at[l & 1], w_sem.at[l & 1])

    def xcopy(i, n=1):
        return pltpu.make_async_copy(x_hbm.at[pl.ds(i, n)], x_buf.at[pl.ds(i, n)], x_sem.at[4 + i])

    def gcopy(g):
        return pltpu.make_async_copy(x_hbm.at[pl.ds(g * XG, XG)], x_buf.at[pl.ds((g & 3) * XG, XG)], x_sem.at[g & 3])

    def ocopy(i):
        return pltpu.make_async_copy(o_buf.at[i & (NO - 1)], o_hbm.at[pl.ds(pl.multiple_of(i * TM, TM), TM), :],
                                     o_sem.at[i & (NO - 1)])

    bcopy = pltpu.make_async_copy(b_hbm, b_buf, m_sem.at[0])
    bcopy.start()
    xcopy(0).start()
    wcopy(0).start()
    ts_ref[...] = jnp.zeros(ts_ref.shape, f32)
    bcopy.wait()
    b = b_buf[...].astype(f32)
    for e in range(4):
        be = cat([cols(b, bc) * S3 ** (e - popc(bc)) for bc in range(8)], 1)
        for l in range(L):
            bt_ref[l * 4 + e] = jnp.broadcast_to(be[l:l + 1], (SR, 8 * Q))
    xcopy(0).wait()
    xs_ref[0] = x_buf[0].astype(f32)
    xs_ref[2] = x_buf[0].astype(f32)
    tb_ref = t_ref.bitcast(bf16)
    wcopy(0).wait()

    def first(l, carry):
        nxt = wcopy(jnp.minimum(l + 1, L - 1))
        pl.when(l + 1 < L)(nxt.start)

        @pl.when(l + 1 == L)
        def _():
            xcopy(1).start()
            xcopy(2).start()

        first_layer(l, w_buf.at[l & 1], xs_ref.at[2], xs_ref.at[l & 1], xs_ref.at[1 - (l & 1)], bt_ref, tb_ref,
                    groups, opt)
        pl.when(l + 1 < L)(nxt.wait)
        return carry

    jax.lax.fori_loop(0, L, first, 0)
    o0_buf[...] = xs_ref[L % 2].astype(bf16)
    o0copy = pltpu.make_async_copy(o0_buf, o_hbm.at[pl.ds(0, TM), :], m_sem.at[3])
    o0copy.start()
    xcopy(1).wait()
    S = Sched(None, opt)
    head(S, load_z(x_buf.at[1]), hs_ref, 0)
    S.drain()

    def dmas(i):
        g, ng = (i + 1) >> 3, nb // XG
        turn = ((i + 1) & (XG - 1)) == 0
        cps = [gcopy(jnp.minimum(g + 1, ng - 1)), ocopy(jnp.maximum(i - 2, 1)),
               gcopy(jnp.minimum(g, ng - 1)), ocopy(jnp.maximum(i - 3, 1))]
        pl.when(turn & (g + 1 < ng))(cps[0].start)
        pl.when(i >= 3)(cps[1].start)
        pl.when(turn & (g < ng))(cps[2].wait)
        pl.when(i == 2)(xcopy(3, XG - 3).wait)
        pl.when(i >= 4)(cps[3].wait)

    def step(i, carry):
        xs = [x_buf.at[jnp.clip(i + u, 0, nb - 1) & (NX - 1)] for u in (-1, 0, 1)]
        body(i, *xs, o_buf.at[(i + 1) & (NO - 1)], bt_ref, tb_ref, hs_ref, ts_ref, L, groups, opt)
        dmas(i + 1)
        return carry

    xcopy(2).wait()
    xcopy(3, XG - 3).start()
    gcopy(1).start()
    jax.lax.fori_loop(1, nb, step, 0)

    last, H = nb - 1, TM // 2
    z = load_z(x_buf.at[last % NX])
    halves = [pltpu.make_async_copy(o_buf.at[last % NO, pl.ds(h * H, H), :],
                                    o_hbm.at[pl.ds(last * TM + h * H, H), :], m_sem.at[1 + h]) for h in range(2)]
    for h in range(2):
        S = Sched(None, opt)
        tail(S, z, bt_ref, o_buf.at[last % NO], ts_ref, L, (2 * h, 2 * h + 1))
        S.drain(bg=True)
        halves[h].start()
    o0copy.wait()
    ocopy(last - 1).wait()
    for h in range(2):
        halves[h].wait()


def make(o=None):
    opt = dict(OPT)
    opt.update(o or {})
    groups, n = plan()

    @jax.jit
    def run(x0, ws, bs):
        B, D = x0.shape
        L = ws.shape[0]
        assert D == 8 * Q and B % (XG * TM) == 0 and B >= 2 * XG * TM and L == 6 and n % 2 == 0
        return pl.pallas_call(
            functools.partial(kernel, L=L, nb=B // TM, groups=groups, opt=opt),
            in_specs=[pl.BlockSpec(memory_space=pl.ANY)] * 3,
            out_specs=pl.BlockSpec(memory_space=pl.ANY),
            out_shape=jax.ShapeDtypeStruct((B, D), x0.dtype),
            scratch_shapes=[
                pltpu.VMEM((L, n // 2, Q // 2, 2 * Q), jnp.uint32),
                pltpu.VMEM((L * 4, SR, D), f32),
                pltpu.VMEM((4, 4 * R, D // 2), f32),
                pltpu.VMEM((10, 4 * R, D // 2), f32),
                pltpu.VMEM((3, TM, D), f32),
                pltpu.VMEM((2, 8, Q, D), bf16),
                pltpu.VMEM((NX, TM, D), bf16),
                pltpu.VMEM((NO, TM, D), bf16),
                pltpu.VMEM((TM, D), bf16),
                pltpu.VMEM((L, D), bf16),
                pltpu.SemaphoreType.DMA((2,)),
                pltpu.SemaphoreType.DMA((8,)),
                pltpu.SemaphoreType.DMA((NO,)),
                pltpu.SemaphoreType.DMA((4,)),
            ],
            compiler_params=pltpu.CompilerParams(vmem_limit_bytes=110 * 1024 * 1024, disable_bounds_checks=True),
        )(x0.reshape(B // TM, TM, D), ws.reshape(L, 8, Q, D), bs)

    return run


_run = make()


@jax.jit
def pallas_standalone__dcn_v2_cross__recsys_kernel(x0: jax.Array, ws: jax.Array, bs: jax.Array):
    return _run(x0, ws, bs)
```

```python
import functools
import math

import jax
import jax.numpy as jnp
import jax.experimental.pallas as pl
import jax.experimental.pallas.tpu as pltpu

f32 = jnp.float32
bf16 = jnp.bfloat16

Q = 128
R = 32
SR = 8
NS = R // SR
TM = 8 * R
CR = 16
XG = 8
NX = 4 * XG
NO = 2
NP = 16
S3 = math.sqrt(3.0)

CORE3 = {1: [(1, 0)], 3: [(1, 1)], 5: [(1, 2)], 2: [(1, 3)],
         4: [(1, 0), (-1, 1)], 7: [(1, 2), (-1, 0)], 6: [(1, 3), (-1, 0)]}
CORE4 = {1: [(1, 0)], 3: [(1, 1)], 5: [(1, 2)], 2: [(1, 3), (1, 0)],
         4: [(1, 0), (-1, 1)], 7: [(1, 2), (-1, 0)], 6: [(1, 3), (-1, 0)]}
SIGMA = {1: 1, 2: 3, 3: 7, 4: 6, 5: 4, 6: 5, 7: 2}
ORDER1 = [3, 5, 1, 4, 7, 6, 2]
QORD = [2, 1, 0, 3]
TORD = [1, 0, 3, 2]
PHI4 = [(3, 1, 0), (0, -1, 1), (0, 1, 1), (1, 1, 2)]
NAMES = ["h", "v", "m4", "m7", "m6", "m2"]
TERMS = {1: [(1, "h")], 0: [(1, "m7"), (1, "v"), (1, "m4")], 3: [(1, "v"), (-1, "m2"), (1, "m6")],
         2: [(1, "m2"), (1, "m6"), (1, "h"), (1, "m4"), (-1, "m7")]}

LIMIT = 6.0

OPT = dict(
    limit=LIMIT, row=2, margin=27, pre=2, ic=18.0, endm=25,
    rates0=[9.2, 9.4, 10, 5.4, 6.8, 5.5, 5.4], rates1=[9.2, 5.4, 11.5, 4.6, 6.6, 5.5, 5.4],
    rates2=[9.2, 7, 11.5, 5.9, 4.2, 5.5, 5.4], rates3=[9.2, 7, 11.5, 6.0, 6.7, 5.5, 5.4],
    rates4=[9.2, 7, 11.5, 5.5, 4.8, 5.5, 5.3], rates5=[9.2, 7, 12.4, 4.3, 6.9, 5.5, 5.4],
    brates=[2.0] * 7, brates0=[2.0, 2.9, 1.0, 2.0, 3.0, 2.0, 3.0], brates1=[2.1, 2.0, 2.0, 2.0, 2.0, 2.0, 2.0],
    od0=[3, 4, 5, 1, 7, 2, 6], od1=[3, 4, 5, 1, 7, 6, 2], od2=[3, 4, 5, 1, 7, 2, 6],
    od3=[3, 4, 1, 5, 6, 2, 7], od4=[3, 6, 1, 5, 7, 2, 4], od5=[3, 4, 5, 1, 7, 6, 2])


def lin(terms):
    pos = [v for s, v in terms if s > 0]
    neg = [v for s, v in terms if s < 0]
    acc = pos[0]
    for v in pos[1:]:
        acc = acc + v
    for v in neg:
        acc = acc - v
    return acc


def chain(terms):
    acc = terms[0][1]
    for s, v in terms[1:]:
        acc = acc + v if s > 0 else acc - v
    return acc


def sadd(a, b):
    if a is None:
        return b
    if a[0] == b[0]:
        return (a[0], b[1] + a[1])
    return (1, a[1] - b[1]) if a[0] > 0 else (1, b[1] - a[1])


def comb2(u, sg, v, x=None, e=None):
    if x is not None:
        u = u + x
    if e is not None:
        v = v + e if sg > 0 else v - e
    return u + v if sg > 0 else u - v


def phi3(a):
    l5 = a[0] + a[1]
    return [a[0] + a[3], a[0] - a[1], l5, 0.5 * (l5 + a[3] + a[2])]


def phi4_inv(e, hf=0.5):
    a11 = hf * (e[1] + e[2])
    a12 = e[2] - a11
    return [a11, a12, e[3] - a12, e[0] - a11]


def psi(c, hf):
    h = hf * c[3]
    c11 = h + c[0]
    return [c11, h, (h + c[1]) + c[2], (c11 + c[1]) - c[2]]


def rc(o, p, q):
    return (o // 2) * 4 + (p // 2) * 2 + q // 2, (o % 2) * 4 + (p % 2) * 2 + q % 2


def popc(v):
    return bin(v).count("1")


def scale(br, bc):
    return S3 ** (popc(br) - popc(bc))


def plan():
    groups, n = {}, 0
    for i in range(1, 8):
        for j in range(1, 8):
            plain = i == 1 or j == 1
            groups[(i, j)] = (n, plain)
            n += 4 if plain else 7
    return groups, n


def cat(xs, axis):
    return jnp.concatenate(list(xs), axis=axis)


def rows(x, p):
    return x[p * R:(p + 1) * R]


def cols(x, q):
    return x[:, q * Q:(q + 1) * Q]


class Sched:
    def __init__(self, it, opt):
        self.it, self.opt = it, opt
        self.q, self.bg, self.lock = [], [], None
        self.g, self.t, self.pace, self.bcredit = None, 0, 0.0, 0.0

    def gated(self, gates, v):
        shape = (len(gates) * SR, len(gates[0]) * Q)
        if all(g is None for r in gates for g in r):
            return v
        if not isinstance(v, jax.Array):
            v = jnp.full(shape, v, f32)
        g = cat([cat([v[i * SR:(i + 1) * SR, j * Q:(j + 1) * Q] if x is None else x for j, x in enumerate(r)], 1)
                 for i, r in enumerate(gates)], 0)
        return jnp.where(jnp.full(shape, self.it, jnp.int32) < 0, g, v)

    def add(self, gen, deadline, cost, bg=False):
        (self.bg if bg else self.q).append([gen, deadline, cost])
        return gen

    def step(self, q, gate=None):
        self.g = gate
        c = None
        while q and c is None:
            c = next(q[0][0], None)
            if c is None:
                q.pop(0)
        if c is not None:
            self.lock = None if isinstance(c, float) else q
            q[0][2] -= c
        self.g = None
        return c

    def tick(self, val, base, brate):
        rate, cum = base, 0.0
        for _, dl, cost in self.q:
            cum += max(cost, 0)
            rate = max(rate, cum / max(dl - self.opt["margin"] - self.t, 1))
        self.bcredit = min(self.bcredit + brate + (0.0 if self.q else base), 40.0)
        self.pace = min(self.pace + rate + (brate if self.bg else 0.0), 40.0)
        if self.pace > 0:
            if self.lock:
                q = self.lock
            elif self.bg and (not self.q or (self.bcredit > 0 and rate <= base)):
                q = self.bg
            else:
                q = self.q
            if q:
                r = self.opt["row"]
                c = self.step(q, val[r * SR:(r + 1) * SR])
                if c:
                    self.pace -= c
                    if q is self.bg:
                        self.bcredit -= c
        self.t += 1

    def drain(self, gen=None, bg=False):
        q = self.bg if bg else self.q
        while q and (gen is None or any(e[0] is gen for e in q)):
            self.step(q)


def load_panel(get, o, p):
    return cat([get(br, bc * Q, (bc + 1) * Q).astype(f32) for br, bc in (rc(o, p, q) for q in range(4))], 1)


def load_z(ref):
    get = lambda br, c0, c1: ref[br * R:(br + 1) * R, c0:c1]
    return [[load_panel(get, o, p) for p in range(4)] for o in range(4)]


def rescale(x, f):
    return cat([cols(x, q) if f(q) == 1.0 else cols(x, q) * f(q) for q in range(4)], 1)


def to_basis(dd, x=None, e=None):
    d = cat(phi3(dd), 0)
    return cat([comb2(cols(d, i), sg, cols(d, j), None if x is None else cols(x, b), None if e is None else cols(e, b))
                for b, (i, sg, j) in enumerate(PHI4)], 1)


def basis1(v):
    d1, d0 = to_basis(v[1]), to_basis(v[0])
    return [to_basis(v[3], d0), d0 - d1, d0 + d1, to_basis(v[2], d1)]


def head(S, z, hs_ref, dl):
    def job():
        g = {o: [[None] * 4 for _ in range(NS)] for o in range(4)}
        for s in range(NS):
            for o in (1, 2, 0, 3):
                for q in QORD:
                    g[o][s][q] = S.g
                    if (s, o, q) == (NS - 1, 3, QORD[-1]):
                        v = [[rescale(z[o][p], lambda q: scale(*rc(o, p, q))) for p in range(4)] for o in range(4)]
                        for b, x in enumerate(basis1([[S.gated(g[o], v[o][0])] + v[o][1:] for o in range(4)])):
                            hs_ref[b] = x
                    yield 22.0 if q == QORD[-1] else 22

    return S.add(job(), dl, 16 * NS * 22)


def cross(S, dl, o, terms, z, bt_ref, l, emit=None, xo=None, out=None, peak=None):
    last = emit is None
    qord = TORD if last else QORD
    post = {1: 23, 0: 13, 3: 13, 2: 13} if last else {q: (4 if o < 2 else 12) * n for q, n in zip(QORD, (0, 1, 2, 1))}
    cost = {q: 17 + 4 * len(terms) + post[q] for q in qord}

    def finish(g1, g2):
        c = chain([(sg, m()) for sg, m in terms])
        y = psi([rows(c, p) for p in range(4)], S.gated(g1, 0.5))
        if peak is not None and o in (0, 3):
            sq = [cols(y[p], q) * cols(y[p], q) for q in (0, 3) for p in (0, 3)]
            sq = jnp.maximum(jnp.maximum(sq[0], sq[1]), jnp.maximum(sq[2], sq[3]))
            peak[o // 3] = functools.reduce(lambda a, b: jnp.maximum(b, a), [sq[s * SR:(s + 1) * SR] for s in range(NS)])
        bias = lambda br, c0, c1: bt_ref[l * 4 + popc(br), :, c0:c1]
        dd = [(y[p] + cat([load_panel(bias, o, p)] * NS, 0)) * z[p] for p in range(4)]
        if not last:
            return emit(dd)
        x = xo()
        x = cat(phi4_inv([cols(x, q) for q in range(4)]), 1)
        e = [rows(x, p) for p in range(4)]
        a11 = S.gated(g2, 0.5) * (e[1] + e[2])
        a22 = e[0] - a11
        xn = [a11, e[2] - a11, ((e[3] - a22) + e[3]) - e[2], a22]
        for p in range(4):
            r = rescale(dd[p] + xn[p], lambda q: 1.0 / scale(*rc(o, p, q)))
            br, bc = rc(o, p, 0)
            for t in range(2):
                out[(br + t) * R:(br + t + 1) * R, bc * Q:(bc + 2) * Q] = r[:, 2 * t * Q:2 * (t + 1) * Q].astype(bf16)

    def job():
        g1, g2 = ([[None] * 4 for _ in range(NS)] for _ in range(2))
        for s in range(NS):
            yield 1
            yield 1
            for q in qord:
                cc = cost[q]
                g1[s][q] = S.g
                if last:
                    cc = cost[q] // 2
                    yield cost[q] - cc
                    g2[s][q] = S.g
                if (s, q) == (NS - 1, qord[-1]):
                    finish(g1, g2)
                yield float(cc) if q == qord[-1] else cc

    return S.add(job(), dl, NS * (2 + sum(cost.values())), bg=last)


def tail(S, z, bt_ref, out, peak, ts_ref, L, quads=(0, 1, 2, 3)):
    for o in quads:
        g = cross(S, 0, o, [(sg, functools.partial(lambda n: ts_ref[n], 4 + NAMES.index(n))) for sg, n in TERMS[o]],
                  z[o], bt_ref, L - 1, xo=functools.partial(lambda n: ts_ref[n], o), out=out, peak=peak)
    return g


def unbasis1(S, X, ts_ref):
    g = [[None] * 2 for _ in range(4 * NS)]
    for s in range(NS):
        for p in range(4):
            for t in range(2):
                g[p * NS + s][t] = S.g
                if (s, p, t) == (NS - 1, 3, 1):
                    hf = S.gated(g, 0.5)
                    if isinstance(hf, jax.Array):
                        hf = cat([cols(hf, q // 2) for q in range(4)], 1)
                    for o, x in enumerate(phi4_inv([X[b]() for b in range(4)], hf)):
                        ts_ref[o] = x
                yield S.opt["ic"]


def level3(mul, order):
    need = {"v": {1: 1, 3: 1, 5: -1}, 1: {3: 1, 5: 1}, 0: {"v": 1, 4: 1, 7: 1}, 3: {"v": 1, 6: 1, 2: -1},
            2: {"h": 1, 4: 1, 7: -1, 6: 1, 2: 1}}
    acc = {n: None for n in need}
    left = {n: set(t) for n, t in need.items()}
    for k in order:
        todo = [(k, mul(k))]
        while todo:
            name, v = todo.pop(0)
            for n, t in need.items():
                if name in left[n]:
                    left[n].discard(name)
                    acc[n] = sadd(acc[n], (t[name], v))
                    if not left[n] and n in ("v", 1):
                        todo.append(("v" if n == "v" else "h", acc[n][1]))
    assert all(a[0] > 0 for a in acc.values())
    return cat([acc[q][1] for q in range(4)], 1)


def level2(mul):
    c0 = mul(1)
    m4 = mul(4)
    c0 = m4 + c0
    c2 = mul(2) + m4
    m7 = mul(7)
    c0 = m7 + c0
    c1 = mul(6) - m7
    m5 = mul(5)
    c0 = c0 - m5
    return cat([c0, c1, c2, mul(3) + m5], 0)


def body(it, x_prev, x_cur, x_next, out, pk_ref, bt_ref, t_ref, hs_ref, ts_ref, L, groups, opt):
    S = Sched(it, opt)
    cum = [0]
    for i in ORDER1:
        cum.append(cum[-1] + sum(8 if groups[(i, j)][1] else 7 for j in range(1, 8)))
    TL, mg = cum[-1], opt["margin"]
    z = load_z(x_cur)
    X = {b: hs_ref[b] for b in range(4)}
    pre = [10 * opt["pre"]]
    need = None
    tl = tail(S, load_z(x_prev), bt_ref, out, pk_ref.at[it - 1, 1], ts_ref, L)

    for l in range(L):
        T0 = l * TL
        last = l == L - 1

        def dot(u, n):
            return jnp.dot(u, t_ref[l, n // 2, :, (n % 2) * Q:(n % 2 + 1) * Q], preferred_element_type=f32)

        def level1(i):
            base = opt["rates%d" % l][ORDER1.index(i)]
            brate = opt.get("brates%d" % l, opt["brates"])[ORDER1.index(i)]

            def group(j):
                a = lin([(s1 * s2, rows(X[b1], b2)) for s1, b1 in CORE4[i] for s2, b2 in CORE3[j]])
                a = [cols(a, q) for q in range(4)]
                n, plain = groups[(i, j)]
                if plain:
                    an = phi4_inv(a)
                    k0 = cat([an[0], an[2]], 0).astype(bf16)
                    k1 = cat([an[1], an[3]], 0).astype(bf16)

                    def mul2(u, k):
                        r = dot(u, n + k)
                        S.tick(r[:R], base, brate)
                        S.tick(r[R:], base, brate)
                        return r

                    c0 = mul2(k0, 0) + mul2(k1, 2)
                    c1 = mul2(k0, 1) + mul2(k1, 3)
                    return cat([c0[:R], c1[:R], c0[R:], c1[R:]], 1)

                def mul(k):
                    u = lin([(s3, a[b]) for s3, b in CORE4[k]])
                    if len(CORE4[k]) == 2:
                        for r0 in (0, 2 * SR):
                            if pre[0] > 0:
                                S.step(S.bg, u[r0:r0 + SR])
                                pre[0] -= 1
                    r = dot(u.astype(bf16), n + k - 1)
                    S.tick(r, base, brate)
                    return r

                return level3(mul, opt["od%d" % l])

            return level2(group)

        XN, D, M, nn = {}, {}, {}, {}

        def emitter(o, X=X, XN=XN, D=D):
            def emit(dd):
                if o < 2:
                    D[o] = to_basis(dd)
                if o == 0:
                    XN[1] = (D[0] + X[1]) - D[1]
                    XN[2] = (D[0] + X[2]) + D[1]
                elif o == 3:
                    XN[0] = to_basis(dd, X[0], D[0])
                elif o == 2:
                    XN[3] = to_basis(dd, X[3], D[1])
            return emit

        def keep(name, m):
            M[name] = m
            if last:
                ts_ref[4 + NAMES.index(name)] = m

        def add(o, dl):
            if not last:
                nn[o] = cross(S, dl, o, [(sg, functools.partial(M.get, n)) for sg, n in TERMS[o]], z[o], bt_ref, l,
                              emit=emitter(o), peak=pk_ref.at[it, 0] if l == 0 else None)

        if last:
            S.drain(tl, bg=True)
        if need:
            S.drain(need[0])
        m3 = level1(3)
        m5 = level1(5)
        if last:
            S.add(unbasis1(S, [functools.partial(X.get, b) for b in range(4)], ts_ref), T0 + TL + opt["endm"],
                  NS * 8 * opt["ic"])
            head(S, load_z(x_next), hs_ref, T0 + TL + opt["endm"])
        keep("h", m5 + m3)
        v = m3 - m5
        add(1, T0 + cum[5] + mg)
        if need:
            S.drain(need[3])
        keep("v", level1(1) + v)
        keep("m4", level1(4))
        keep("m7", level1(7))
        add(0, T0 + TL)
        if need:
            S.drain(need[2])
        keep("m6", level1(6))
        keep("m2", level1(2))
        add(3, T0 + TL + cum[2])
        add(2, T0 + TL + cum[5])
        need, X = nn, XN
    S.drain()


def tform(e, k):
    if k == 1:
        return e[0] + e[0]
    return lin([(s, e[b]) for s, b in CORE4[SIGMA[k]]])


def table_job(S, w_ref, tb_ref, l, groups):
    ga = {o: [[None] * 4 for _ in range(Q // SR)] for o in range(4)}
    gb = {(i, b): [None] * (Q // CR) for i in range(1, 8) for b in range(4)}
    js = {b: [j for j in range(1, 8) if max(t for _, t in CORE3[SIGMA[j]]) == b] for b in range(4)}
    for c in range(Q // CR):
        for s in range(c * CR // SR, (c + 1) * CR // SR):
            for o in (1, 2, 0, 3):
                for q in QORD:
                    ga[o][s][q] = S.g
                    yield 23
        for i in range(1, 8):
            for b in range(4):
                gb[(i, b)][c] = S.g
                yield 16 + 21 * len(js[b])
    v = []
    for o in range(4):
        w = [load_panel(lambda br, c0, c1: w_ref[br, :, c0:c1], o, p) for p in range(4)]
        sc = cat([jnp.full((Q, Q), 0.25 * scale(*rc(o, 0, q)), f32) for q in range(4)], 1)
        v.append([w[0] * S.gated(ga[o], sc)]
                 + [rescale(w[p], lambda q: 0.25 * scale(*rc(o, p, q))) for p in range(1, 4)])
    E = basis1(v)
    for i in range(1, 8):
        if i == 1:
            two = S.gated([[gb[(i, b)][c]] for b in range(4) for c in range(Q // CR)], 2.0)
            two = cat([two[t // 2 * SR:(t // 2 + 1) * SR] for t in range(4 * Q // SR)], 0)
            s1 = cat([two] * 4, 1) * E[0]
        else:
            first = CORE4[SIGMA[i]][0][1]
            g = [[gb[(i, b)][s * SR // CR]] * 4 for b in range(4) for s in range(Q // SR)]
            s1 = tform([S.gated(g, E[b]) if b == first else E[b] for b in range(4)], i)
        for j in range(1, 8):
            e = lin([(sg, s1[b * Q:(b + 1) * Q]) for sg, b in CORE3[SIGMA[j]]])
            e = [cols(e, q) for q in range(4)]
            n, plain = groups[(i, j)]
            if plain:
                a, b = e[1] + e[2], e[2] - e[1]
                outs = [a, b, (e[3] - b) + e[3], (e[0] - a) + e[0]]
            else:
                outs = [tform(e, k) for k in range(1, 8)]
            for k, t in enumerate(outs):
                c0 = ((n + k) % 2) * Q
                tb_ref.at[l, (n + k) // 2][:, c0:c0 + Q] = t.astype(bf16)


def first_layer(l, w_ref, z_ref, xi_ref, xo_ref, pr_ref, wn_ref, bt_ref, tb_ref, groups, opt):
    S = Sched(l, opt)
    S.add(table_job(S, w_ref, tb_ref, l, groups), 0, 0)
    rate = (Q // CR) * (32 * 23 + 7 * (4 * 16 + 7 * 21)) / (16 * TM // SR)
    pace = 0.0
    x = xi_ref[...]
    xb = cat([x, pr_ref[...]], 0).astype(bf16)
    wn = None
    for n in range(8):
        cs = slice(n * Q, (n + 1) * Q)
        acc = None
        for kh in range(2):
            rs = [jnp.dot(cols(xb, k), w_ref[k, :, cs], preferred_element_type=f32) for k in range(4 * kh, 4 * kh + 4)]
            oth = (rs[1] + rs[2]) + rs[3]
            acc = oth if acc is None else acc + oth
            for g in range(TM // SR):
                pace += rate
                for r in (rs[0], rs[3]):
                    if pace > 0:
                        pace -= S.step(S.q, r[g * SR:(g + 1) * SR]) or 0
            acc = acc + rs[0]
        xo_ref[:, cs] = z_ref[:, cs] * (acc[:TM] + bt_ref[l * 4 + popc(n), 0:1, cs]) + x[:, cs]
        wn = acc[TM:] * acc[TM:] if wn is None else wn + acc[TM:] * acc[TM:]
    wn_ref[l] = wn
    S.drain()


def kernel(x_hbm, w_hbm, b_hbm, o_hbm, t_ref, bt_ref, hs_ref, ts_ref, xs_ref, w_buf, x_buf, o_buf, o0_buf, b_buf,
           pr_ref, wn_ref, pk_ref, w_sem, x_sem, o_sem, m_sem, *, L, nb, groups, opt):
    D = 8 * Q

    def wcopy(l):
        return pltpu.make_async_copy(w_hbm.at[l], w_buf.at[l], w_sem.at[l & 1])

    def xcopy(i, n=1):
        return pltpu.make_async_copy(x_hbm.at[pl.ds(i, n)], x_buf.at[pl.ds(i, n)], x_sem.at[4 + i])

    def gcopy(g):
        return pltpu.make_async_copy(x_hbm.at[pl.ds(g * XG, XG)], x_buf.at[pl.ds((g & 3) * XG, XG)], x_sem.at[g & 3])

    def ocopy(i):
        return pltpu.make_async_copy(o_buf.at[i & (NO - 1)], o_hbm.at[pl.ds(pl.multiple_of(i * TM, TM), TM), :],
                                     o_sem.at[i & (NO - 1)])

    bcopy = pltpu.make_async_copy(b_hbm, b_buf, m_sem.at[0])
    bcopy.start()
    xcopy(0).start()
    wcopy(0).start()
    ts_ref[...] = jnp.zeros(ts_ref.shape, f32)
    bcopy.wait()
    b = b_buf[...].astype(f32)
    for e in range(4):
        be = cat([cols(b, bc) * S3 ** (e - popc(bc)) for bc in range(8)], 1)
        for l in range(L):
            bt_ref[l * 4 + e] = jnp.broadcast_to(be[l:l + 1], (SR, 8 * Q))
    hsh = (jax.lax.broadcasted_iota(jnp.int32, (NP, D), 0) * D + jax.lax.broadcasted_iota(jnp.int32, (NP, D), 1))
    for _ in range(2):
        hsh = (hsh ^ (hsh >> 15)) * 739982445
    pr_ref[...] = jnp.where((hsh ^ (hsh >> 15)) & 256 == 0, 1.0, -1.0)
    xcopy(0).wait()
    xs_ref[0] = x_buf[0].astype(f32)
    xs_ref[2] = x_buf[0].astype(f32)
    tb_ref = t_ref.bitcast(bf16)
    wcopy(0).wait()

    def first(l, carry):
        nxt = wcopy(jnp.minimum(l + 1, L - 1))
        pl.when(l + 1 < L)(nxt.start)

        @pl.when(l + 1 == L)
        def _():
            xcopy(1).start()
            xcopy(2).start()

        first_layer(l, w_buf.at[l], xs_ref.at[2], xs_ref.at[l & 1], xs_ref.at[1 - (l & 1)], pr_ref, wn_ref, bt_ref,
                    tb_ref, groups, opt)
        pl.when(l + 1 < L)(nxt.wait)
        return carry

    jax.lax.fori_loop(0, L, first, 0)
    o0_buf[...] = xs_ref[L % 2].astype(bf16)
    o0copy = pltpu.make_async_copy(o0_buf, o_hbm.at[pl.ds(0, TM), :], m_sem.at[1])
    o0copy.start()
    xcopy(1).wait()
    S = Sched(None, opt)
    head(S, load_z(x_buf.at[1]), hs_ref, 0)
    S.drain()

    def dmas(i):
        g, ng = (i + 1) >> 3, nb // XG
        turn = ((i + 1) & (XG - 1)) == 0
        cps = [gcopy(jnp.minimum(g + 1, ng - 1)), ocopy(jnp.maximum(i - 2, 1)),
               gcopy(jnp.minimum(g, ng - 1)), ocopy(jnp.maximum(i - 3, 1))]
        pl.when(turn & (g + 1 < ng))(cps[0].start)
        pl.when(i >= 3)(cps[1].start)
        pl.when(turn & (g < ng))(cps[2].wait)
        pl.when(i == 2)(xcopy(3, XG - 3).wait)
        pl.when(i >= 4)(cps[3].wait)

    def step(i, carry):
        xs = [x_buf.at[jnp.clip(i + u, 0, nb - 1) & (NX - 1)] for u in (-1, 0, 1)]
        body(i, *xs, o_buf.at[(i + 1) & (NO - 1)], pk_ref, bt_ref, tb_ref, hs_ref, ts_ref, L, groups, opt)
        dmas(i + 1)
        return carry

    xcopy(2).wait()
    xcopy(3, XG - 3).start()
    gcopy(1).start()
    jax.lax.fori_loop(1, nb, step, 0)

    last, H = nb - 1, TM // 2
    z = load_z(x_buf.at[last % NX])
    halves = [pltpu.make_async_copy(o_buf.at[last % NO, pl.ds(h * H, H), :],
                                    o_hbm.at[pl.ds(last * TM + h * H, H), :], m_sem.at[2 + h]) for h in range(2)]
    S = Sched(None, opt)
    for h in range(2):
        tail(S, z, bt_ref, o_buf.at[last % NO], pk_ref.at[last, 1], ts_ref, L, (2 * h, 2 * h + 1))
        S.drain(bg=True)
        halves[h].start()
    o0copy.wait()
    ocopy(last - 1).wait()

    wn = [jnp.sum(jnp.sum(wn_ref[l], axis=0, keepdims=True), axis=1, keepdims=True) for l in range(L)]
    tot = functools.reduce(lambda a, b: a + b, wn) * (1.0 / Q)
    gain = [tot / wn[0], tot / wn[L - 1]]

    def risky(i, n):
        pk = [jnp.maximum(pk_ref[pl.ds(i, n), t, 0], pk_ref[pl.ds(i, n), t, 1]).reshape(n * SR, Q) * gain[t]
              for t in range(2)]
        return jnp.logical_not(jnp.max(jnp.sum(jnp.maximum(pk[0], pk[1]), axis=1, keepdims=True)) <= opt["limit"])

    redo = risky(1, last)
    for h in range(2):
        halves[h].wait()

    def chunk(c, carry):
        rs = pl.ds(pl.multiple_of(c * R, R), R)
        z = o0_buf[rs, :].astype(f32)

        def layer(l, x):
            y = jnp.dot(x.astype(bf16), w_buf[l].reshape(D, D), preferred_element_type=f32)
            b = cat([bt_ref[l * 4 + popc(n), 0:1, n * Q:(n + 1) * Q] for n in range(8)], 1)
            return z * (y + b) + x

        o0_buf[rs, :] = jax.lax.fori_loop(0, L, layer, z).astype(bf16)
        return carry

    def again(i, carry):
        @pl.when(risky(i, 1))
        def _():
            cp = pltpu.make_async_copy(x_hbm.at[i], o0_buf, m_sem.at[0])
            cp.start()
            cp.wait()
            jax.lax.fori_loop(0, TM // R, chunk, 0)
            cp = pltpu.make_async_copy(o0_buf, o_hbm.at[pl.ds(pl.multiple_of(i * TM, TM), TM), :], m_sem.at[0])
            cp.start()
            cp.wait()

        return carry

    @pl.when(redo)
    def _():
        jax.lax.fori_loop(1, nb, again, 0)


def make(o=None):
    opt = dict(OPT)
    opt.update(o or {})
    groups, n = plan()

    @jax.jit
    def run(x0, ws, bs):
        B, D = x0.shape
        L = ws.shape[0]
        assert D == 8 * Q and B % (XG * TM) == 0 and B >= 2 * XG * TM and L == 6 and n % 2 == 0
        return pl.pallas_call(
            functools.partial(kernel, L=L, nb=B // TM, groups=groups, opt=opt),
            in_specs=[pl.BlockSpec(memory_space=pl.ANY)] * 3,
            out_specs=pl.BlockSpec(memory_space=pl.ANY),
            out_shape=jax.ShapeDtypeStruct((B, D), x0.dtype),
            scratch_shapes=[
                pltpu.VMEM((L, n // 2, Q // 2, 2 * Q), jnp.uint32),
                pltpu.VMEM((L * 4, SR, D), f32),
                pltpu.VMEM((4, 4 * R, D // 2), f32),
                pltpu.VMEM((10, 4 * R, D // 2), f32),
                pltpu.VMEM((3, TM, D), f32),
                pltpu.VMEM((L, 8, Q, D), bf16),
                pltpu.VMEM((NX, TM, D), bf16),
                pltpu.VMEM((NO, TM, D), bf16),
                pltpu.VMEM((TM, D), bf16),
                pltpu.VMEM((L, D), bf16),
                pltpu.VMEM((NP, D), f32),
                pltpu.VMEM((L, NP, Q), f32),
                pltpu.VMEM((B // TM, 2, 2, SR, Q), f32),
                pltpu.SemaphoreType.DMA((2,)),
                pltpu.SemaphoreType.DMA((8,)),
                pltpu.SemaphoreType.DMA((NO,)),
                pltpu.SemaphoreType.DMA((4,)),
            ],
            compiler_params=pltpu.CompilerParams(vmem_limit_bytes=116 * 1024 * 1024, disable_bounds_checks=True),
        )(x0.reshape(B // TM, TM, D), ws.reshape(L, 8, Q, D), bs)

    return run


_run = make()


@jax.jit
def pallas_standalone__dcn_v2_cross__recsys_kernel(x0: jax.Array, ws: jax.Array, bs: jax.Array):
    return _run(x0, ws, bs)
```

```python
import functools
import math

import jax
import jax.numpy as jnp
import jax.experimental.pallas as pl
import jax.experimental.pallas.tpu as pltpu

f32 = jnp.float32
bf16 = jnp.bfloat16

Q = 128
R = 32
SR = 8
NS = R // SR
TM = 8 * R
CR = 16
XG = 8
NX = 4 * XG
NO = 2
NP = 16
S3 = math.sqrt(3.0)

CORE3 = {1: [(1, 0)], 3: [(1, 1)], 5: [(1, 2)], 2: [(1, 3)],
         4: [(1, 0), (-1, 1)], 7: [(1, 2), (-1, 0)], 6: [(1, 3), (-1, 0)]}
CORE4 = {1: [(1, 0)], 3: [(1, 1)], 5: [(1, 2)], 2: [(1, 3), (1, 0)],
         4: [(1, 0), (-1, 1)], 7: [(1, 2), (-1, 0)], 6: [(1, 3), (-1, 0)]}
SIGMA = {1: 1, 2: 3, 3: 7, 4: 6, 5: 4, 6: 5, 7: 2}
ORDER1 = [3, 5, 1, 4, 7, 6, 2]
QORD = [2, 1, 0, 3]
TORD = [1, 0, 3, 2]
PHI4 = [(3, 1, 0), (0, -1, 1), (0, 1, 1), (1, 1, 2)]
NAMES = ["h", "v", "m4", "m7", "m6", "m2"]
TERMS = {1: [(1, "h")], 0: [(1, "m7"), (1, "v"), (1, "m4")], 3: [(1, "v"), (-1, "m2"), (1, "m6")],
         2: [(1, "m2"), (1, "m6"), (1, "h"), (1, "m4"), (-1, "m7")]}

LIMIT = 6.0

OPT = dict(
    pc=[26, 18, 21], pres=0, pg=1, pi=[1, 6, 2, 3, 4, 5, 7],
    limit=LIMIT, row=2, margin=27, pre=2, ic=18.0, endm=25,
    rates0=[9.2, 9.4, 10, 5.4, 6.8, 5.5, 5.4], rates1=[9.2, 5.4, 11.5, 4.6, 6.6, 5.5, 5.4],
    rates2=[9.2, 7, 11.5, 5.9, 4.2, 5.5, 5.4], rates3=[9.2, 7, 11.5, 6.0, 6.7, 5.5, 5.4],
    rates4=[9.2, 7, 11.5, 5.5, 4.8, 5.5, 5.3], rates5=[9.2, 7, 12.4, 4.3, 6.9, 5.5, 5.4],
    brates=[2.0] * 7, brates0=[2.0, 2.9, 1.0, 2.0, 3.0, 2.0, 3.0], brates1=[2.1, 2.0, 2.0, 2.0, 2.0, 2.0, 2.0],
    od0=[3, 4, 5, 1, 7, 2, 6], od1=[3, 4, 5, 1, 7, 6, 2], od2=[3, 4, 5, 1, 7, 2, 6],
    od3=[3, 4, 1, 5, 6, 2, 7], od4=[3, 6, 1, 5, 7, 2, 4], od5=[3, 4, 5, 1, 7, 6, 2])


def lin(terms):
    pos = [v for s, v in terms if s > 0]
    neg = [v for s, v in terms if s < 0]
    acc = pos[0]
    for v in pos[1:]:
        acc = acc + v
    for v in neg:
        acc = acc - v
    return acc


def chain(terms):
    acc = terms[0][1]
    for s, v in terms[1:]:
        acc = acc + v if s > 0 else acc - v
    return acc


def sadd(a, b):
    if a is None:
        return b
    if a[0] == b[0]:
        return (a[0], b[1] + a[1])
    return (1, a[1] - b[1]) if a[0] > 0 else (1, b[1] - a[1])


def comb2(u, sg, v, x=None, e=None):
    if x is not None:
        u = u + x
    if e is not None:
        v = v + e if sg > 0 else v - e
    return u + v if sg > 0 else u - v


def phi3(a):
    l5 = a[0] + a[1]
    return [a[0] + a[3], a[0] - a[1], l5, 0.5 * (l5 + a[3] + a[2])]


def phi4_inv(e, hf=0.5):
    a11 = hf * (e[1] + e[2])
    a12 = e[2] - a11
    return [a11, a12, e[3] - a12, e[0] - a11]


def psi(c, hf):
    h = hf * c[3]
    c11 = h + c[0]
    return [c11, h, (h + c[1]) + c[2], (c11 + c[1]) - c[2]]


def rc(o, p, q):
    return (o // 2) * 4 + (p // 2) * 2 + q // 2, (o % 2) * 4 + (p % 2) * 2 + q % 2


def popc(v):
    return bin(v).count("1")


def scale(br, bc):
    return S3 ** (popc(br) - popc(bc))


def plan():
    groups, n = {}, 0
    for i in range(1, 8):
        for j in range(1, 8):
            plain = i == 1 or j == 1
            groups[(i, j)] = (n, plain)
            n += 4 if plain else 7
    return groups, n


def cat(xs, axis):
    return jnp.concatenate(list(xs), axis=axis)


def rows(x, p):
    return x[p * R:(p + 1) * R]


def cols(x, q):
    return x[:, q * Q:(q + 1) * Q]


class Sched:
    def __init__(self, it, opt):
        self.it, self.opt = it, opt
        self.q, self.bg, self.lock = [], [], None
        self.g, self.t, self.pace, self.bcredit = None, 0, 0.0, 0.0

    def gated(self, gates, v):
        shape = (len(gates) * SR, len(gates[0]) * Q)
        if all(g is None for r in gates for g in r):
            return v
        if not isinstance(v, jax.Array):
            v = jnp.full(shape, v, f32)
        g = cat([cat([v[i * SR:(i + 1) * SR, j * Q:(j + 1) * Q] if x is None else x for j, x in enumerate(r)], 1)
                 for i, r in enumerate(gates)], 0)
        return jnp.where(jnp.full(shape, self.it, jnp.int32) < 0, g, v)

    def add(self, gen, deadline, cost, bg=False):
        (self.bg if bg else self.q).append([gen, deadline, cost])
        return gen

    def step(self, q, gate=None):
        self.g = gate
        c = None
        while q and c is None:
            c = next(q[0][0], None)
            if c is None:
                q.pop(0)
        if c is not None:
            self.lock = None if isinstance(c, float) else q
            q[0][2] -= c
        self.g = None
        return c

    def tick(self, val, base, brate):
        rate, cum = base, 0.0
        for _, dl, cost in self.q:
            cum += max(cost, 0)
            rate = max(rate, cum / max(dl - self.opt["margin"] - self.t, 1))
        self.bcredit = min(self.bcredit + brate + (0.0 if self.q else base), 40.0)
        self.pace = min(self.pace + rate + (brate if self.bg else 0.0), 40.0)
        if self.pace > 0:
            if self.lock:
                q = self.lock
            elif self.bg and (not self.q or (self.bcredit > 0 and rate <= base)):
                q = self.bg
            else:
                q = self.q
            if q:
                r = self.opt["row"]
                c = self.step(q, val[r * SR:(r + 1) * SR])
                if c:
                    self.pace -= c
                    if q is self.bg:
                        self.bcredit -= c
        self.t += 1

    def drain(self, gen=None, bg=False):
        q = self.bg if bg else self.q
        while q and (gen is None or any(e[0] is gen for e in q)):
            self.step(q)


def load_panel(get, o, p):
    return cat([get(br, bc * Q, (bc + 1) * Q).astype(f32) for br, bc in (rc(o, p, q) for q in range(4))], 1)


def load_z(ref):
    get = lambda br, c0, c1: ref[br * R:(br + 1) * R, c0:c1]
    return [[load_panel(get, o, p) for p in range(4)] for o in range(4)]


def rescale(x, f):
    return cat([cols(x, q) if f(q) == 1.0 else cols(x, q) * f(q) for q in range(4)], 1)


def to_basis(dd, x=None, e=None):
    d = cat(phi3(dd), 0)
    return cat([comb2(cols(d, i), sg, cols(d, j), None if x is None else cols(x, b), None if e is None else cols(e, b))
                for b, (i, sg, j) in enumerate(PHI4)], 1)


def basis1(v):
    d1, d0 = to_basis(v[1]), to_basis(v[0])
    return [to_basis(v[3], d0), d0 - d1, d0 + d1, to_basis(v[2], d1)]


def head(S, z, hs_ref, dl):
    def job():
        g = {o: [[None] * 4 for _ in range(NS)] for o in range(4)}
        for s in range(NS):
            for o in (1, 2, 0, 3):
                for q in QORD:
                    g[o][s][q] = S.g
                    if (s, o, q) == (NS - 1, 3, QORD[-1]):
                        v = [[rescale(z[o][p], lambda q: scale(*rc(o, p, q))) for p in range(4)] for o in range(4)]
                        for b, x in enumerate(basis1([[S.gated(g[o], v[o][0])] + v[o][1:] for o in range(4)])):
                            hs_ref[b] = x
                    yield 22.0 if q == QORD[-1] else 22

    return S.add(job(), dl, 16 * NS * 22)


def cross(S, dl, o, terms, z, bt_ref, l, emit=None, xo=None, out=None, peak=None):
    last = emit is None
    qord = TORD if last else QORD
    post = {1: 23, 0: 13, 3: 13, 2: 13} if last else {q: (4 if o < 2 else 12) * n for q, n in zip(QORD, (0, 1, 2, 1))}
    cost = {q: 17 + 4 * len(terms) + post[q] for q in qord}

    def finish(g1, g2):
        c = chain([(sg, m()) for sg, m in terms])
        y = psi([rows(c, p) for p in range(4)], S.gated(g1, 0.5))
        if peak is not None and o in (0, 3):
            sq = [cols(y[p], q) * cols(y[p], q) for q in (0, 3) for p in (0, 3)]
            sq = jnp.maximum(jnp.maximum(sq[0], sq[1]), jnp.maximum(sq[2], sq[3]))
            peak[o // 3] = functools.reduce(lambda a, b: jnp.maximum(b, a), [sq[s * SR:(s + 1) * SR] for s in range(NS)])
        bias = lambda br, c0, c1: bt_ref[l * 4 + popc(br), :, c0:c1]
        dd = [(y[p] + cat([load_panel(bias, o, p)] * NS, 0)) * z[p] for p in range(4)]
        if not last:
            return emit(dd)
        x = xo()
        x = cat(phi4_inv([cols(x, q) for q in range(4)]), 1)
        e = [rows(x, p) for p in range(4)]
        a11 = S.gated(g2, 0.5) * (e[1] + e[2])
        a22 = e[0] - a11
        xn = [a11, e[2] - a11, ((e[3] - a22) + e[3]) - e[2], a22]
        for p in range(4):
            r = rescale(dd[p] + xn[p], lambda q: 1.0 / scale(*rc(o, p, q)))
            br, bc = rc(o, p, 0)
            for t in range(2):
                out[(br + t) * R:(br + t + 1) * R, bc * Q:(bc + 2) * Q] = r[:, 2 * t * Q:2 * (t + 1) * Q].astype(bf16)

    def job():
        g1, g2 = ([[None] * 4 for _ in range(NS)] for _ in range(2))
        for s in range(NS):
            yield 1
            yield 1
            for q in qord:
                cc = cost[q]
                g1[s][q] = S.g
                if last:
                    cc = cost[q] // 2
                    yield cost[q] - cc
                    g2[s][q] = S.g
                if (s, q) == (NS - 1, qord[-1]):
                    finish(g1, g2)
                yield float(cc) if q == qord[-1] else cc

    return S.add(job(), dl, NS * (2 + sum(cost.values())), bg=last)


def tail(S, z, bt_ref, out, peak, ts_ref, L, quads=(0, 1, 2, 3)):
    for o in quads:
        g = cross(S, 0, o, [(sg, functools.partial(lambda n: ts_ref[n], 4 + NAMES.index(n))) for sg, n in TERMS[o]],
                  z[o], bt_ref, L - 1, xo=functools.partial(lambda n: ts_ref[n], o), out=out, peak=peak)
    return g


def unbasis1(S, X, ts_ref):
    g = [[None] * 2 for _ in range(4 * NS)]
    for s in range(NS):
        for p in range(4):
            for t in range(2):
                g[p * NS + s][t] = S.g
                if (s, p, t) == (NS - 1, 3, 1):
                    hf = S.gated(g, 0.5)
                    if isinstance(hf, jax.Array):
                        hf = cat([cols(hf, q // 2) for q in range(4)], 1)
                    for o, x in enumerate(phi4_inv([X[b]() for b in range(4)], hf)):
                        ts_ref[o] = x
                yield S.opt["ic"]


def level3(mul, order):
    need = {"v": {1: 1, 3: 1, 5: -1}, 1: {3: 1, 5: 1}, 0: {"v": 1, 4: 1, 7: 1}, 3: {"v": 1, 6: 1, 2: -1},
            2: {"h": 1, 4: 1, 7: -1, 6: 1, 2: 1}}
    acc = {n: None for n in need}
    left = {n: set(t) for n, t in need.items()}
    for k in order:
        todo = [(k, mul(k))]
        while todo:
            name, v = todo.pop(0)
            for n, t in need.items():
                if name in left[n]:
                    left[n].discard(name)
                    acc[n] = sadd(acc[n], (t[name], v))
                    if not left[n] and n in ("v", 1):
                        todo.append(("v" if n == "v" else "h", acc[n][1]))
    assert all(a[0] > 0 for a in acc.values())
    return cat([acc[q][1] for q in range(4)], 1)


def level2(mul):
    c0 = mul(1)
    m4 = mul(4)
    c0 = m4 + c0
    c2 = mul(2) + m4
    m7 = mul(7)
    c0 = m7 + c0
    c1 = mul(6) - m7
    m5 = mul(5)
    c0 = c0 - m5
    return cat([c0, c1, c2, mul(3) + m5], 0)


def body(it, x_prev, x_cur, x_next, out, pk_ref, bt_ref, t_ref, hs_ref, ts_ref, L, groups, opt):
    S = Sched(it, opt)
    cum = [0]
    for i in ORDER1:
        cum.append(cum[-1] + sum(8 if groups[(i, j)][1] else 7 for j in range(1, 8)))
    TL, mg = cum[-1], opt["margin"]
    z = load_z(x_cur)
    X = {b: hs_ref[b] for b in range(4)}
    pre = [10 * opt["pre"]]
    need = None
    tl = tail(S, load_z(x_prev), bt_ref, out, pk_ref.at[it - 1, 1], ts_ref, L)

    for l in range(L):
        T0 = l * TL
        last = l == L - 1

        def dot(u, n):
            return jnp.dot(u, t_ref[l, n // 2, :, (n % 2) * Q:(n % 2 + 1) * Q], preferred_element_type=f32)

        def level1(i):
            base = opt["rates%d" % l][ORDER1.index(i)]
            brate = opt.get("brates%d" % l, opt["brates"])[ORDER1.index(i)]

            def group(j):
                a = lin([(s1 * s2, rows(X[b1], b2)) for s1, b1 in CORE4[i] for s2, b2 in CORE3[j]])
                a = [cols(a, q) for q in range(4)]
                n, plain = groups[(i, j)]
                if plain:
                    an = phi4_inv(a)
                    k0 = cat([an[0], an[2]], 0).astype(bf16)
                    k1 = cat([an[1], an[3]], 0).astype(bf16)

                    def mul2(u, k):
                        r = dot(u, n + k)
                        S.tick(r[:R], base, brate)
                        S.tick(r[R:], base, brate)
                        return r

                    c0 = mul2(k0, 0) + mul2(k1, 2)
                    c1 = mul2(k0, 1) + mul2(k1, 3)
                    return cat([c0[:R], c1[:R], c0[R:], c1[R:]], 1)

                def mul(k):
                    u = lin([(s3, a[b]) for s3, b in CORE4[k]])
                    if len(CORE4[k]) == 2:
                        for r0 in (0, 2 * SR):
                            if pre[0] > 0:
                                S.step(S.bg, u[r0:r0 + SR])
                                pre[0] -= 1
                    r = dot(u.astype(bf16), n + k - 1)
                    S.tick(r, base, brate)
                    return r

                return level3(mul, opt["od%d" % l])

            return level2(group)

        XN, D, M, nn = {}, {}, {}, {}

        def emitter(o, X=X, XN=XN, D=D):
            def emit(dd):
                if o < 2:
                    D[o] = to_basis(dd)
                if o == 0:
                    XN[1] = (D[0] + X[1]) - D[1]
                    XN[2] = (D[0] + X[2]) + D[1]
                elif o == 3:
                    XN[0] = to_basis(dd, X[0], D[0])
                elif o == 2:
                    XN[3] = to_basis(dd, X[3], D[1])
            return emit

        def keep(name, m):
            M[name] = m
            if last:
                ts_ref[4 + NAMES.index(name)] = m

        def add(o, dl):
            if not last:
                nn[o] = cross(S, dl, o, [(sg, functools.partial(M.get, n)) for sg, n in TERMS[o]], z[o], bt_ref, l,
                              emit=emitter(o), peak=pk_ref.at[it, 0] if l == 0 else None)

        if last:
            S.drain(tl, bg=True)
        if need:
            S.drain(need[0])
        m3 = level1(3)
        m5 = level1(5)
        if last:
            S.add(unbasis1(S, [functools.partial(X.get, b) for b in range(4)], ts_ref), T0 + TL + opt["endm"],
                  NS * 8 * opt["ic"])
            head(S, load_z(x_next), hs_ref, T0 + TL + opt["endm"])
        keep("h", m5 + m3)
        v = m3 - m5
        add(1, T0 + cum[5] + mg)
        if need:
            S.drain(need[3])
        keep("v", level1(1) + v)
        keep("m4", level1(4))
        keep("m7", level1(7))
        add(0, T0 + TL)
        if need:
            S.drain(need[2])
        keep("m6", level1(6))
        keep("m2", level1(2))
        add(3, T0 + TL + cum[2])
        add(2, T0 + TL + cum[5])
        need, X = nn, XN
    S.drain()


def tform(e, k):
    if k == 1:
        return e[0] + e[0]
    return lin([(s, e[b]) for s, b in CORE4[SIGMA[k]]])


def table_job(S, w_ref, tb_ref, l, groups):
    ga = {o: [[None] * 4 for _ in range(Q // SR)] for o in range(4)}
    gb = {(i, b): [None] * (Q // CR) for i in range(1, 8) for b in range(4)}
    js = {b: [j for j in range(1, 8) if max(t for _, t in CORE3[SIGMA[j]]) == b] for b in range(4)}
    for c in range(Q // CR):
        for s in range(c * CR // SR, (c + 1) * CR // SR):
            for o in (1, 2, 0, 3):
                for q in QORD:
                    ga[o][s][q] = S.g
                    yield S.opt["pc"][0]
        for i in S.opt["pi"]:
            for b in range(4):
                gb[(i, b)][c] = S.g
                yield S.opt["pc"][1] + S.opt["pc"][2] * len(js[b])
    v = []
    for o in range(4):
        w = [load_panel(lambda br, c0, c1: w_ref[br, :, c0:c1], o, p) for p in range(4)]
        sc = cat([jnp.full((Q, Q), 0.25 * scale(*rc(o, 0, q)), f32) for q in range(4)], 1)
        v.append([w[0] * S.gated(ga[o], sc)]
                 + [rescale(w[p], lambda q: 0.25 * scale(*rc(o, p, q))) for p in range(1, 4)])
    E = basis1(v)
    for i in range(1, 8):
        if i == 1:
            two = S.gated([[gb[(i, b)][c]] for b in range(4) for c in range(Q // CR)], 2.0)
            two = cat([two[t // 2 * SR:(t // 2 + 1) * SR] for t in range(4 * Q // SR)], 0)
            s1 = cat([two] * 4, 1) * E[0]
        else:
            first = CORE4[SIGMA[i]][0][1]
            g = [[gb[(i, b)][s * SR // CR]] * 4 for b in range(4) for s in range(Q // SR)]
            s1 = tform([S.gated(g, E[b]) if b == first else E[b] for b in range(4)], i)
        for j in range(1, 8):
            e = lin([(sg, s1[b * Q:(b + 1) * Q]) for sg, b in CORE3[SIGMA[j]]])
            e = [cols(e, q) for q in range(4)]
            n, plain = groups[(i, j)]
            if plain:
                a, b = e[1] + e[2], e[2] - e[1]
                outs = [a, b, (e[3] - b) + e[3], (e[0] - a) + e[0]]
            else:
                outs = [tform(e, k) for k in range(1, 8)]
            for k, t in enumerate(outs):
                c0 = ((n + k) % 2) * Q
                tb_ref.at[l, (n + k) // 2][:, c0:c0 + Q] = t.astype(bf16)


def first_layer(l, w_ref, z_ref, xi_ref, xo_ref, pr_ref, wn_ref, bt_ref, tb_ref, groups, opt):
    S = Sched(l, opt)
    S.add(table_job(S, w_ref, tb_ref, l, groups), 0, 0)
    pc = opt["pc"]
    rate = (Q // CR) * (32 * pc[0] + 7 * (4 * pc[1] + 7 * pc[2])) / (16 * TM // SR - opt["pres"])
    pace = 0.0
    x = xi_ref[...]
    xb = cat([x, pr_ref[...]], 0).astype(bf16)
    wn = None
    for n in range(8):
        cs = slice(n * Q, (n + 1) * Q)
        acc = None
        for kh in range(2):
            rs = [jnp.dot(cols(xb, k), w_ref[k, :, cs], preferred_element_type=f32) for k in range(4 * kh, 4 * kh + 4)]
            oth = (rs[1] + rs[2]) + rs[3]
            acc = oth if acc is None else acc + oth
            for g in range(TM // SR):
                pace += rate
                for r in (rs[opt["pg"]], rs[3]):
                    if pace > 0:
                        pace -= S.step(S.q, r[g * SR:(g + 1) * SR]) or 0
            acc = acc + rs[0]
        xo_ref[:, cs] = z_ref[:, cs] * (acc[:TM] + bt_ref[l * 4 + popc(n), 0:1, cs]) + x[:, cs]
        wn = acc[TM:] * acc[TM:] if wn is None else wn + acc[TM:] * acc[TM:]
    wn_ref[l] = wn
    S.drain()


def kernel(x_hbm, w_hbm, b_hbm, o_hbm, t_ref, bt_ref, hs_ref, ts_ref, xs_ref, w_buf, x_buf, o_buf, o0_buf, b_buf,
           pr_ref, wn_ref, pk_ref, w_sem, x_sem, o_sem, m_sem, *, L, nb, groups, opt):
    D = 8 * Q

    def wcopy(l):
        return pltpu.make_async_copy(w_hbm.at[l], w_buf.at[l], w_sem.at[l & 1])

    def xcopy(i, n=1):
        return pltpu.make_async_copy(x_hbm.at[pl.ds(i, n)], x_buf.at[pl.ds(i, n)], x_sem.at[4 + i])

    def gcopy(g):
        return pltpu.make_async_copy(x_hbm.at[pl.ds(g * XG, XG)], x_buf.at[pl.ds((g & 3) * XG, XG)], x_sem.at[g & 3])

    def ocopy(i):
        return pltpu.make_async_copy(o_buf.at[i & (NO - 1)], o_hbm.at[pl.ds(pl.multiple_of(i * TM, TM), TM), :],
                                     o_sem.at[i & (NO - 1)])

    bcopy = pltpu.make_async_copy(b_hbm, b_buf, m_sem.at[0])
    bcopy.start()
    xcopy(0).start()
    wcopy(0).start()
    ts_ref[...] = jnp.zeros(ts_ref.shape, f32)
    bcopy.wait()
    b = b_buf[...].astype(f32)
    for e in range(4):
        be = cat([cols(b, bc) * S3 ** (e - popc(bc)) for bc in range(8)], 1)
        for l in range(L):
            bt_ref[l * 4 + e] = jnp.broadcast_to(be[l:l + 1], (SR, 8 * Q))
    hsh = (jax.lax.broadcasted_iota(jnp.int32, (NP, D), 0) * D + jax.lax.broadcasted_iota(jnp.int32, (NP, D), 1))
    for _ in range(2):
        hsh = (hsh ^ (hsh >> 15)) * 739982445
    pr_ref[...] = jnp.where((hsh ^ (hsh >> 15)) & 256 == 0, 1.0, -1.0)
    xcopy(0).wait()
    xs_ref[0] = x_buf[0].astype(f32)
    xs_ref[2] = x_buf[0].astype(f32)
    tb_ref = t_ref.bitcast(bf16)
    wcopy(0).wait()

    def first(l, carry):
        nxt = wcopy(jnp.minimum(l + 1, L - 1))
        pl.when(l + 1 < L)(nxt.start)

        @pl.when(l + 1 == L)
        def _():
            xcopy(1).start()
            xcopy(2).start()

        first_layer(l, w_buf.at[l], xs_ref.at[2], xs_ref.at[l & 1], xs_ref.at[1 - (l & 1)], pr_ref, wn_ref, bt_ref,
                    tb_ref, groups, opt)
        pl.when(l + 1 < L)(nxt.wait)
        return carry

    jax.lax.fori_loop(0, L, first, 0)
    o0_buf[...] = xs_ref[L % 2].astype(bf16)
    o0copy = pltpu.make_async_copy(o0_buf, o_hbm.at[pl.ds(0, TM), :], m_sem.at[1])
    o0copy.start()
    xcopy(1).wait()
    S = Sched(None, opt)
    head(S, load_z(x_buf.at[1]), hs_ref, 0)
    S.drain()

    def dmas(i):
        g, ng = (i + 1) >> 3, nb // XG
        turn = ((i + 1) & (XG - 1)) == 0
        cps = [gcopy(jnp.minimum(g + 1, ng - 1)), ocopy(jnp.maximum(i - 2, 1)),
               gcopy(jnp.minimum(g, ng - 1)), ocopy(jnp.maximum(i - 3, 1))]
        pl.when(turn & (g + 1 < ng))(cps[0].start)
        pl.when(i >= 3)(cps[1].start)
        pl.when(turn & (g < ng))(cps[2].wait)
        pl.when(i == 2)(xcopy(3, XG - 3).wait)
        pl.when(i >= 4)(cps[3].wait)

    def step(i, carry):
        xs = [x_buf.at[jnp.clip(i + u, 0, nb - 1) & (NX - 1)] for u in (-1, 0, 1)]
        body(i, *xs, o_buf.at[(i + 1) & (NO - 1)], pk_ref, bt_ref, tb_ref, hs_ref, ts_ref, L, groups, opt)
        dmas(i + 1)
        return carry

    xcopy(2).wait()
    xcopy(3, XG - 3).start()
    gcopy(1).start()
    jax.lax.fori_loop(1, nb, step, 0)

    last, H = nb - 1, TM // 2
    z = load_z(x_buf.at[last % NX])
    halves = [pltpu.make_async_copy(o_buf.at[last % NO, pl.ds(h * H, H), :],
                                    o_hbm.at[pl.ds(last * TM + h * H, H), :], m_sem.at[2 + h]) for h in range(2)]
    S = Sched(None, opt)
    for h in range(2):
        tail(S, z, bt_ref, o_buf.at[last % NO], pk_ref.at[last, 1], ts_ref, L, (2 * h, 2 * h + 1))
        S.drain(bg=True)
        halves[h].start()
    o0copy.wait()
    ocopy(last - 1).wait()

    wn = [jnp.sum(jnp.sum(wn_ref[l], axis=0, keepdims=True), axis=1, keepdims=True) for l in range(L)]
    tot = functools.reduce(lambda a, b: a + b, wn) * (1.0 / Q)
    gain = [tot / wn[0], tot / wn[L - 1]]

    def risky(i, n):
        pk = [jnp.maximum(pk_ref[pl.ds(i, n), t, 0], pk_ref[pl.ds(i, n), t, 1]).reshape(n * SR, Q) * gain[t]
              for t in range(2)]
        return jnp.logical_not(jnp.max(jnp.sum(jnp.maximum(pk[0], pk[1]), axis=1, keepdims=True)) <= opt["limit"])

    redo = risky(1, last)
    for h in range(2):
        halves[h].wait()

    def chunk(c, carry):
        rs = pl.ds(pl.multiple_of(c * R, R), R)
        z = o0_buf[rs, :].astype(f32)

        def layer(l, x):
            y = jnp.dot(x.astype(bf16), w_buf[l].reshape(D, D), preferred_element_type=f32)
            b = cat([bt_ref[l * 4 + popc(n), 0:1, n * Q:(n + 1) * Q] for n in range(8)], 1)
            return z * (y + b) + x

        o0_buf[rs, :] = jax.lax.fori_loop(0, L, layer, z).astype(bf16)
        return carry

    def again(i, carry):
        @pl.when(risky(i, 1))
        def _():
            cp = pltpu.make_async_copy(x_hbm.at[i], o0_buf, m_sem.at[0])
            cp.start()
            cp.wait()
            jax.lax.fori_loop(0, TM // R, chunk, 0)
            cp = pltpu.make_async_copy(o0_buf, o_hbm.at[pl.ds(pl.multiple_of(i * TM, TM), TM), :], m_sem.at[0])
            cp.start()
            cp.wait()

        return carry

    @pl.when(redo)
    def _():
        jax.lax.fori_loop(1, nb, again, 0)


def make(o=None):
    opt = dict(OPT)
    opt.update(o or {})
    groups, n = plan()

    @jax.jit
    def run(x0, ws, bs):
        B, D = x0.shape
        L = ws.shape[0]
        assert D == 8 * Q and B % (XG * TM) == 0 and B >= 2 * XG * TM and L == 6 and n % 2 == 0
        return pl.pallas_call(
            functools.partial(kernel, L=L, nb=B // TM, groups=groups, opt=opt),
            in_specs=[pl.BlockSpec(memory_space=pl.ANY)] * 3,
            out_specs=pl.BlockSpec(memory_space=pl.ANY),
            out_shape=jax.ShapeDtypeStruct((B, D), x0.dtype),
            scratch_shapes=[
                pltpu.VMEM((L, n // 2, Q // 2, 2 * Q), jnp.uint32),
                pltpu.VMEM((L * 4, SR, D), f32),
                pltpu.VMEM((4, 4 * R, D // 2), f32),
                pltpu.VMEM((10, 4 * R, D // 2), f32),
                pltpu.VMEM((3, TM, D), f32),
                pltpu.VMEM((L, 8, Q, D), bf16),
                pltpu.VMEM((NX, TM, D), bf16),
                pltpu.VMEM((NO, TM, D), bf16),
                pltpu.VMEM((TM, D), bf16),
                pltpu.VMEM((L, D), bf16),
                pltpu.VMEM((NP, D), f32),
                pltpu.VMEM((L, NP, Q), f32),
                pltpu.VMEM((B // TM, 2, 2, SR, Q), f32),
                pltpu.SemaphoreType.DMA((2,)),
                pltpu.SemaphoreType.DMA((8,)),
                pltpu.SemaphoreType.DMA((NO,)),
                pltpu.SemaphoreType.DMA((4,)),
            ],
            compiler_params=pltpu.CompilerParams(vmem_limit_bytes=116 * 1024 * 1024, disable_bounds_checks=True),
        )(x0.reshape(B // TM, TM, D), ws.reshape(L, 8, Q, D), bs)

    return run


_run = make()


@jax.jit
def pallas_standalone__dcn_v2_cross__recsys_kernel(x0: jax.Array, ws: jax.Array, bs: jax.Array):
    return _run(x0, ws, bs)
```

```python
import functools
import math

import jax
import jax.numpy as jnp
import jax.experimental.pallas as pl
import jax.experimental.pallas.tpu as pltpu

f32 = jnp.float32
bf16 = jnp.bfloat16

Q = 128
R = 32
SR = 8
NS = R // SR
TM = 8 * R
CR = 16
XG = 8
NX = 4 * XG
NO = 2
NP = 16
TW = 19
S3 = math.sqrt(3.0)

CORE3 = {1: [(1, 0)], 3: [(1, 1)], 5: [(1, 2)], 2: [(1, 3)],
         4: [(1, 0), (-1, 1)], 7: [(1, 2), (-1, 0)], 6: [(1, 3), (-1, 0)]}
CORE4 = {1: [(1, 0)], 3: [(1, 1)], 5: [(1, 2)], 2: [(1, 3), (1, 0)],
         4: [(1, 0), (-1, 1)], 7: [(1, 2), (-1, 0)], 6: [(1, 3), (-1, 0)]}
SIGMA = {1: 1, 2: 3, 3: 7, 4: 6, 5: 4, 6: 5, 7: 2}
ORDER1 = [3, 5, 1, 4, 7, 6, 2]
QORD = [2, 1, 0, 3]
TORD = [1, 0, 3, 2]
PHI4 = [(3, 1, 0), (0, -1, 1), (0, 1, 1), (1, 1, 2)]
NAMES = ["h", "v", "m4", "m7", "m6", "m2"]
TERMS = {1: [(1, "h")], 0: [(1, "m7"), (1, "v"), (1, "m4")], 3: [(1, "v"), (-1, "m2"), (1, "m6")],
         2: [(1, "m2"), (1, "m6"), (1, "h"), (1, "m4"), (-1, "m7")]}

LIMIT = 6.0

OPT = dict(
    pc=[26, 18, 21], pres=0, pg=1, pi=[1, 6, 2, 3, 4, 5, 7],
    limit=LIMIT, row=2, margin=27, pre=2, ic=18.0, endm=25,
    rates0=[9.2, 9.4, 10, 5.4, 6.8, 5.5, 5.4], rates1=[9.2, 5.4, 11.5, 4.6, 6.6, 5.5, 5.4],
    rates2=[9.2, 7, 11.5, 5.9, 4.2, 5.5, 5.4], rates3=[9.2, 7, 11.5, 6.0, 6.7, 5.5, 5.4],
    rates4=[9.2, 7, 11.5, 5.5, 4.8, 5.5, 5.3], rates5=[9.2, 7, 12.4, 4.3, 6.9, 5.5, 5.4],
    brates=[2.0] * 7, brates0=[2.0, 2.9, 1.0, 2.0, 3.0, 2.0, 3.0], brates1=[2.1, 2.0, 2.0, 2.0, 2.0, 2.0, 2.0],
    od0=[3, 4, 5, 1, 7, 2, 6], od1=[3, 4, 5, 1, 7, 6, 2], od2=[3, 4, 5, 1, 7, 2, 6],
    od3=[3, 4, 1, 5, 6, 2, 7], od4=[3, 6, 1, 5, 7, 2, 4], od5=[3, 4, 5, 1, 7, 6, 2])


def lin(terms):
    pos = [v for s, v in terms if s > 0]
    neg = [v for s, v in terms if s < 0]
    acc = pos[0]
    for v in pos[1:]:
        acc = acc + v
    for v in neg:
        acc = acc - v
    return acc


def chain(terms):
    acc = terms[0][1]
    for s, v in terms[1:]:
        acc = acc + v if s > 0 else acc - v
    return acc


def sadd(a, b):
    if a is None:
        return b
    if a[0] == b[0]:
        return (a[0], b[1] + a[1])
    return (1, a[1] - b[1]) if a[0] > 0 else (1, b[1] - a[1])


def comb2(u, sg, v, x=None, e=None):
    if x is not None:
        u = u + x
    if e is not None:
        v = v + e if sg > 0 else v - e
    return u + v if sg > 0 else u - v


def phi3(a):
    l5 = a[0] + a[1]
    return [a[0] + a[3], a[0] - a[1], l5, 0.5 * (l5 + a[3] + a[2])]


def phi4_inv(e, hf=0.5):
    a11 = hf * (e[1] + e[2])
    a12 = e[2] - a11
    return [a11, a12, e[3] - a12, e[0] - a11]


def psi(c, hf):
    h = hf * c[3]
    c11 = h + c[0]
    return [c11, h, (h + c[1]) + c[2], (c11 + c[1]) - c[2]]


def rc(o, p, q):
    return (o // 2) * 4 + (p // 2) * 2 + q // 2, (o % 2) * 4 + (p % 2) * 2 + q % 2


def popc(v):
    return bin(v).count("1")


def scale(br, bc):
    return S3 ** (popc(br) - popc(bc))


def plan():
    groups, n = {}, 0
    for i in range(1, 8):
        for j in range(1, 8):
            plain = i == 1 or j == 1
            groups[(i, j)] = (n, plain)
            n += 4 if plain else 7
    return groups, n


def cat(xs, axis):
    return jnp.concatenate(list(xs), axis=axis)


def rows(x, p):
    return x[p * R:(p + 1) * R]


def cols(x, q):
    return x[:, q * Q:(q + 1) * Q]


class Sched:
    def __init__(self, it, opt):
        self.it, self.opt = it, opt
        self.q, self.bg, self.lock = [], [], None
        self.g, self.t, self.pace, self.bcredit = None, 0, 0.0, 0.0

    def gated(self, gates, v):
        shape = (len(gates) * SR, len(gates[0]) * Q)
        if all(g is None for r in gates for g in r):
            return v
        if not isinstance(v, jax.Array):
            v = jnp.full(shape, v, f32)
        g = cat([cat([v[i * SR:(i + 1) * SR, j * Q:(j + 1) * Q] if x is None else x for j, x in enumerate(r)], 1)
                 for i, r in enumerate(gates)], 0)
        return jnp.where(jnp.full(shape, self.it, jnp.int32) < 0, g, v)

    def add(self, gen, deadline, cost, bg=False):
        (self.bg if bg else self.q).append([gen, deadline, cost])
        return gen

    def step(self, q, gate=None):
        self.g = gate
        c = None
        while q and c is None:
            c = next(q[0][0], None)
            if c is None:
                q.pop(0)
        if c is not None:
            self.lock = None if isinstance(c, float) else q
            q[0][2] -= c
        self.g = None
        return c

    def tick(self, val, base, brate):
        rate, cum = base, 0.0
        for _, dl, cost in self.q:
            cum += max(cost, 0)
            rate = max(rate, cum / max(dl - self.opt["margin"] - self.t, 1))
        self.bcredit = min(self.bcredit + brate + (0.0 if self.q else base), 40.0)
        self.pace = min(self.pace + rate + (brate if self.bg else 0.0), 40.0)
        if self.pace > 0:
            if self.lock:
                q = self.lock
            elif self.bg and (not self.q or (self.bcredit > 0 and rate <= base)):
                q = self.bg
            else:
                q = self.q
            if q:
                r = self.opt["row"]
                c = self.step(q, val[r * SR:(r + 1) * SR])
                if c:
                    self.pace -= c
                    if q is self.bg:
                        self.bcredit -= c
        self.t += 1

    def drain(self, gen=None, bg=False):
        q = self.bg if bg else self.q
        while q and (gen is None or any(e[0] is gen for e in q)):
            self.step(q)


def load_panel(get, o, p):
    return cat([get(br, bc * Q, (bc + 1) * Q).astype(f32) for br, bc in (rc(o, p, q) for q in range(4))], 1)


def load_z(ref):
    get = lambda br, c0, c1: ref[br * R:(br + 1) * R, c0:c1]
    return [[load_panel(get, o, p) for p in range(4)] for o in range(4)]


def rescale(x, f):
    return cat([cols(x, q) if f(q) == 1.0 else cols(x, q) * f(q) for q in range(4)], 1)


def to_basis(dd, x=None, e=None):
    d = cat(phi3(dd), 0)
    return cat([comb2(cols(d, i), sg, cols(d, j), None if x is None else cols(x, b), None if e is None else cols(e, b))
                for b, (i, sg, j) in enumerate(PHI4)], 1)


def basis1(v):
    d1, d0 = to_basis(v[1]), to_basis(v[0])
    return [to_basis(v[3], d0), d0 - d1, d0 + d1, to_basis(v[2], d1)]


def head(S, z, hs_ref, dl):
    def job():
        g = {o: [[None] * 4 for _ in range(NS)] for o in range(4)}
        for s in range(NS):
            for o in (1, 2, 0, 3):
                for q in QORD:
                    g[o][s][q] = S.g
                    if (s, o, q) == (NS - 1, 3, QORD[-1]):
                        v = [[rescale(z[o][p], lambda q: scale(*rc(o, p, q))) for p in range(4)] for o in range(4)]
                        for b, x in enumerate(basis1([[S.gated(g[o], v[o][0])] + v[o][1:] for o in range(4)])):
                            hs_ref[b] = x
                    yield 22.0 if q == QORD[-1] else 22

    return S.add(job(), dl, 16 * NS * 22)


def cross(S, dl, o, terms, z, bt_ref, l, emit=None, xo=None, out=None, peak=None):
    last = emit is None
    qord = TORD if last else QORD
    post = {1: 23, 0: 13, 3: 13, 2: 13} if last else {q: (4 if o < 2 else 12) * n for q, n in zip(QORD, (0, 1, 2, 1))}
    cost = {q: 17 + 4 * len(terms) + post[q] for q in qord}

    def finish(g1, g2):
        c = chain([(sg, m()) for sg, m in terms])
        y = psi([rows(c, p) for p in range(4)], S.gated(g1, 0.5))
        if peak is not None and o in (0, 3):
            sq = [cols(y[p], q) * cols(y[p], q) for q in (0, 3) for p in (0, 3)]
            sq = jnp.maximum(jnp.maximum(sq[0], sq[1]), jnp.maximum(sq[2], sq[3]))
            peak[o // 3] = functools.reduce(lambda a, b: jnp.maximum(b, a), [sq[s * SR:(s + 1) * SR] for s in range(NS)])
        bias = lambda br, c0, c1: bt_ref[l * 4 + popc(br), :, c0:c1]
        dd = [(y[p] + cat([load_panel(bias, o, p)] * NS, 0)) * z[p] for p in range(4)]
        if not last:
            return emit(dd)
        x = xo()
        x = cat(phi4_inv([cols(x, q) for q in range(4)]), 1)
        e = [rows(x, p) for p in range(4)]
        a11 = S.gated(g2, 0.5) * (e[1] + e[2])
        a22 = e[0] - a11
        xn = [a11, e[2] - a11, ((e[3] - a22) + e[3]) - e[2], a22]
        for p in range(4):
            r = rescale(dd[p] + xn[p], lambda q: 1.0 / scale(*rc(o, p, q)))
            br, bc = rc(o, p, 0)
            for t in range(2):
                out[(br + t) * R:(br + t + 1) * R, bc * Q:(bc + 2) * Q] = r[:, 2 * t * Q:2 * (t + 1) * Q].astype(bf16)

    def job():
        g1, g2 = ([[None] * 4 for _ in range(NS)] for _ in range(2))
        for s in range(NS):
            yield 1
            yield 1
            for q in qord:
                cc = cost[q]
                g1[s][q] = S.g
                if last:
                    cc = cost[q] // 2
                    yield cost[q] - cc
                    g2[s][q] = S.g
                if (s, q) == (NS - 1, qord[-1]):
                    finish(g1, g2)
                yield float(cc) if q == qord[-1] else cc

    return S.add(job(), dl, NS * (2 + sum(cost.values())), bg=last)


def tail(S, z, bt_ref, out, peak, ts_ref, L, quads=(0, 1, 2, 3)):
    for o in quads:
        g = cross(S, 0, o, [(sg, functools.partial(lambda n: ts_ref[n], 4 + NAMES.index(n))) for sg, n in TERMS[o]],
                  z[o], bt_ref, L - 1, xo=functools.partial(lambda n: ts_ref[n], o), out=out, peak=peak)
    return g


def unbasis1(S, X, ts_ref):
    g = [[None] * 2 for _ in range(4 * NS)]
    for s in range(NS):
        for p in range(4):
            for t in range(2):
                g[p * NS + s][t] = S.g
                if (s, p, t) == (NS - 1, 3, 1):
                    hf = S.gated(g, 0.5)
                    if isinstance(hf, jax.Array):
                        hf = cat([cols(hf, q // 2) for q in range(4)], 1)
                    for o, x in enumerate(phi4_inv([X[b]() for b in range(4)], hf)):
                        ts_ref[o] = x
                yield S.opt["ic"]


def level3(mul, order):
    need = {"v": {1: 1, 3: 1, 5: -1}, 1: {3: 1, 5: 1}, 0: {"v": 1, 4: 1, 7: 1}, 3: {"v": 1, 6: 1, 2: -1},
            2: {"h": 1, 4: 1, 7: -1, 6: 1, 2: 1}}
    acc = {n: None for n in need}
    left = {n: set(t) for n, t in need.items()}
    for k in order:
        todo = [(k, mul(k))]
        while todo:
            name, v = todo.pop(0)
            for n, t in need.items():
                if name in left[n]:
                    left[n].discard(name)
                    acc[n] = sadd(acc[n], (t[name], v))
                    if not left[n] and n in ("v", 1):
                        todo.append(("v" if n == "v" else "h", acc[n][1]))
    assert all(a[0] > 0 for a in acc.values())
    return cat([acc[q][1] for q in range(4)], 1)


def level2(mul):
    c0 = mul(1)
    m4 = mul(4)
    c0 = m4 + c0
    c2 = mul(2) + m4
    m7 = mul(7)
    c0 = m7 + c0
    c1 = mul(6) - m7
    m5 = mul(5)
    c0 = c0 - m5
    return cat([c0, c1, c2, mul(3) + m5], 0)


def body(it, x_prev, x_cur, x_next, out, pk_ref, bt_ref, t_ref, hs_ref, ts_ref, L, groups, opt):
    S = Sched(it, opt)
    cum = [0]
    for i in ORDER1:
        cum.append(cum[-1] + sum(8 if groups[(i, j)][1] else 7 for j in range(1, 8)))
    TL, mg = cum[-1], opt["margin"]
    z = load_z(x_cur)
    X = {b: hs_ref[b] for b in range(4)}
    pre = [10 * opt["pre"]]
    need = None
    tl = tail(S, load_z(x_prev), bt_ref, out, pk_ref.at[it - 1, 1], ts_ref, L)

    for l in range(L):
        T0 = l * TL
        last = l == L - 1

        def dot(u, n):
            return jnp.dot(u, t_ref[l, n // TW, :, (n % TW) * Q:(n % TW + 1) * Q], preferred_element_type=f32)

        def level1(i):
            base = opt["rates%d" % l][ORDER1.index(i)]
            brate = opt.get("brates%d" % l, opt["brates"])[ORDER1.index(i)]

            def group(j):
                a = lin([(s1 * s2, rows(X[b1], b2)) for s1, b1 in CORE4[i] for s2, b2 in CORE3[j]])
                a = [cols(a, q) for q in range(4)]
                n, plain = groups[(i, j)]
                if plain:
                    an = phi4_inv(a)
                    k0 = cat([an[0], an[2]], 0).astype(bf16)
                    k1 = cat([an[1], an[3]], 0).astype(bf16)

                    def mul2(u, k):
                        r = dot(u, n + k)
                        S.tick(r[:R], base, brate)
                        S.tick(r[R:], base, brate)
                        return r

                    c0 = mul2(k0, 0) + mul2(k1, 2)
                    c1 = mul2(k0, 1) + mul2(k1, 3)
                    return cat([c0[:R], c1[:R], c0[R:], c1[R:]], 1)

                def mul(k):
                    u = lin([(s3, a[b]) for s3, b in CORE4[k]])
                    if len(CORE4[k]) == 2:
                        for r0 in (0, 2 * SR):
                            if pre[0] > 0:
                                S.step(S.bg, u[r0:r0 + SR])
                                pre[0] -= 1
                    r = dot(u.astype(bf16), n + k - 1)
                    S.tick(r, base, brate)
                    return r

                return level3(mul, opt["od%d" % l])

            return level2(group)

        XN, D, M, nn = {}, {}, {}, {}

        def emitter(o, X=X, XN=XN, D=D):
            def emit(dd):
                if o < 2:
                    D[o] = to_basis(dd)
                if o == 0:
                    XN[1] = (D[0] + X[1]) - D[1]
                    XN[2] = (D[0] + X[2]) + D[1]
                elif o == 3:
                    XN[0] = to_basis(dd, X[0], D[0])
                elif o == 2:
                    XN[3] = to_basis(dd, X[3], D[1])
            return emit

        def keep(name, m):
            M[name] = m
            if last:
                ts_ref[4 + NAMES.index(name)] = m

        def add(o, dl):
            if not last:
                nn[o] = cross(S, dl, o, [(sg, functools.partial(M.get, n)) for sg, n in TERMS[o]], z[o], bt_ref, l,
                              emit=emitter(o), peak=pk_ref.at[it, 0] if l == 0 else None)

        if last:
            S.drain(tl, bg=True)
        if need:
            S.drain(need[0])
        m3 = level1(3)
        m5 = level1(5)
        if last:
            S.add(unbasis1(S, [functools.partial(X.get, b) for b in range(4)], ts_ref), T0 + TL + opt["endm"],
                  NS * 8 * opt["ic"])
            head(S, load_z(x_next), hs_ref, T0 + TL + opt["endm"])
        keep("h", m5 + m3)
        v = m3 - m5
        add(1, T0 + cum[5] + mg)
        if need:
            S.drain(need[3])
        keep("v", level1(1) + v)
        keep("m4", level1(4))
        keep("m7", level1(7))
        add(0, T0 + TL)
        if need:
            S.drain(need[2])
        keep("m6", level1(6))
        keep("m2", level1(2))
        add(3, T0 + TL + cum[2])
        add(2, T0 + TL + cum[5])
        need, X = nn, XN
    S.drain()


def tform(e, k):
    if k == 1:
        return e[0] + e[0]
    return lin([(s, e[b]) for s, b in CORE4[SIGMA[k]]])


def table_job(S, w_ref, tb_ref, l, groups):
    ga = {o: [[None] * 4 for _ in range(Q // SR)] for o in range(4)}
    gb = {(i, b): [None] * (Q // CR) for i in range(1, 8) for b in range(4)}
    js = {b: [j for j in range(1, 8) if max(t for _, t in CORE3[SIGMA[j]]) == b] for b in range(4)}
    for c in range(Q // CR):
        for s in range(c * CR // SR, (c + 1) * CR // SR):
            for o in (1, 2, 0, 3):
                for q in QORD:
                    ga[o][s][q] = S.g
                    yield S.opt["pc"][0]
        for i in S.opt["pi"]:
            for b in range(4):
                gb[(i, b)][c] = S.g
                yield S.opt["pc"][1] + S.opt["pc"][2] * len(js[b])
    v = []
    for o in range(4):
        w = [load_panel(lambda br, c0, c1: w_ref[br, :, c0:c1], o, p) for p in range(4)]
        sc = cat([jnp.full((Q, Q), 0.25 * scale(*rc(o, 0, q)), f32) for q in range(4)], 1)
        v.append([w[0] * S.gated(ga[o], sc)]
                 + [rescale(w[p], lambda q: 0.25 * scale(*rc(o, p, q))) for p in range(1, 4)])
    E = basis1(v)
    for i in range(1, 8):
        if i == 1:
            two = S.gated([[gb[(i, b)][c]] for b in range(4) for c in range(Q // CR)], 2.0)
            two = cat([two[t // 2 * SR:(t // 2 + 1) * SR] for t in range(4 * Q // SR)], 0)
            s1 = cat([two] * 4, 1) * E[0]
        else:
            first = CORE4[SIGMA[i]][0][1]
            g = [[gb[(i, b)][s * SR // CR]] * 4 for b in range(4) for s in range(Q // SR)]
            s1 = tform([S.gated(g, E[b]) if b == first else E[b] for b in range(4)], i)
        for j in range(1, 8):
            e = lin([(sg, s1[b * Q:(b + 1) * Q]) for sg, b in CORE3[SIGMA[j]]])
            e = [cols(e, q) for q in range(4)]
            n, plain = groups[(i, j)]
            if plain:
                a, b = e[1] + e[2], e[2] - e[1]
                outs = [a, b, (e[3] - b) + e[3], (e[0] - a) + e[0]]
            else:
                outs = [tform(e, k) for k in range(1, 8)]
            for k, t in enumerate(outs):
                c0 = ((n + k) % TW) * Q
                tb_ref.at[l, (n + k) // TW][:, c0:c0 + Q] = t.astype(bf16)


def first_layer(l, w_ref, z_ref, xi_ref, xo_ref, pr_ref, wn_ref, bt_ref, tb_ref, groups, opt):
    S = Sched(l, opt)
    S.add(table_job(S, w_ref, tb_ref, l, groups), 0, 0)
    pc = opt["pc"]
    rate = (Q // CR) * (32 * pc[0] + 7 * (4 * pc[1] + 7 * pc[2])) / (16 * TM // SR - opt["pres"])
    pace = 0.0
    x = xi_ref[...]
    xb = cat([x, pr_ref[...]], 0).astype(bf16)
    wn = None
    for n in range(8):
        cs = slice(n * Q, (n + 1) * Q)
        acc = None
        for kh in range(2):
            rs = [jnp.dot(cols(xb, k), w_ref[k, :, cs], preferred_element_type=f32) for k in range(4 * kh, 4 * kh + 4)]
            oth = (rs[1] + rs[2]) + rs[3]
            acc = oth if acc is None else acc + oth
            for g in range(TM // SR):
                pace += rate
                for r in (rs[opt["pg"]], rs[3]):
                    if pace > 0:
                        pace -= S.step(S.q, r[g * SR:(g + 1) * SR]) or 0
            acc = acc + rs[0]
        xo_ref[:, cs] = z_ref[:, cs] * (acc[:TM] + bt_ref[l * 4 + popc(n), 0:1, cs]) + x[:, cs]
        wn = acc[TM:] * acc[TM:] if wn is None else wn + acc[TM:] * acc[TM:]
    wn_ref[pl.ds(pl.multiple_of(l * NP, NP), NP), :] = wn
    S.drain()


def kernel(x_hbm, w_hbm, b_hbm, o_hbm, t_ref, bt_ref, hs_ref, ts_ref, xs_ref, w_buf, x_buf, o_buf, o0_buf, b_buf,
           pr_ref, wn_ref, pk_ref, w_sem, x_sem, o_sem, m_sem, *, L, nb, groups, opt):
    D = 8 * Q

    def wcopy(l):
        return pltpu.make_async_copy(w_hbm.at[l], w_buf.at[l], w_sem.at[l & 1])

    def xcopy(i, n=1):
        return pltpu.make_async_copy(x_hbm.at[pl.ds(i, n)], x_buf.at[pl.ds(i, n)], x_sem.at[4 + i])

    def gcopy(g):
        return pltpu.make_async_copy(x_hbm.at[pl.ds(g * XG, XG)], x_buf.at[pl.ds((g & 3) * XG, XG)], x_sem.at[g & 3])

    def ocopy(i):
        return pltpu.make_async_copy(o_buf.at[i & (NO - 1)], o_hbm.at[pl.ds(pl.multiple_of(i * TM, TM), TM), :],
                                     o_sem.at[i & (NO - 1)])

    bcopy = pltpu.make_async_copy(b_hbm, b_buf, m_sem.at[0])
    bcopy.start()
    xcopy(0).start()
    wcopy(0).start()
    ts_ref[...] = jnp.zeros(ts_ref.shape, f32)
    bcopy.wait()
    b = b_buf[...].astype(f32)
    for e in range(4):
        be = cat([cols(b, bc) * S3 ** (e - popc(bc)) for bc in range(8)], 1)
        for l in range(L):
            bt_ref[l * 4 + e] = jnp.broadcast_to(be[l:l + 1], (SR, 8 * Q))
    hsh = (jax.lax.broadcasted_iota(jnp.int32, (NP, D), 0) * D + jax.lax.broadcasted_iota(jnp.int32, (NP, D), 1))
    for _ in range(2):
        hsh = (hsh ^ (hsh >> 15)) * 739982445
    pr_ref[...] = jnp.where((hsh ^ (hsh >> 15)) & 256 == 0, 1.0, -1.0)
    xcopy(0).wait()
    xs_ref[0] = x_buf[0].astype(f32)
    xs_ref[2] = x_buf[0].astype(f32)
    tb_ref = t_ref.bitcast(bf16)
    wcopy(0).wait()

    def first(l, carry):
        nxt = wcopy(jnp.minimum(l + 1, L - 1))
        pl.when(l + 1 < L)(nxt.start)

        @pl.when(l + 1 == L)
        def _():
            xcopy(1).start()
            xcopy(2).start()

        first_layer(l, w_buf.at[l], xs_ref.at[2], xs_ref.at[l & 1], xs_ref.at[1 - (l & 1)], pr_ref, wn_ref, bt_ref,
                    tb_ref, groups, opt)
        pl.when(l + 1 < L)(nxt.wait)
        return carry

    jax.lax.fori_loop(0, L, first, 0)
    o0_buf[...] = xs_ref[L % 2].astype(bf16)
    o0copy = pltpu.make_async_copy(o0_buf, o_hbm.at[pl.ds(0, TM), :], m_sem.at[1])
    o0copy.start()
    xcopy(1).wait()
    S = Sched(None, opt)
    head(S, load_z(x_buf.at[1]), hs_ref, 0)
    S.drain()

    def dmas(i):
        g, ng = (i + 1) >> 3, nb // XG
        turn = ((i + 1) & (XG - 1)) == 0
        cps = [gcopy(jnp.minimum(g + 1, ng - 1)), ocopy(jnp.maximum(i - 2, 1)),
               gcopy(jnp.minimum(g, ng - 1)), ocopy(jnp.maximum(i - 3, 1))]
        pl.when(turn & (g + 1 < ng))(cps[0].start)
        pl.when(i >= 3)(cps[1].start)
        pl.when(turn & (g < ng))(cps[2].wait)
        pl.when(i == 2)(xcopy(3, XG - 3).wait)
        pl.when(i >= 4)(cps[3].wait)

    def step(i, carry):
        xs = [x_buf.at[jnp.clip(i + u, 0, nb - 1) & (NX - 1)] for u in (-1, 0, 1)]
        body(i, *xs, o_buf.at[(i + 1) & (NO - 1)], pk_ref, bt_ref, tb_ref, hs_ref, ts_ref, L, groups, opt)
        dmas(i + 1)
        return carry

    xcopy(2).wait()
    xcopy(3, XG - 3).start()
    gcopy(1).start()
    jax.lax.fori_loop(1, nb, step, 0)

    last, H = nb - 1, TM // 2
    z = load_z(x_buf.at[last % NX])
    halves = [pltpu.make_async_copy(o_buf.at[last % NO, pl.ds(h * H, H), :],
                                    o_hbm.at[pl.ds(last * TM + h * H, H), :], m_sem.at[2 + h]) for h in range(2)]
    S = Sched(None, opt)
    for h in range(2):
        tail(S, z, bt_ref, o_buf.at[last % NO], pk_ref.at[last, 1], ts_ref, L, (2 * h, 2 * h + 1))
        S.drain(bg=True)
        halves[h].start()
    o0copy.wait()
    ocopy(last - 1).wait()

    wn = [jnp.sum(jnp.sum(wn_ref[l * NP:(l + 1) * NP, :], axis=0, keepdims=True), axis=1, keepdims=True) for l in range(L)]
    tot = functools.reduce(lambda a, b: a + b, wn) * (1.0 / Q)
    gain = [tot / wn[0], tot / wn[L - 1]]

    def risky(i, n):
        pk = [jnp.maximum(pk_ref[pl.ds(i, n), t, 0], pk_ref[pl.ds(i, n), t, 1]).reshape(n * SR, Q) * gain[t]
              for t in range(2)]
        return jnp.logical_not(jnp.max(jnp.sum(jnp.maximum(pk[0], pk[1]), axis=1, keepdims=True)) <= opt["limit"])

    redo = risky(1, last)
    for h in range(2):
        halves[h].wait()

    def chunk(c, carry):
        rs = pl.ds(pl.multiple_of(c * R, R), R)
        z = o0_buf[rs, :].astype(f32)

        def layer(l, x):
            y = jnp.dot(x.astype(bf16), w_buf[l].reshape(D, D), preferred_element_type=f32)
            b = cat([bt_ref[l * 4 + popc(n), 0:1, n * Q:(n + 1) * Q] for n in range(8)], 1)
            return z * (y + b) + x

        o0_buf[rs, :] = jax.lax.fori_loop(0, L, layer, z).astype(bf16)
        return carry

    def again(i, carry):
        @pl.when(risky(i, 1))
        def _():
            cp = pltpu.make_async_copy(x_hbm.at[i], o0_buf, m_sem.at[0])
            cp.start()
            cp.wait()
            jax.lax.fori_loop(0, TM // R, chunk, 0)
            cp = pltpu.make_async_copy(o0_buf, o_hbm.at[pl.ds(pl.multiple_of(i * TM, TM), TM), :], m_sem.at[0])
            cp.start()
            cp.wait()

        return carry

    @pl.when(redo)
    def _():
        jax.lax.fori_loop(1, nb, again, 0)


def make(o=None):
    opt = dict(OPT)
    opt.update(o or {})
    groups, n = plan()

    @jax.jit
    def run(x0, ws, bs):
        B, D = x0.shape
        L = ws.shape[0]
        assert D == 8 * Q and B % (XG * TM) == 0 and B >= 2 * XG * TM and L == 6 and n % TW == 0
        return pl.pallas_call(
            functools.partial(kernel, L=L, nb=B // TM, groups=groups, opt=opt),
            in_specs=[pl.BlockSpec(memory_space=pl.ANY)] * 3,
            out_specs=pl.BlockSpec(memory_space=pl.ANY),
            out_shape=jax.ShapeDtypeStruct((B, D), x0.dtype),
            scratch_shapes=[
                pltpu.VMEM((L, n // TW, Q // 2, TW * Q), jnp.uint32),
                pltpu.VMEM((L * 4, SR, D), f32),
                pltpu.VMEM((4, 4 * R, D // 2), f32),
                pltpu.VMEM((10, 4 * R, D // 2), f32),
                pltpu.VMEM((3, TM, D), f32),
                pltpu.VMEM((L, 8, Q, D), bf16),
                pltpu.VMEM((NX, TM, D), bf16),
                pltpu.VMEM((NO, TM, D), bf16),
                pltpu.VMEM((TM, D), bf16),
                pltpu.VMEM((L, D), bf16),
                pltpu.VMEM((NP, D), f32),
                pltpu.VMEM((L * NP + 3 * SR, Q), f32),
                pltpu.VMEM((B // TM, 2, 2, SR, Q), f32),
                pltpu.SemaphoreType.DMA((2,)),
                pltpu.SemaphoreType.DMA((8,)),
                pltpu.SemaphoreType.DMA((NO,)),
                pltpu.SemaphoreType.DMA((4,)),
            ],
            compiler_params=pltpu.CompilerParams(vmem_limit_bytes=116 * 1024 * 1024, disable_bounds_checks=True),
        )(x0.reshape(B // TM, TM, D), ws.reshape(L, 8, Q, D), bs)

    return run


_run = make()


@jax.jit
def pallas_standalone__dcn_v2_cross__recsys_kernel(x0: jax.Array, ws: jax.Array, bs: jax.Array):
    return _run(x0, ws, bs)
```
